```python
import jax
import jax.numpy as jnp

def _softmax(x, axis=-1):
    return jax.nn.softmax(x, axis=axis)

def _gelu(x):
    return jax.nn.gelu(x, approximate=True)

def _silu(x):
    return jax.nn.silu(x)

def _sigmoid(x):
    return jax.nn.sigmoid(x)

def _layernorm(x, axis=-1, eps=1e-05):
    m = jnp.mean(x, axis=axis, keepdims=True)
    v = jnp.var(x, axis=axis, keepdims=True)
    return (x - m) / jnp.sqrt(v + eps)

def _scatter_add(tgt, idx, src, axis=0):
    return tgt.at[idx].add(src)

def _segment_sum(src, seg, n):
    return jax.ops.segment_sum(src, seg, n)

class _Rng:

    def __init__(self, key):
        self._k = key

    def _next(self):
        self._k, sub = jax.random.split(self._k)
        return sub

    def normal(self, shape):
        return jax.random.normal(self._next(), shape, dtype=jnp.bfloat16)

    def randint(self, lo, hi, shape):
        return jax.random.randint(self._next(), shape, lo, hi, dtype=jnp.int32)

    def uniform(self, shape, lo=0.0, hi=1.0):
        return jax.random.uniform(self._next(), shape, jnp.bfloat16, lo, hi)

    def permutation(self, n):
        return jax.random.permutation(self._next(), n)
kernel_name = 'adaLN_cond__compressed_kv_cla__moe_arch_mod__prompt'

def setup_inputs():
    _rng = _Rng(jax.random.key(int.from_bytes(__import__("os").urandom(4), "little")))
    _w = lambda a: (lambda t: t.astype(jnp.bfloat16) if jnp.issubdtype(t.dtype, jnp.floating) else t)(jnp.asarray(a))

    def _A_setup():
        B, H, Sq, Sk, D, M = (1, 32, 2048, 2048, 128, 640)
        Dc = 4 * D
        return {'x': _w((lambda *s: _rng.normal(s) * 0.05)(B, Sq, M)), 'c_kv': _w((lambda *s: _rng.normal(s) * 0.05)(B, Sk, Dc)), 'w_q': _w((lambda *s: _rng.normal(s) * 0.05)(M, H, D) * M ** (-0.5)), 'w_uk': _w((lambda *s: _rng.normal(s) * 0.05)(Dc, H, D) * Dc ** (-0.5)), 'w_uv': _w((lambda *s: _rng.normal(s) * 0.05)(Dc, H, D) * Dc ** (-0.5)), 'w_o': _w((lambda *s: _rng.normal(s) * 0.05)(H, D, M) * (H * D) ** (-0.5))}
    _A_in = _A_setup()

    def _B_setup():
        B, S, D, F, C = (1, 2048, 640, 1728, 8)
        return {'x': _w((lambda *s: _rng.normal(s) * 0.05)(B, S, D)), 'w_r': _w((lambda *s: _rng.normal(s) * 0.05)(D)), 'w_gate': _w((lambda *s: _rng.normal(s) * 0.05)(D, F)), 'w_up': _w((lambda *s: _rng.normal(s) * 0.05)(D, F)), 'w_down': _w((lambda *s: _rng.normal(s) * 0.05)(F, D))}
    _B_in = _B_setup()
    return {'A_x': _A_in['x'], 'A_c_kv': _A_in['c_kv'], 'A_w_q': _A_in['w_q'], 'A_w_uk': _A_in['w_uk'], 'A_w_uv': _A_in['w_uv'], 'A_w_o': _A_in['w_o'], 'B_x': _B_in['x'], 'B_w_r': _B_in['w_r'], 'B_w_gate': _B_in['w_gate'], 'B_w_up': _B_in['w_up'], 'B_w_down': _B_in['w_down'], 'c': _w((lambda *s: _rng.normal(s) * 0.05)(1, 640)), 'w_mod': _w((lambda *s: _rng.normal(s) * 0.05)(640, 6 * 640) * 640 ** (-0.5))}

def reference(A_x, A_c_kv, A_w_q, A_w_uk, A_w_uv, A_w_o, B_x, B_w_r, B_w_gate, B_w_up, B_w_down, c, w_mod):

    def _A_ref(x, c_kv, w_q, w_uk, w_uv, w_o):
        B, Sq, M = (x.shape[0], x.shape[1], x.shape[2])
        Sk = c_kv.shape[1]
        H, D = (w_q.shape[1], w_q.shape[2])
        q = jnp.einsum('bqm,mhd->bhqd', x, w_q)
        k = jnp.einsum('bkc,chd->bhkd', c_kv, w_uk)
        v = jnp.einsum('bkc,chd->bhkd', c_kv, w_uv)
        scores = jnp.einsum('bhqd,bhkd->bhqk', q, k) * D ** (-0.5)
        off = Sk - Sq
        qi = jnp.arange(Sq)[:, None]
        kj = jnp.arange(Sk)[None, :]
        cmask = kj <= qi + off
        scores = jnp.where(cmask[None, None], scores, -1000000000.0)
        p = _softmax(scores, axis=-1)
        ctx = jnp.einsum('bhqk,bhkd->bhqd', p, v)
        return jnp.einsum('bhqd,hdm->bqm', ctx, w_o)

    def _B_ref(x, w_r, w_gate, w_up, w_down):
        B, S, D = x.shape
        C = 8
        r = x @ w_r
        idx = jnp.argsort(-r, axis=-1)[:, :C]
        idx_e = jnp.repeat(idx.reshape(B, C, 1), D, axis=2)
        x_sel = jnp.take_along_axis(x, idx_e, axis=1)
        g = _silu(x_sel @ w_gate)
        u = x_sel @ w_up
        y = g * u @ w_down
        r_sel = _sigmoid(jnp.take_along_axis(r, idx, axis=1))
        y = y * r_sel.reshape(B, C, 1)
        b_off = (jnp.arange(B) * S).reshape(B, 1)
        flat_idx = (idx + b_off).reshape(B * C)
        zero = (x * 0.0).reshape(B * S, D)
        upd = _scatter_add(zero, flat_idx, y.reshape(B * C, D), axis=0)
        return x + upd.reshape(B, S, D)
    x = A_x
    mod = (_silu(c) @ w_mod).reshape(c.shape[0], 6, 1, -1)
    sa, ca, ga, sb, cb, gb = (mod[:, 0].copy(), mod[:, 1].copy(), mod[:, 2].copy(), mod[:, 3].copy(), mod[:, 4].copy(), mod[:, 5].copy())
    h = _layernorm(x, axis=-1) * (1 + ca) + sa
    x = x + ga * _A_ref(h, A_c_kv, A_w_q, A_w_uk, A_w_uv, A_w_o)
    h = _layernorm(x, axis=-1) * (1 + cb) + sb
    x = x + gb * _B_ref(h, B_w_r, B_w_gate, B_w_up, B_w_down)
    return x
```

```python
import jax
import jax.numpy as jnp
from jax import lax
import jax.experimental.pallas as pl
import jax.experimental.pallas.tpu as pltpu

S, M, C, D, H, F, TOPK = 2048, 640, 512, 128, 32, 1728, 8
G = 8
NG = H // G
T = 128
NB = S // T
CH = 4
RB = 256
EPS = 1e-5
QSCALE = D ** -0.5 * 1.4426950408889634
NT = (((1,), (1,)), ((), ()))

f32, bf16, u32, i32 = jnp.float32, jnp.bfloat16, jnp.uint32, jnp.int32


def _rb(a):
    return a.astype(bf16).astype(f32)


def _sigmoid(a):
    return _rb(1.0 / _rb(1.0 + _rb(jnp.exp(-a))))


def _rows(r0, n):
    if isinstance(r0, int):
        return pl.ds(r0, n)
    return pl.ds(pl.multiple_of(r0, n), n)


def _ld(ref, *idx, r0, n):
    return pltpu.bitcast(ref[(*idx, _rows(r0 // 2, n // 2), slice(None))], bf16)


def _st(ref, *idx, r0, val):
    ref[(*idx, _rows(r0 // 2, val.shape[0] // 2), slice(None))] = pltpu.bitcast(
        val.astype(bf16), u32)


def _dot(a, b):
    return jnp.dot(a, b, preferred_element_type=f32)


def _dot_nt(a, b):
    return lax.dot_general(a, b, NT, preferred_element_type=f32)


class _Blk:
    def __init__(self, i):
        self.i, self.s, self.mx, self.m, self.l, self.acc = i, {}, None, None, None, None


def _attention(q_s, k_s, v_s, ctx_s, hd, slot, filler):
    tri = (lax.broadcasted_iota(i32, (T, T), 1) <= lax.broadcasted_iota(i32, (T, T), 0))

    def chunks(b):
        n = b.i + 1 if b else 0
        return [(a, min(a + CH, n)) for a in range(0, n, CH)]

    def scores(b, a, e):
        return _dot_nt(_ld(q_s, slot, r0=b.i * T, n=T), _ld(k_s, hd, r0=a * T, n=(e - a) * T))

    def keep(b, a, e, s):
        for t in range(a, e):
            x = s[:, (t - a) * T:(t - a + 1) * T]
            if t == b.i:
                x = jnp.where(tri, x, -1e9)
            b.mx = x if b.mx is None else jnp.maximum(b.mx, x)
            b.s[t] = x

    def context(b, a, e):
        ps = []
        for t in range(a, e):
            p = jnp.exp2(b.s[t] - b.m)
            b.l = p if b.l is None else b.l + p
            ps.append(p)
        p = (jnp.concatenate(ps, axis=1) if len(ps) > 1 else ps[0]).astype(bf16)
        o = _dot(p, _ld(v_s, slot, r0=a * T, n=(e - a) * T))
        b.acc = o if b.acc is None else b.acc + o

    def finish(b):
        l = jnp.sum(b.l, axis=1, keepdims=True)
        r = pltpu.reciprocal(l, approx=True)
        r = r * (2.0 - l * r)
        _st(ctx_s, hd, r0=b.i * T, val=b.acc * r)

    filler(0)
    prev = None
    for n, i in enumerate(list(range(NB - 1, -1, -1)) + [None]):
        b = _Blk(i) if i is not None else None
        ca, cb = chunks(b), chunks(prev)
        for c in range(max(len(ca), len(cb))):
            s = scores(b, *ca[c]) if c < len(ca) else None
            if c < len(cb):
                context(prev, *cb[c])
            if s is not None:
                keep(b, *ca[c], s)
        if b:
            b.m = jnp.max(b.mx, axis=1, keepdims=True)
        if prev:
            finish(prev)
        filler(n + 1)
        prev = b


def _kernel(x_hbm, ckv_hbm, wq_hbm, wk_hbm, wv_hbm, wo_hbm, wr_hbm, wg_hbm, wu_hbm, wd_hbm,
            c_hbm, wmod_hbm, out_hbm,
            x_s, ckv_s, wq_raw, wk_raw, wv_raw, wq_s, wk_s, wv_s, wo_s, wr_s, wg_s, wu_s, wd_s,
            c_s, wmod_s, mod_s, h_s, k_s, q_s, v_s, ctx_s, y_s, x1_s, h2_s, r_s, out_s,
            in_sem, out_sem, fix_sem):
    sem_ids = {}

    def copy(name, src, dst):
        return pltpu.make_async_copy(src, dst, in_sem.at[sem_ids.setdefault(name, len(sem_ids))])

    def group(name, hbm, raw, g):
        return copy((name, g), hbm.at[:, pl.ds(g * G, G), :], raw.at[g])

    NC = 4
    ckv_cp = [copy(("ckv", j), ckv_hbm.at[pl.ds(j * (S // NC), S // NC)],
                   ckv_s.at[pl.ds(j * (S // NC), S // NC)]) for j in range(NC)]
    wk_cp = [group("wk", wk_hbm, wk_raw, g) for g in range(NG)]
    wq_cp = [group("wq", wq_hbm, wq_raw, g) for g in range(NG)]
    wv_cp = [group("wv", wv_hbm, wv_raw, g) for g in range(NG)]
    x_cp, c_cp, wmod_cp = copy("x", x_hbm, x_s), copy("c", c_hbm, c_s), copy("wm", wmod_hbm, wmod_s)
    late_cp = [copy("wo", wo_hbm, wo_s), copy("wr", wr_hbm, wr_s), copy("wg", wg_hbm, wg_s),
               copy("wu", wu_hbm, wu_s), copy("wd", wd_hbm, wd_s)]

    def relayout(raw, g):
        return raw[g].reshape(raw.shape[1], G * D)

    def per_head(raw, dst, g):
        w = relayout(raw, g)
        for j in range(G):
            dst[g * G + j] = w[:, j * D:(j + 1) * D]

    def kproj(g, r0, n):
        k = _dot(ckv_s[pl.ds(r0, n), :], wk_s[g % 2])
        for j in range(G):
            _st(k_s, g * G + j, r0=r0, val=k[:, j * D:(j + 1) * D])

    def mod(j):
        return mod_s[:, pl.ds(j * M, M)]

    def qproj(hd, slot, i):
        _st(q_s, slot, r0=i * T, val=_dot(_ld(h_s, r0=i * T, n=T), wq_s[hd]) * QSCALE)

    def vproj(hd, slot, i):
        _st(v_s, slot, r0=i * T, val=_dot(ckv_s[pl.ds(i * T, T), :], wv_s[hd]))

    wk_cp[0].start()
    ckv_cp[0].start()
    wk_cp[0].wait()
    for cp in ckv_cp[1:]:
        cp.start()
    wk_cp[1].start()
    wk_s[0] = relayout(wk_raw, 0)
    for j in range(NC):
        ckv_cp[j].wait()
        if j == 1:
            for cp in (c_cp, wmod_cp, x_cp, wk_cp[2]):
                cp.start()
        if j == NC - 1:
            wk_cp[1].wait()
            wk_s[1] = relayout(wk_raw, 1)
        kproj(0, j * (S // NC), S // NC)

    for cp in [wk_cp[3]] + wq_cp + wv_cp:
        cp.start()
    kproj(1, 0, S // 2)
    for cp in (c_cp, wmod_cp, x_cp, wk_cp[2]):
        cp.wait()
    cf = c_s[...].astype(f32)
    sc = jnp.broadcast_to(cf * _sigmoid(cf), (16, M)).astype(bf16)
    mod_s[...] = _rb(_dot(sc, wmod_s[...])[0:1])
    kproj(1, S // 2, S // 2)
    wk_s[0] = relayout(wk_raw, 2)

    wk_cp[3].wait()
    kproj(2, 0, S)
    wk_s[1] = relayout(wk_raw, 3)
    sa, ca = mod(0), 1.0 + mod(1)
    for i in range(NB):
        xf = x_s[pl.ds(i * T, T), :].astype(f32)
        xc = xf - jnp.mean(xf, axis=1, keepdims=True)
        xn = xc * lax.rsqrt(jnp.mean(xc * xc, axis=1, keepdims=True) + EPS)
        _st(h_s, r0=i * T, val=xn * ca + sa)

    for cp in wq_cp + wv_cp:
        cp.wait()
    for cp in late_cp:
        cp.start()
    kproj(3, 0, S)
    for g in range(NG):
        per_head(wq_raw, wq_s, g)
        per_head(wv_raw, wv_s, g)
    for i in range(NB):
        qproj(0, 0, i)
        vproj(0, 0, i)

    def next_head(hd, slot):
        jobs = [(f, i) for i in range(NB) for f in (qproj, vproj)]
        cuts = [0, 1] + [1 + (27 * n) // NB for n in range(1, NB + 1)] + [len(jobs)]

        def filler(n):
            for f, i in jobs[cuts[n]:cuts[n + 1]]:
                f(hd, slot, i)
        return filler

    def pair(p, _):
        _attention(q_s, k_s, v_s, ctx_s, 2 * p, 0, next_head(2 * p + 1, 1))
        _attention(q_s, k_s, v_s, ctx_s, 2 * p + 1, 1, next_head(2 * p + 2, 0))

    lax.fori_loop(0, H // 2 - 1, pair, None)

    for cp in late_cp:
        cp.wait()

    def oproj(r0, slot):
        ctx = jnp.concatenate([_ld(ctx_s, hd, r0=r0, n=RB) for hd in range(H)], axis=1)
        y_s[slot] = _dot(ctx, wo_s[...])

    def out_copy(b):
        return pltpu.make_async_copy(out_s.at[_rows(b * RB, RB)], out_hbm.at[_rows(b * RB, RB)],
                                     out_sem.at[b])

    def epilogue(b, slot):
        rows = _rows(b * RB, RB)
        ga, sb, cb, gb = mod(2), mod(3), _rb(1.0 + mod(4)), mod(5)
        x1 = _rb(x_s[rows, :].astype(f32) + _rb(ga * _rb(y_s[slot])))
        mean = jnp.mean(x1, axis=1, keepdims=True)
        xc = x1 - mean
        var = _rb(jnp.mean(xc * xc, axis=1, keepdims=True))
        inv = 1.0 / _rb(jnp.sqrt(_rb(var + EPS)))
        h2 = _rb(_rb(_rb(_rb(x1 - _rb(mean)) * inv) * cb) + sb)
        x1_s[rows, :] = x1
        h2_s[rows, :] = h2
        out_s[rows, :] = (x1 + _rb(gb * h2)).astype(bf16)
        wr = wr_s[...].astype(f32)
        part = h2[:, 0:D] * wr[0:1]
        for j in range(1, M // D):
            part = part + h2[:, j * D:(j + 1) * D] * wr[j:j + 1]
        r = jnp.sum(part, axis=1, keepdims=True)
        lane = lax.broadcasted_iota(i32, (8, S // 8), 1) - b * (RB // 8)
        acc = r_s[...]
        for t in range(RB // 8):
            acc = jnp.where(lane == t, r[8 * t:8 * t + 8], acc)
        r_s[...] = acc

    NR = S // RB
    r_s[...] = jnp.zeros(r_s.shape, f32)
    _attention(q_s, k_s, v_s, ctx_s, H - 2, 0, next_head(H - 1, 1))

    def last_filler(n):
        if n == 3:
            oproj((NR - 1) * RB, (NR - 1) % 2)

    _attention(q_s, k_s, v_s, ctx_s, H - 1, 1, last_filler)

    def block(n, _):
        b = NR - 2 - n
        oproj(b * RB, b % 2)
        epilogue(b + 1, (b + 1) % 2)
        out_copy(b + 1).start()

    lax.fori_loop(0, NR - 1, block, None)
    epilogue(0, 0)
    out_copy(0).start()

    r = _rb(r_s[...])
    bits = lax.bitcast_convert_type(r, i32)
    code = lax.shift_right_logical(bits, 16)
    code = jnp.where(bits < 0, 0xFFFF - code, code + 0x8000)
    code = jnp.where(r == 0.0, 0x8000, code)
    code = jnp.where(r != r, 0, code)
    tok = (lax.broadcasted_iota(i32, r.shape, 1) * 8 + lax.broadcasted_iota(i32, r.shape, 0))
    key = lax.bitcast_convert_type(code * S + (S - 1 - tok) + 0x00800000, f32)
    top = jnp.zeros((TOPK, D), f32)
    sub = lax.broadcasted_iota(i32, (TOPK, D), 0)
    for j in range(TOPK):
        best = jnp.max(jnp.max(key, axis=0, keepdims=True), axis=1, keepdims=True)
        key = jnp.where(key == best, 0.0, key)
        top = jnp.where(sub == j, best, top)
    top = lax.bitcast_convert_type(top, i32) - 0x00800000
    sel = S - 1 - (top & (S - 1))
    code = lax.shift_right_logical(top, 11)
    code = jnp.where(code >= 0x8000, code - 0x8000, 0xFFFF - code)
    r_sel = lax.bitcast_convert_type(code * 0x10000, f32)[:, 0:1]
    idx = [sel[j, 0] for j in range(TOPK)]

    hsel = jnp.concatenate([h2_s[pl.ds(t, 1), :] for t in idx], axis=0)
    xsel = jnp.concatenate([x1_s[pl.ds(t, 1), :] for t in idx], axis=0)
    lhs = jnp.concatenate([hsel, hsel], axis=0).astype(bf16)
    gate = _rb(_dot_nt(lhs, wg_s[...]))
    act = _rb(gate * _sigmoid(gate)) * _rb(_dot_nt(lhs, wu_s[...]))
    y = _rb(_rb(_dot(act.astype(bf16), wd_s[...])[0:TOPK]) * _sigmoid(r_sel))
    fixed = xsel + _rb(mod(5) * _rb(hsel + y))

    for b in range(NR):
        out_copy(b).wait()
    tiles = [pl.multiple_of((t // 16) * 16, 16) for t in idx]
    row = lax.broadcasted_iota(i32, (16, M), 0)
    for j in range(TOPK):
        cur = out_s[pl.ds(tiles[j], 16), :].astype(f32)
        cur = jnp.where(row == idx[j] - tiles[j], fixed[j:j + 1], cur)
        out_s[pl.ds(tiles[j], 16), :] = cur.astype(bf16)

    def fix_copy(j):
        return pltpu.make_async_copy(out_s.at[pl.ds(tiles[j], 16)], out_hbm.at[pl.ds(tiles[j], 16)],
                                     fix_sem.at[j])

    fresh = []
    for j in range(TOPK):
        new = tiles[j] >= 0
        for k in range(j):
            new = jnp.logical_and(new, tiles[j] != tiles[k])
        fresh.append(new)
    for j in range(TOPK):
        pl.when(fresh[j])(fix_copy(j).start)
    for j in range(TOPK):
        pl.when(fresh[j])(fix_copy(j).wait)


@jax.jit
def pallas_adaLN_cond__compressed_kv_cla__moe_arch_mod__prompt_kernel(
    A_x: jax.Array,
    A_c_kv: jax.Array,
    A_w_q: jax.Array,
    A_w_uk: jax.Array,
    A_w_uv: jax.Array,
    A_w_o: jax.Array,
    B_x: jax.Array,
    B_w_r: jax.Array,
    B_w_gate: jax.Array,
    B_w_up: jax.Array,
    B_w_down: jax.Array,
    c: jax.Array,
    w_mod: jax.Array,
):
    del B_x
    V = pltpu.VMEM
    scratch = [
        V((S, M), bf16), V((S, C), bf16),
        V((NG, M, G, D), bf16), V((NG, C, G, D), bf16), V((NG, C, G, D), bf16),
        V((H, M, D), bf16), V((2, C, G * D), bf16), V((H, C, D), bf16),
        V((H * D, M), bf16), V((M // D, D), bf16),
        V((F, M), bf16), V((F, M), bf16), V((F, M), bf16),
        V((1, M), bf16), V((M, 6 * M), bf16), V((1, 6 * M), f32),
        V((S // 2, M), u32), V((H, S // 2, D), u32),
        V((2, S // 2, D), u32), V((2, S // 2, D), u32), V((H, S // 2, D), u32),
        V((2, RB, M), f32), V((S, M), f32), V((S, M), f32),
        V((8, S // 8), f32), V((S, M), bf16),
        pltpu.SemaphoreType.DMA((32,)), pltpu.SemaphoreType.DMA((S // RB,)),
        pltpu.SemaphoreType.DMA((TOPK,)),
    ]
    out = pl.pallas_call(
        _kernel,
        in_specs=[pl.BlockSpec(memory_space=pltpu.HBM)] * 12,
        out_specs=pl.BlockSpec(memory_space=pltpu.HBM),
        out_shape=jax.ShapeDtypeStruct((S, M), bf16),
        scratch_shapes=scratch,
        compiler_params=pltpu.CompilerParams(vmem_limit_bytes=120 * 2 ** 20),
    )(A_x.reshape(S, M), A_c_kv.reshape(S, C), A_w_q, A_w_uk, A_w_uv, A_w_o.reshape(H * D, M),
      B_w_r.reshape(M // D, D), B_w_gate.T, B_w_up.T, B_w_down, c, w_mod)
    return out.reshape(A_x.shape)
```

```python
import functools

import jax
import jax.numpy as jnp
from jax import lax
import jax.experimental.pallas as pl
import jax.experimental.pallas.tpu as pltpu

S, M, C, D, H, F, TOPK = 2048, 640, 512, 128, 32, 1728, 8
G = 8
NG = H // G
T = 128
NB = S // T
CH = 4
RB = 256
EPS = 1e-5
KEY0 = 0x00800000
QSCALE = D ** -0.5 * 1.4426950408889634
NT = (((1,), (1,)), ((), ()))

f32, bf16, u32, i32 = jnp.float32, jnp.bfloat16, jnp.uint32, jnp.int32


def _rb(a):
    return a.astype(bf16).astype(f32)


def _sigmoid(a):
    return _rb(1.0 / _rb(1.0 + _rb(jnp.exp(-a))))


def _rows(r0, n):
    if isinstance(r0, int):
        return pl.ds(r0, n)
    return pl.ds(pl.multiple_of(r0, n & -n), n)


def _ld(ref, *idx, r0, n):
    return pltpu.bitcast(ref[(*idx, _rows(r0 // 2, n // 2), slice(None))], bf16)


def _st(ref, *idx, r0, val):
    ref[(*idx, _rows(r0 // 2, val.shape[0] // 2), slice(None))] = pltpu.bitcast(
        val.astype(bf16), u32)


def _dot(a, b):
    return jnp.dot(a, b, preferred_element_type=f32)


def _dot_nt(a, b):
    return lax.dot_general(a, b, NT, preferred_element_type=f32)


class _Blk:
    def __init__(self, i):
        self.i, self.s, self.mx, self.m, self.l, self.acc = i, {}, None, None, None, None


def _attention(q_s, k_s, v_s, ctx_s, hd, slot, filler):
    tri = (lax.broadcasted_iota(i32, (T, T), 1) <= lax.broadcasted_iota(i32, (T, T), 0))

    def chunks(b):
        n = b.i + 1 if b else 0
        return [(a, min(a + CH, n)) for a in range(0, n, CH)]

    def scores(b, a, e):
        return _dot_nt(_ld(q_s, slot, r0=b.i * T, n=T), _ld(k_s, hd, r0=a * T, n=(e - a) * T))

    def keep(b, a, e, s):
        for t in range(a, e):
            x = s[:, (t - a) * T:(t - a + 1) * T]
            if t == b.i:
                x = jnp.where(tri, x, -1e9)
            b.mx = x if b.mx is None else jnp.maximum(b.mx, x)
            b.s[t] = x

    def context(b, a, e):
        ps = []
        for t in range(a, e):
            p = jnp.exp2(b.s[t] - b.m)
            b.l = p if b.l is None else b.l + p
            ps.append(p)
        p = (jnp.concatenate(ps, axis=1) if len(ps) > 1 else ps[0]).astype(bf16)
        o = _dot(p, _ld(v_s, slot, r0=a * T, n=(e - a) * T))
        b.acc = o if b.acc is None else b.acc + o

    def finish(b):
        l = jnp.sum(b.l, axis=1, keepdims=True)
        r = pltpu.reciprocal(l, approx=True)
        r = r * (2.0 - l * r)
        _st(ctx_s, hd, r0=b.i * T, val=b.acc * r)

    filler(0)
    prev = None
    for n, i in enumerate(list(range(NB - 1, -1, -1)) + [None]):
        b = _Blk(i) if i is not None else None
        ca, cb = chunks(b), chunks(prev)
        for c in range(max(len(ca), len(cb))):
            s = scores(b, *ca[c]) if c < len(ca) else None
            if c < len(cb):
                context(prev, *cb[c])
            if s is not None:
                keep(b, *ca[c], s)
        if b:
            b.m = jnp.max(b.mx, axis=1, keepdims=True)
        if prev:
            finish(prev)
        filler(n + 1)
        prev = b


def _weave(mxu, *others):
    for n, job in enumerate(mxu):
        out = job()
        todo = [other for vpu in others
                for other in vpu[n * len(vpu) // len(mxu):(n + 1) * len(vpu) // len(mxu)]]
        if todo:
            zero = _zero(out[0:8, 0:D])
            for other in todo:
                other(zero)


def _zero(a):
    return jnp.minimum(pltpu.bitcast(a, i32)[0, 0] & 0xFFFF, 0)


def _kernel(x_hbm, ckv_hbm, wq_hbm, wk_hbm, wv_hbm, wo_hbm, wr_hbm, wg_hbm, wu_hbm, wd_hbm,
            c_hbm, wmod_hbm, out_hbm,
            x_s, ckv_s, wo_s, wr_s, wg_s, wu_s, wd_s, mod_s, w_s, k_s, q_s, v_s, ctx_s,
            in_sem, out_sem, fix_sem):
    copies = []

    def copy(src, dst):
        copies.append(pltpu.make_async_copy(src, dst, in_sem.at[len(copies)]))
        return copies[-1]

    def part(hbm, vmem, *idx):
        return copy(hbm.at[idx], vmem.at[idx])

    def start(cps):
        for cp in cps:
            cp.start()

    def wait(cps):
        for cp in cps:
            cp.wait()

    stage4 = [copy(wo_hbm, wo_s), copy(wr_hbm, wr_s), copy(wg_hbm, wg_s), copy(wu_hbm, wu_s),
              copy(wd_hbm, wd_s)]

    def mod(j):
        return mod_s[:, pl.ds(j * M, M)]

    def qproj(hd, slot, i):
        h = jnp.concatenate([_ld(w_s, H + j, r0=i * T, n=T) for j in range(M // D)], axis=1)
        _st(q_s, slot, r0=i * T, val=_dot(h, _ld(w_s, hd, r0=0, n=M)) * QSCALE)

    def vproj(hd, slot, i):
        _st(v_s, slot, r0=i * T, val=_dot(ckv_s[pl.ds(i * T, T), :], _ld(w_s, hd, r0=M + C, n=C)))

    def qv(hd, slot):
        return [functools.partial(f, hd, slot, i) for i in range(NB) for f in (qproj, vproj)]

    def phase1(wq_raw, wk_raw, wv_raw, c_s, wmod_s):
        R0 = 512
        wk0_cp = part(wk_hbm, wk_raw, slice(None), pl.ds(0, G))
        ckv0_cp = part(ckv_hbm, ckv_s, pl.ds(0, R0))
        stage1 = [part(ckv_hbm, ckv_s, pl.ds(R0, S - R0)), part(wk_hbm, wk_raw, slice(None), pl.ds(G, G))]
        stage2 = [part(wk_hbm, wk_raw, slice(None), pl.ds(2 * G, 2 * G)),
                  copy(c_hbm, c_s), copy(wmod_hbm, wmod_s), copy(x_hbm, x_s)]
        stage3 = [copy(wq_hbm, wq_raw), copy(wv_hbm, wv_raw)]

        def per_head(raw, base, g):
            def job(r0, z=0):
                w = raw[pl.ds(z + r0, 16), pl.ds(g * G, G), :].reshape(16, G * D)
                for j in range(G):
                    _st(w_s, g * G + j, r0=base + r0, val=w[:, j * D:(j + 1) * D])
            return [functools.partial(job, r0) for r0 in range(0, raw.shape[0], 16)]

        def kproj(heads, lo, hi):
            def job(hd, r0):
                k = _dot(ckv_s[pl.ds(r0, 256), :], _ld(w_s, hd, r0=M, n=C))
                _st(k_s, hd, r0=r0, val=k)
                return k
            return [functools.partial(job, hd, r0) for hd in heads for r0 in range(lo, hi, 256)]

        def modulation():
            cf = c_s[...].astype(f32)
            col = jnp.broadcast_to(_rb(cf * _sigmoid(cf)), (D, M)).T

            def job(j, z):
                w = wmod_s[_rows(z, M), pl.ds(j * D, D)].astype(f32)
                m = _rb(jnp.sum(w * col, axis=0, keepdims=True))
                mod_s[:, pl.ds(j * D, D)] = m
            return [functools.partial(job, j) for j in range(6 * M // D)]

        def norm1(r0, z):
            xf = x_s[_rows(z + r0, 48 if r0 + 48 <= S else S - r0), :].astype(f32)
            xc = xf - jnp.mean(xf, axis=1, keepdims=True)
            xn = xc * lax.rsqrt(jnp.mean(xc * xc, axis=1, keepdims=True) + EPS)
            h = xn * (1.0 + mod(1)) + mod(0)
            for j in range(M // D):
                _st(w_s, H + j, r0=r0, val=h[:, j * D:(j + 1) * D])

        start([wk0_cp, ckv0_cp])
        wk0_cp.wait()
        start(stage1)
        _weave(per_head(wk_raw, M, 0), [])
        ckv0_cp.wait()
        _weave(kproj(range(8), 0, R0), [])
        wait(stage1)
        start(stage2)
        _weave(kproj(range(8), R0, S), per_head(wk_raw, M, 1))
        _weave(kproj(range(8, 12), 0, S), [])
        wait(stage2)
        start(stage3)
        _weave(kproj(range(12, 16), 0, S), per_head(wk_raw, M, 2), modulation())
        _weave(kproj(range(16, 22), 0, S), per_head(wk_raw, M, 3),
               [functools.partial(norm1, r0) for r0 in range(0, S, 48)])
        wait(stage3)
        start(stage4)
        _weave(kproj(range(22, H), 0, S),
               [job for g in range(NG) for job in per_head(wq_raw, 0, g) + per_head(wv_raw, M + C, g)])
        _weave(qv(0, 0))

    V = pltpu.VMEM
    pl.run_scoped(phase1, V((M, H, D), bf16), V((C, H, D), bf16), V((C, H, D), bf16),
                  V((1, M), bf16), V((M, 6 * M), bf16))

    def next_head(hd, slot):
        jobs = qv(hd, slot)
        cuts = [0, 1] + [1 + (27 * n) // NB for n in range(1, NB + 1)] + [len(jobs)]
        return lambda n: _weave(jobs[cuts[n]:cuts[n + 1]], [])

    def pair(p, _):
        _attention(q_s, k_s, v_s, ctx_s, 2 * p, 0, next_head(2 * p + 1, 1))
        _attention(q_s, k_s, v_s, ctx_s, 2 * p + 1, 1, next_head(2 * p + 2, 0))

    lax.fori_loop(0, H // 2 - 1, pair, None)

    def phase3(y_s, key_s, top_s, xh_s, out_s, wgu_s):
        wait(stage4)
        sub = lax.broadcasted_iota(i32, (TOPK, D), 0)
        lane = lax.broadcasted_iota(i32, (TOPK, D), 1)

        def oproj(r0, n, slot):
            acc = {}

            def job(j, h0):
                ctx = jnp.concatenate([_ld(ctx_s, h0 + t, r0=r0, n=n) for t in range(CH)], axis=1)
                y = _dot(ctx, wo_s[pl.ds(h0 * D, CH * D), pl.ds(j * D, D)])
                acc[j] = acc[j] + y if h0 else y
                if h0 + CH == H:
                    y_s[slot][pl.ds(0, n), pl.ds(j * D, D)] = acc[j]
                return y
            return [functools.partial(job, j, h0) for j in range(M // D) for h0 in range(0, H, CH)]

        def out_copy(b):
            return pltpu.make_async_copy(out_s.at[_rows(b * RB, RB)], out_hbm.at[_rows(b * RB, RB)],
                                         out_sem.at[b])

        def epilogue(r0, slot, off, n, z=0):
            rows = _rows(r0, n)
            ga, sb, cb, gb = mod(2), mod(3), _rb(1.0 + mod(4)), mod(5)
            x1 = _rb(x_s[_rows(z + r0, n), :].astype(f32) + _rb(ga * _rb(y_s[slot][_rows(z + off, n), :])))
            mean = jnp.mean(x1, axis=1, keepdims=True)
            xc = x1 - mean
            var = _rb(jnp.mean(xc * xc, axis=1, keepdims=True))
            inv = 1.0 / _rb(jnp.sqrt(_rb(var + EPS)))
            h2 = _rb(_rb(_rb(_rb(x1 - _rb(mean)) * inv) * cb) + sb)
            xh_s[rows, :] = pltpu.bitcast(x1, u32) | (pltpu.bitcast(h2, u32) >> 16)
            out_s[rows, :] = (x1 + _rb(gb * h2)).astype(bf16)
            wr = wr_s[...].astype(f32)
            prod = h2[:, 0:D] * wr[0:1]
            for j in range(1, M // D):
                prod = prod + h2[:, j * D:(j + 1) * D] * wr[j:j + 1]
            r = jnp.broadcast_to(_rb(jnp.sum(prod, axis=1, keepdims=True)), (n, D))
            bits = lax.bitcast_convert_type(r, i32)
            code = lax.shift_right_logical(bits, 16)
            code = jnp.where(bits < 0, 0xFFFF - code, code + 0x8000)
            code = jnp.where(r == 0.0, 0x8000, code)
            code = jnp.where(r != r, 0, code)
            key = code * S + (S - 1 + KEY0 - r0) - lax.broadcasted_iota(i32, (n, D), 0)
            key_s[pl.ds(off % T, n), :] = lax.bitcast_convert_type(key, f32)

        def select(z=0):
            best = top_s[...]
            cols = [key_s[pl.ds(8 * t, 8), :] for t in range(T // 8)]
            flat = jnp.zeros((TOPK, D), f32)
            for t, col in enumerate(cols):
                flat = jnp.where(lane - sub == 8 * t, col, flat)
            new = None
            for cand in (flat, jnp.where(lane == sub, best, 0.0)):
                cand = jnp.broadcast_to(jnp.max(cand, axis=0, keepdims=True), (TOPK, D))
                above = sum((col > cand).astype(f32) for col in cols + [best])
                rank = jnp.sum(above, axis=0, keepdims=True)
                pick = jnp.where(rank == sub.astype(f32), cand, 0.0)
                new = pick if new is None else jnp.maximum(new, pick)
            top_s[...] = jnp.broadcast_to(jnp.max(new, axis=1, keepdims=True), (TOPK, D))

        def epilogues(r0, slot, rows=RB, n=16):
            jobs = []
            for off in range(0, rows, n):
                jobs.append(functools.partial(epilogue, r0 + off, slot, off, n))
                if (off + n) % T == 0:
                    jobs.append(select)
            return jobs

        def flip(t, src):
            def job(r0, z):
                wgu_s[t, :, pl.ds(r0, D)] = src[pl.ds(pl.multiple_of(z + r0, 64), D), :].T
            return [functools.partial(job, r0) for r0 in range(0, F - D, D)] + [
                functools.partial(job, F - D)]

        NR = S // RB
        top_s[...] = jnp.zeros(top_s.shape, f32)
        _attention(q_s, k_s, v_s, ctx_s, H - 2, 0, next_head(H - 1, 1))
        last = oproj((NR - 1) * RB, RB, 1)
        cuts = [0] * 4 + [len(last) * n // 15 for n in range(1, 16)]
        _attention(q_s, k_s, v_s, ctx_s, H - 1, 1, lambda n: _weave(last[cuts[n]:cuts[n + 1]]))

        def blocks(n, _):
            b = NR - 2 - 2 * n
            _weave(oproj(b * RB, RB, 0), epilogues((b + 1) * RB, 1))
            out_copy(b + 1).start()
            _weave(oproj((b - 1) * RB, RB, 1), epilogues(b * RB, 0))
            out_copy(b).start()

        lax.fori_loop(0, NR // 2 - 1, blocks, None)
        _weave(oproj(T, T, 0), epilogues(RB, 1), flip(0, wg_s))
        out_copy(1).start()
        _weave(oproj(0, T, 1), epilogues(T, 0, T), flip(1, wu_s))
        _weave(epilogues(0, 1, T, T))
        out_copy(0).start()

        top = lax.bitcast_convert_type(top_s[...], i32) - KEY0
        sel = S - 1 - (top & (S - 1))
        code = lax.shift_right_logical(top, 11)
        code = jnp.where(code >= 0x8000, code - 0x8000, 0xFFFF - code)
        r_sel = lax.bitcast_convert_type(code * 0x10000, f32)[:, 0:1]
        idx = [sel[j, 0] for j in range(TOPK)]

        both = jnp.concatenate([xh_s[pl.ds(t, 1), :] for t in idx], axis=0)
        hsel = pltpu.bitcast(both << 16, f32)
        xsel = pltpu.bitcast((both >> 16) << 16, f32)
        lhs = jnp.concatenate([hsel, hsel], axis=0).astype(bf16)
        gate = _rb(_dot(lhs, wgu_s[0]))
        act = _rb(gate * _sigmoid(gate)) * _rb(_dot(lhs, wgu_s[1]))
        y = _rb(_rb(_dot(act.astype(bf16), wd_s[...])[0:TOPK]) * _sigmoid(r_sel))
        fixed = xsel + _rb(mod(5) * _rb(hsel + y))

        for b in range(NR):
            out_copy(b).wait()
        tiles = [pl.multiple_of((t // 16) * 16, 16) for t in idx]
        row = lax.broadcasted_iota(i32, (16, M), 0)
        for j in range(TOPK):
            cur = out_s[pl.ds(tiles[j], 16), :].astype(f32)
            cur = jnp.where(row == idx[j] - tiles[j], fixed[j:j + 1], cur)
            out_s[pl.ds(tiles[j], 16), :] = cur.astype(bf16)

        def fix_copy(j):
            return pltpu.make_async_copy(out_s.at[pl.ds(tiles[j], 16)], out_hbm.at[pl.ds(tiles[j], 16)],
                                         fix_sem.at[j])

        fresh = []
        for j in range(TOPK):
            new = tiles[j] >= 0
            for k in range(j):
                new = jnp.logical_and(new, tiles[j] != tiles[k])
            fresh.append(new)
        for j in range(TOPK):
            pl.when(fresh[j])(fix_copy(j).start)
        for j in range(TOPK):
            pl.when(fresh[j])(fix_copy(j).wait)

    pl.run_scoped(phase3, [V((RB, M), f32)] * 2, V((T, D), f32), V((TOPK, D), f32),
                  V((S, M), u32), V((S, M), bf16), V((2, M, F), bf16))


@jax.jit
def pallas_adaLN_cond__compressed_kv_cla__moe_arch_mod__prompt_kernel(
    A_x: jax.Array,
    A_c_kv: jax.Array,
    A_w_q: jax.Array,
    A_w_uk: jax.Array,
    A_w_uv: jax.Array,
    A_w_o: jax.Array,
    B_x: jax.Array,
    B_w_r: jax.Array,
    B_w_gate: jax.Array,
    B_w_up: jax.Array,
    B_w_down: jax.Array,
    c: jax.Array,
    w_mod: jax.Array,
):
    del B_x
    V = pltpu.VMEM
    scratch = [
        V((S, M), bf16), V((S, C), bf16),
        V((H * D, M), bf16), V((M // D, D), bf16),
        V((F, M), bf16), V((F, M), bf16), V((F, M), bf16),
        V((1, 6 * M), f32),
        V((H + M // D, S // 2, D), u32),
        V((H, S // 2, D), u32),
        V((2, S // 2, D), u32), V((2, S // 2, D), u32),
        V((H, S // 2, D), u32),
        pltpu.SemaphoreType.DMA((16,)), pltpu.SemaphoreType.DMA((S // RB,)),
        pltpu.SemaphoreType.DMA((TOPK,)),
    ]
    out = pl.pallas_call(
        _kernel,
        in_specs=[pl.BlockSpec(memory_space=pltpu.HBM)] * 12,
        out_specs=pl.BlockSpec(memory_space=pltpu.HBM),
        out_shape=jax.ShapeDtypeStruct((S, M), bf16),
        scratch_shapes=scratch,
        compiler_params=pltpu.CompilerParams(vmem_limit_bytes=120 * 2 ** 20),
    )(A_x.reshape(S, M), A_c_kv.reshape(S, C), A_w_q, A_w_uk, A_w_uv, A_w_o.reshape(H * D, M),
      B_w_r.reshape(M // D, D), B_w_gate.T, B_w_up.T, B_w_down, c, w_mod)
    return out.reshape(A_x.shape)
```

```python
import functools

import jax
import jax.numpy as jnp
from jax import lax
import jax.experimental.pallas as pl
import jax.experimental.pallas.tpu as pltpu

S, M, C, D, H, F, TOPK = 2048, 640, 512, 128, 32, 1728, 8
G = 8
NG = H // G
T = 128
NB = S // T
CH = 4
RB = 256
EPS = 1e-5
KEY0 = 0x00800000
QSCALE = D ** -0.5 * 1.4426950408889634
NT = (((1,), (1,)), ((), ()))

f32, bf16, u32, i32 = jnp.float32, jnp.bfloat16, jnp.uint32, jnp.int32


def _rb(a):
    return a.astype(bf16).astype(f32)


def _sigmoid(a):
    return _rb(1.0 / _rb(1.0 + _rb(jnp.exp(-a))))


def _rows(r0, n):
    if isinstance(r0, int):
        return pl.ds(r0, n)
    return pl.ds(pl.multiple_of(r0, n & -n), n)


def _ld(ref, *idx, r0, n):
    return pltpu.bitcast(ref[(*idx, _rows(r0 // 2, n // 2), slice(None))], bf16)


def _st(ref, *idx, r0, val):
    ref[(*idx, _rows(r0 // 2, val.shape[0] // 2), slice(None))] = pltpu.bitcast(
        val.astype(bf16), u32)


def _dot(a, b):
    return jnp.dot(a, b, preferred_element_type=f32)


def _dot_nt(a, b):
    return lax.dot_general(a, b, NT, preferred_element_type=f32)


class _Blk:
    def __init__(self, i):
        self.i, self.s, self.mx, self.m, self.l, self.acc = i, {}, None, None, None, None


def _attention(q_s, k_s, v_s, ctx_s, hd, slot, filler):
    tri = (lax.broadcasted_iota(i32, (T, T), 1) <= lax.broadcasted_iota(i32, (T, T), 0))

    def chunks(b):
        n = b.i + 1 if b else 0
        return [(a, min(a + CH, n)) for a in range(0, n, CH)]

    def scores(b, a, e):
        return _dot_nt(_ld(q_s, slot, r0=b.i * T, n=T), _ld(k_s, hd, r0=a * T, n=(e - a) * T))

    def keep(b, a, e, s):
        for t in range(a, e):
            x = s[:, (t - a) * T:(t - a + 1) * T]
            if t == b.i:
                x = jnp.where(tri, x, -1e9)
            b.mx = x if b.mx is None else jnp.maximum(b.mx, x)
            b.s[t] = x

    def context(b, a, e):
        ps = []
        for t in range(a, e):
            p = jnp.exp2(b.s[t] - b.m)
            b.l = p if b.l is None else b.l + p
            ps.append(p)
        p = (jnp.concatenate(ps, axis=1) if len(ps) > 1 else ps[0]).astype(bf16)
        o = _dot(p, _ld(v_s, slot, r0=a * T, n=(e - a) * T))
        b.acc = o if b.acc is None else b.acc + o

    def finish(b):
        l = jnp.sum(b.l, axis=1, keepdims=True)
        r = pltpu.reciprocal(l, approx=True)
        r = r * (2.0 - l * r)
        _st(ctx_s, hd, r0=b.i * T, val=b.acc * r)

    filler(0)
    prev = None
    for n, i in enumerate(list(range(NB - 1, -1, -1)) + [None]):
        b = _Blk(i) if i is not None else None
        ca, cb = chunks(b), chunks(prev)
        for c in range(max(len(ca), len(cb))):
            s = scores(b, *ca[c]) if c < len(ca) else None
            if c < len(cb):
                context(prev, *cb[c])
            if s is not None:
                keep(b, *ca[c], s)
        if b:
            b.m = jnp.max(b.mx, axis=1, keepdims=True)
        if prev:
            finish(prev)
        filler(n + 1)
        prev = b


def _weave(mxu, *others):
    for n, job in enumerate(mxu):
        out = job()
        todo = [other for vpu in others
                for other in vpu[n * len(vpu) // len(mxu):(n + 1) * len(vpu) // len(mxu)]]
        for t, other in enumerate(todo):
            r0 = t * (out.shape[0] // 8) // len(todo) * 8
            other(_zero(out[r0:r0 + 8, 0:D]))


def _zero(a):
    return jnp.minimum(pltpu.bitcast(a, i32)[0, 0] & 0xFFFF, 0)


def _kernel(x_hbm, ckv_hbm, wq_hbm, wk_hbm, wv_hbm, wo_hbm, wr_hbm, wg_hbm, wu_hbm, wd_hbm,
            c_hbm, wmod_hbm, out_hbm,
            x_s, ckv_s, wo_s, wr_s, wg_s, wu_s, wd_s, mod_s, w_s, k_s, q_s, v_s, ctx_s,
            in_sem, out_sem, fix_sem):
    copies = []

    def copy(src, dst):
        copies.append(pltpu.make_async_copy(src, dst, in_sem.at[len(copies)]))
        return copies[-1]

    def part(hbm, vmem, *idx):
        return copy(hbm.at[idx], vmem.at[idx])

    def start(cps):
        for cp in cps:
            cp.start()

    def wait(cps):
        for cp in cps:
            cp.wait()

    stage4 = [copy(wo_hbm, wo_s), copy(wr_hbm, wr_s), copy(wg_hbm, wg_s), copy(wu_hbm, wu_s),
              copy(wd_hbm, wd_s)]

    def mod(j):
        return mod_s[:, pl.ds(j * M, M)]

    def qproj(hd, slot, i):
        h = jnp.concatenate([_ld(w_s, H + j, r0=i * T, n=T) for j in range(M // D)], axis=1)
        _st(q_s, slot, r0=i * T, val=_dot(h, _ld(w_s, hd, r0=0, n=M)) * QSCALE)

    def vproj(hd, slot, i):
        _st(v_s, slot, r0=i * T, val=_dot(_ld(ckv_s, r0=i * T, n=T), _ld(w_s, hd, r0=M + C, n=C)))

    def qv(hd, slot):
        return [functools.partial(f, hd, slot, i) for i in range(NB) for f in (qproj, vproj)]

    def phase1(ckv_raw, wq_raw, wk_raw, wv_raw, c_s, wmod_s):
        R0 = 768
        wk0_cp = part(wk_hbm, wk_raw, slice(None), pl.ds(0, G))
        ckv0_cp = part(ckv_hbm, ckv_raw, pl.ds(0, R0))
        stage1 = [part(ckv_hbm, ckv_raw, pl.ds(R0, S - R0)), part(wk_hbm, wk_raw, slice(None), pl.ds(G, G))]
        stage2 = [part(wk_hbm, wk_raw, slice(None), pl.ds(2 * G, 2 * G)),
                  copy(c_hbm, c_s), copy(wmod_hbm, wmod_s), copy(x_hbm, x_s)]
        stage3 = [copy(wq_hbm, wq_raw), copy(wv_hbm, wv_raw)]

        def per_head(raw, base, g):
            def job(r0, z=0):
                w = raw[pl.ds(z + r0, 16), pl.ds(g * G, G), :].reshape(16, G * D)
                for j in range(G):
                    _st(w_s, g * G + j, r0=base + r0, val=w[:, j * D:(j + 1) * D])
            return [functools.partial(job, r0) for r0 in range(0, raw.shape[0], 16)]

        def kproj(heads, lo, hi):
            def job(hd, r0):
                if hd == 0:
                    ckv = ckv_raw[pl.ds(r0, 256), :]
                    _st(ckv_s, r0=r0, val=ckv)
                else:
                    ckv = _ld(ckv_s, r0=r0, n=256)
                k = _dot(ckv, _ld(w_s, hd, r0=M, n=C))
                _st(k_s, hd, r0=r0, val=k)
                return k
            return [functools.partial(job, hd, r0) for hd in heads for r0 in range(lo, hi, 256)]

        def modulation():
            cf = c_s[...].astype(f32)
            col = jnp.broadcast_to(_rb(cf * _sigmoid(cf)), (D, M)).T

            def job(j, z):
                w = wmod_s[_rows(z, M), pl.ds(j * D, D)].astype(f32)
                m = _rb(jnp.sum(w * col, axis=0, keepdims=True))
                mod_s[:, pl.ds(j * D, D)] = m
            return [functools.partial(job, j) for j in range(6 * M // D)]

        def norm1(r0, z):
            xf = x_s[_rows(z + r0, 16), :].astype(f32)
            xc = xf - jnp.mean(xf, axis=1, keepdims=True)
            xn = xc * lax.rsqrt(jnp.mean(xc * xc, axis=1, keepdims=True) + EPS)
            h = xn * (1.0 + mod(1)) + mod(0)
            for j in range(M // D):
                _st(w_s, H + j, r0=r0, val=h[:, j * D:(j + 1) * D])

        start([wk0_cp, ckv0_cp])
        start(stage1)
        wk0_cp.wait()
        _weave(per_head(wk_raw, M, 0), [])
        ckv0_cp.wait()
        _weave(kproj(range(8), 0, R0), [])
        start(stage2)
        wait(stage1)
        _weave(kproj(range(8), R0, S), per_head(wk_raw, M, 1))
        _weave(kproj(range(8, 10), 0, S))
        start(stage3)
        wait(stage2)
        _weave(kproj(range(10, 15), 0, S), per_head(wk_raw, M, 2), modulation())
        _weave(kproj(range(15, 21), 0, S), per_head(wk_raw, M, 3),
               [functools.partial(norm1, r0) for r0 in range(0, S, 16)])
        start(stage4)
        wait(stage3)
        _weave(kproj(range(21, H), 0, S),
               [job for g in range(NG) for job in per_head(wq_raw, 0, g) + per_head(wv_raw, M + C, g)])
        _weave(qv(0, 0))

    V = pltpu.VMEM
    pl.run_scoped(phase1, V((S, C), bf16), V((M, H, D), bf16), V((C, H, D), bf16), V((C, H, D), bf16),
                  V((1, M), bf16), V((M, 6 * M), bf16))

    def next_head(hd, slot):
        jobs = qv(hd, slot)
        cuts = [0, 1] + [1 + (27 * n) // NB for n in range(1, NB + 1)] + [len(jobs)]
        return lambda n: _weave(jobs[cuts[n]:cuts[n + 1]], [])

    def pair(p, _):
        _attention(q_s, k_s, v_s, ctx_s, 2 * p + 1, 1, next_head(2 * p + 2, 0))
        _attention(q_s, k_s, v_s, ctx_s, 2 * p + 2, 0, next_head(2 * p + 3, 1))

    _attention(q_s, k_s, v_s, ctx_s, 0, 0, next_head(1, 1))
    lax.fori_loop(0, H // 2 - 1, pair, None)

    def phase3(y_s, key_s, top_s, xh_s, out_s, wgu_s):
        wait(stage4)
        sub = lax.broadcasted_iota(i32, (TOPK, D), 0)
        lane = lax.broadcasted_iota(i32, (TOPK, D), 1)

        def oproj(r0, n, slot):
            acc = {}

            def job(j, h0):
                ctx = jnp.concatenate([_ld(ctx_s, h0 + t, r0=r0, n=n) for t in range(CH)], axis=1)
                y = _dot(ctx, wo_s[pl.ds(h0 * D, CH * D), pl.ds(j * D, D)])
                acc[j] = acc[j] + y if h0 else y
                if h0 + CH == H:
                    y_s[slot][pl.ds(0, n), pl.ds(j * D, D)] = acc[j]
                return y
            return [functools.partial(job, j, h0) for j in range(M // D) for h0 in range(0, H, CH)]

        def out_copy(b):
            return pltpu.make_async_copy(out_s.at[_rows(b * RB, RB)], out_hbm.at[_rows(b * RB, RB)],
                                         out_sem.at[b])

        def epilogue(r0, slot, off, n, z=0):
            rows = _rows(r0, n)
            ga, sb, cb, gb = mod(2), mod(3), _rb(1.0 + mod(4)), mod(5)
            x1 = _rb(x_s[_rows(z + r0, n), :].astype(f32) + _rb(ga * _rb(y_s[slot][_rows(z + off, n), :])))
            mean = jnp.mean(x1, axis=1, keepdims=True)
            xc = x1 - mean
            var = _rb(jnp.mean(xc * xc, axis=1, keepdims=True))
            inv = 1.0 / _rb(jnp.sqrt(_rb(var + EPS)))
            h2 = _rb(_rb(_rb(_rb(x1 - _rb(mean)) * inv) * cb) + sb)
            xh_s[rows, :] = pltpu.bitcast(x1, u32) | (pltpu.bitcast(h2, u32) >> 16)
            out_s[rows, :] = (x1 + _rb(gb * h2)).astype(bf16)
            wr = wr_s[...].astype(f32)
            prod = h2[:, 0:D] * wr[0:1]
            for j in range(1, M // D):
                prod = prod + h2[:, j * D:(j + 1) * D] * wr[j:j + 1]
            r = jnp.broadcast_to(_rb(jnp.sum(prod, axis=1, keepdims=True)), (n, D))
            bits = lax.bitcast_convert_type(r, i32)
            code = lax.shift_right_logical(bits, 16)
            code = jnp.where(bits < 0, 0xFFFF - code, code + 0x8000)
            code = jnp.where(r == 0.0, 0x8000, code)
            code = jnp.where(r != r, 0, code)
            key = code * S + (S - 1 + KEY0 - r0) - lax.broadcasted_iota(i32, (n, D), 0)
            key_s[pl.ds(off % T, n), :] = lax.bitcast_convert_type(key, f32)

        def select(z=0):
            best = top_s[...]
            cols = [key_s[pl.ds(8 * t, 8), :] for t in range(T // 8)]
            flat = jnp.zeros((TOPK, D), f32)
            for t, col in enumerate(cols):
                flat = jnp.where(lane - sub == 8 * t, col, flat)
            new = None
            for cand in (flat, jnp.where(lane == sub, best, 0.0)):
                cand = jnp.broadcast_to(jnp.max(cand, axis=0, keepdims=True), (TOPK, D))
                above = sum((col > cand).astype(f32) for col in cols + [best])
                rank = jnp.sum(above, axis=0, keepdims=True)
                pick = jnp.where(rank == sub.astype(f32), cand, 0.0)
                new = pick if new is None else jnp.maximum(new, pick)
            top_s[...] = jnp.broadcast_to(jnp.max(new, axis=1, keepdims=True), (TOPK, D))

        def epilogues(r0, slot, rows=RB, n=16):
            jobs = []
            for off in range(0, rows, n):
                jobs.append(functools.partial(epilogue, r0 + off, slot, off, n))
                if (off + n) % T == 0:
                    jobs.append(select)
            return jobs

        def flip(t, src):
            def job(r0, z):
                wgu_s[t, :, pl.ds(r0, D)] = src[pl.ds(pl.multiple_of(z + r0, 64), D), :].T
            return [functools.partial(job, r0) for r0 in range(0, F - D, D)] + [
                functools.partial(job, F - D)]

        NR = S // RB
        top_s[...] = jnp.zeros(top_s.shape, f32)
        last = oproj((NR - 1) * RB, RB, 1)
        cuts = [0] * 4 + [len(last) * n // 15 for n in range(1, 16)]
        _attention(q_s, k_s, v_s, ctx_s, H - 1, 1, lambda n: _weave(last[cuts[n]:cuts[n + 1]]))

        def blocks(n, _):
            b = NR - 2 - 2 * n
            _weave(oproj(b * RB, RB, 0), epilogues((b + 1) * RB, 1))
            out_copy(b + 1).start()
            _weave(oproj((b - 1) * RB, RB, 1), epilogues(b * RB, 0))
            out_copy(b).start()

        lax.fori_loop(0, NR // 2 - 1, blocks, None)
        _weave(oproj(T, T, 0), epilogues(RB, 1), flip(0, wg_s))
        out_copy(1).start()
        _weave(oproj(0, T, 1), epilogues(T, 0, T), flip(1, wu_s))
        _weave(epilogues(0, 1, T, T))
        out_copy(0).start()

        top = lax.bitcast_convert_type(top_s[...], i32) - KEY0
        sel = S - 1 - (top & (S - 1))
        code = lax.shift_right_logical(top, 11)
        code = jnp.where(code >= 0x8000, code - 0x8000, 0xFFFF - code)
        r_sel = lax.bitcast_convert_type(code * 0x10000, f32)[:, 0:1]
        idx = [sel[j, 0] for j in range(TOPK)]

        both = jnp.concatenate([xh_s[pl.ds(t, 1), :] for t in idx], axis=0)
        hsel = pltpu.bitcast(both << 16, f32)
        xsel = pltpu.bitcast((both >> 16) << 16, f32)
        lhs = jnp.concatenate([hsel, hsel], axis=0).astype(bf16)
        gate = _rb(_dot(lhs, wgu_s[0]))
        act = _rb(gate * _sigmoid(gate)) * _rb(_dot(lhs, wgu_s[1]))
        y = _rb(_rb(_dot(act.astype(bf16), wd_s[...])[0:TOPK]) * _sigmoid(r_sel))
        fixed = xsel + _rb(mod(5) * _rb(hsel + y))

        for b in range(NR):
            out_copy(b).wait()
        tiles = [pl.multiple_of((t // 16) * 16, 16) for t in idx]
        row = lax.broadcasted_iota(i32, (16, M), 0)
        for j in range(TOPK):
            cur = out_s[pl.ds(tiles[j], 16), :].astype(f32)
            cur = jnp.where(row == idx[j] - tiles[j], fixed[j:j + 1], cur)
            out_s[pl.ds(tiles[j], 16), :] = cur.astype(bf16)

        def fix_copy(j):
            return pltpu.make_async_copy(out_s.at[pl.ds(tiles[j], 16)], out_hbm.at[pl.ds(tiles[j], 16)],
                                         fix_sem.at[j])

        fresh = []
        for j in range(TOPK):
            new = tiles[j] >= 0
            for k in range(j):
                new = jnp.logical_and(new, tiles[j] != tiles[k])
            fresh.append(new)
        for j in range(TOPK):
            pl.when(fresh[j])(fix_copy(j).start)
        for j in range(TOPK):
            pl.when(fresh[j])(fix_copy(j).wait)

    pl.run_scoped(phase3, [V((RB, M), f32)] * 2, V((T, D), f32), V((TOPK, D), f32),
                  V((S, M), u32), V((S, M), bf16), V((2, M, F), bf16))


@jax.jit
def pallas_adaLN_cond__compressed_kv_cla__moe_arch_mod__prompt_kernel(
    A_x: jax.Array,
    A_c_kv: jax.Array,
    A_w_q: jax.Array,
    A_w_uk: jax.Array,
    A_w_uv: jax.Array,
    A_w_o: jax.Array,
    B_x: jax.Array,
    B_w_r: jax.Array,
    B_w_gate: jax.Array,
    B_w_up: jax.Array,
    B_w_down: jax.Array,
    c: jax.Array,
    w_mod: jax.Array,
):
    del B_x
    V = pltpu.VMEM
    scratch = [
        V((S, M), bf16), V((S // 2, C), u32),
        V((H * D, M), bf16), V((M // D, D), bf16),
        V((F, M), bf16), V((F, M), bf16), V((F, M), bf16),
        V((1, 6 * M), f32),
        V((H + M // D, S // 2, D), u32),
        V((H, S // 2, D), u32),
        V((2, S // 2, D), u32), V((2, S // 2, D), u32),
        V((H, S // 2, D), u32),
        pltpu.SemaphoreType.DMA((16,)), pltpu.SemaphoreType.DMA((S // RB,)),
        pltpu.SemaphoreType.DMA((TOPK,)),
    ]
    out = pl.pallas_call(
        _kernel,
        in_specs=[pl.BlockSpec(memory_space=pltpu.HBM)] * 12,
        out_specs=pl.BlockSpec(memory_space=pltpu.HBM),
        out_shape=jax.ShapeDtypeStruct((S, M), bf16),
        scratch_shapes=scratch,
        compiler_params=pltpu.CompilerParams(vmem_limit_bytes=120 * 2 ** 20),
    )(A_x.reshape(S, M), A_c_kv.reshape(S, C), A_w_q, A_w_uk, A_w_uv, A_w_o.reshape(H * D, M),
      B_w_r.reshape(M // D, D), B_w_gate.T, B_w_up.T, B_w_down, c, w_mod)
    return out.reshape(A_x.shape)
```

```python
import functools

import jax
import jax.numpy as jnp
from jax import lax
import jax.experimental.pallas as pl
import jax.experimental.pallas.tpu as pltpu

S, M, C, D, H, F, TOPK = 2048, 640, 512, 128, 32, 1728, 8
G = 8
NG = H // G
T = 128
NB = S // T
CH = 4
RB = 256
PAD = 16
EPS = 1e-5
KEY0 = 0x00800000
QSCALE = D ** -0.5 * 1.4426950408889634
NT = (((1,), (1,)), ((), ()))

f32, bf16, u32, i32 = jnp.float32, jnp.bfloat16, jnp.uint32, jnp.int32


def _rb(a):
    return a.astype(bf16).astype(f32)


def _sigmoid(a):
    return _rb(1.0 / _rb(1.0 + _rb(jnp.exp(-a))))


def _rows(r0, n):
    if isinstance(r0, int):
        return pl.ds(r0, n)
    return pl.ds(pl.multiple_of(r0, n & -n), n)


def _ld(ref, *idx, r0, n):
    return pltpu.bitcast(ref[(*idx, _rows(r0 // 2, n // 2), slice(None))], bf16)


def _st(ref, *idx, r0, val):
    ref[(*idx, _rows(r0 // 2, val.shape[0] // 2), slice(None))] = pltpu.bitcast(
        val.astype(bf16), u32)


def _dot(a, b):
    return jnp.dot(a, b, preferred_element_type=f32)


def _dot_nt(a, b):
    return lax.dot_general(a, b, NT, preferred_element_type=f32)


class _Blk:
    def __init__(self, i):
        self.i, self.s, self.mx, self.m, self.l, self.acc = i, {}, None, None, None, None


def _attention(q_s, k_s, v_s, ctx_s, hd, slot, filler):
    tri = (lax.broadcasted_iota(i32, (T, T), 1) <= lax.broadcasted_iota(i32, (T, T), 0))

    def chunks(b):
        n = b.i + 1 if b else 0
        return [(a, min(a + CH, n)) for a in range(0, n, CH)]

    def scores(b, a, e):
        return _dot_nt(_ld(q_s, slot, r0=b.i * T, n=T), _ld(k_s, hd, r0=a * T, n=(e - a) * T))

    def keep(b, a, e, s):
        for t in range(a, e):
            x = s[:, (t - a) * T:(t - a + 1) * T]
            if t == b.i:
                x = jnp.where(tri, x, -1e9)
            b.mx = x if b.mx is None else jnp.maximum(b.mx, x)
            b.s[t] = x

    def context(b, a, e):
        ps = []
        for t in range(a, e):
            p = jnp.exp2(b.s[t] - b.m)
            b.l = p if b.l is None else b.l + p
            ps.append(p)
        p = (jnp.concatenate(ps, axis=1) if len(ps) > 1 else ps[0]).astype(bf16)
        o = _dot(p, _ld(v_s, slot, r0=a * T, n=(e - a) * T))
        b.acc = o if b.acc is None else b.acc + o

    def finish(b):
        l = jnp.sum(b.l, axis=1, keepdims=True)
        r = pltpu.reciprocal(l, approx=True)
        r = r * (2.0 - l * r)
        _st(ctx_s, hd, r0=b.i * T, val=b.acc * r)

    filler(0)
    prev = None
    for n, i in enumerate(list(range(NB - 1, -1, -1)) + [None]):
        b = _Blk(i) if i is not None else None
        ca, cb = chunks(b), chunks(prev)
        for c in range(max(len(ca), len(cb))):
            s = scores(b, *ca[c]) if c < len(ca) else None
            if c < len(cb):
                context(prev, *cb[c])
            if s is not None:
                keep(b, *ca[c], s)
        if b:
            b.m = jnp.max(b.mx, axis=1, keepdims=True)
        if prev:
            finish(prev)
        filler(n + 1)
        prev = b


def _weave(mxu, *others):
    for n, job in enumerate(mxu):
        out = job()
        todo = [other for vpu in others
                for other in vpu[n * len(vpu) // len(mxu):(n + 1) * len(vpu) // len(mxu)]]
        for t, other in enumerate(todo):
            r0 = t * (out.shape[0] // PAD) // len(todo) * PAD
            other(out[r0:r0 + PAD, 0:D])


def _zero(a):
    return jnp.minimum(pltpu.bitcast(a, i32)[0, 0] & 0xFFFF, 0)


def _after(tok, zero, *refs):
    if tok is None:
        return
    for ref in refs:
        if len(ref.shape) == 3:
            ref[zero + ref.shape[0] - 1, pl.ds(0, PAD), :] = tok.astype(ref.dtype)
        else:
            ref[_rows(zero + ref.shape[0] - PAD, PAD), pl.ds(0, D)] = tok.astype(ref.dtype)


def _kernel(x_hbm, ckv_hbm, wq_hbm, wk_hbm, wv_hbm, wo_hbm, wr_hbm, wg_hbm, wu_hbm, wd_hbm,
            c_hbm, wmod_hbm, out_hbm,
            x_s, ckv_s, wo_s, wr_s, wg_s, wu_s, wd_s, mod_s, w_s, k_s, q_s, v_s, ctx_s,
            in_sem, out_sem, fix_sem):
    copies = []

    def copy(hbm, vmem, *idx):
        if not idx and hbm.shape != vmem.shape:
            idx = (pl.ds(0, hbm.shape[0]),)
        if idx:
            hbm, vmem = hbm.at[idx], vmem.at[idx]
        copies.append(pltpu.make_async_copy(hbm, vmem, in_sem.at[len(copies)]))
        return copies[-1]

    def start(cps):
        for cp in cps:
            cp.start()

    def wait(cps):
        for cp in cps:
            cp.wait()

    stage4 = [copy(wo_hbm, wo_s), copy(wr_hbm, wr_s), copy(wg_hbm, wg_s), copy(wu_hbm, wu_s),
              copy(wd_hbm, wd_s)]

    def mod(j):
        return mod_s[:, pl.ds(j * M, M)]

    def qproj(hd, slot, i):
        h = jnp.concatenate([_ld(w_s, H + j, r0=i * T, n=T) for j in range(M // D)], axis=1)
        _st(q_s, slot, r0=i * T, val=_dot(h, _ld(w_s, hd, r0=0, n=M)) * QSCALE)

    def vproj(hd, slot, i):
        _st(v_s, slot, r0=i * T, val=_dot(_ld(ckv_s, r0=i * T, n=T), _ld(w_s, hd, r0=M + C, n=C)))

    def qv(hd, slot):
        return [functools.partial(f, hd, slot, i) for i in range(NB) for f in (qproj, vproj)]

    def phase1(ckv_raw, wq_raw, wk_raw, wv_raw, c_s, wmod_s):
        R0 = 768
        wk0_cp = copy(wk_hbm, wk_raw, pl.ds(0, C), pl.ds(0, G))
        ckv0_cp = copy(ckv_hbm, ckv_raw, pl.ds(0, R0))
        stage1 = [copy(ckv_hbm, ckv_raw, pl.ds(R0, S - R0)), copy(wk_hbm, wk_raw, pl.ds(0, C), pl.ds(G, G))]
        stage2 = [copy(wk_hbm, wk_raw, pl.ds(0, C), pl.ds(2 * G, 2 * G)),
                  copy(c_hbm, c_s), copy(wmod_hbm, wmod_s), copy(x_hbm, x_s)]
        stage3 = [copy(wq_hbm, wq_raw), copy(wv_hbm, wv_raw)]

        def per_head(raw, base, g):
            def job(r0, tok=None):
                _after(tok, zero, raw)
                w = raw[pl.ds(r0, 16), pl.ds(g * G, G), :].reshape(16, G * D)
                for j in range(G):
                    _st(w_s, g * G + j, r0=base + r0, val=w[:, j * D:(j + 1) * D])
            return [functools.partial(job, r0) for r0 in range(0, raw.shape[0] - 1, 16)]

        def kproj(heads, lo, hi):
            def job(hd, r0):
                if hd == 0:
                    ckv = ckv_raw[pl.ds(r0, 256), :]
                    _st(ckv_s, r0=r0, val=ckv)
                else:
                    ckv = _ld(ckv_s, r0=r0, n=256)
                k = _dot(ckv, _ld(w_s, hd, r0=M, n=C))
                _st(k_s, hd, r0=r0, val=k)
                return k
            return [functools.partial(job, hd, r0) for hd in heads for r0 in range(lo, hi, 256)]

        def modulation():
            cf = c_s[...].astype(f32)
            col = jnp.broadcast_to(_rb(cf * _sigmoid(cf)), (D, M)).T

            def job(j, tok):
                _after(tok, zero, wmod_s)
                w = wmod_s[pl.ds(0, M), pl.ds(j * D, D)].astype(f32)
                m = _rb(jnp.sum(w * col, axis=0, keepdims=True))
                mod_s[:, pl.ds(j * D, D)] = m
            return [functools.partial(job, j) for j in range(6 * M // D)]

        def norm1(r0, tok):
            _after(tok, zero, x_s)
            xf = x_s[pl.ds(r0, 16), :].astype(f32)
            xc = xf - jnp.mean(xf, axis=1, keepdims=True)
            xn = xc * lax.rsqrt(jnp.mean(xc * xc, axis=1, keepdims=True) + EPS)
            h = xn * (1.0 + mod(1)) + mod(0)
            for j in range(M // D):
                _st(w_s, H + j, r0=r0, val=h[:, j * D:(j + 1) * D])

        start([wk0_cp, ckv0_cp])
        start(stage1)
        wk0_cp.wait()
        zero = _zero(wk_raw[0, pl.ds(0, G), :])
        _weave(per_head(wk_raw, M, 0), [])
        ckv0_cp.wait()
        _weave(kproj(range(8), 0, R0), [])
        start(stage2)
        wait(stage1)
        _weave(kproj(range(8), R0, S), per_head(wk_raw, M, 1))
        _weave(kproj(range(8, 12), 0, S))
        start(stage3)
        wait(stage2)
        _weave(kproj(range(12, 16), 0, S), per_head(wk_raw, M, 2), modulation())
        _weave(kproj(range(16, 22), 0, S), per_head(wk_raw, M, 3),
               [functools.partial(norm1, r0) for r0 in range(0, S, 16)])
        start(stage4)
        wait(stage3)
        _weave(kproj(range(22, H), 0, S),
               [job for g in range(NG) for job in per_head(wq_raw, 0, g) + per_head(wv_raw, M + C, g)])
        _weave(qv(0, 0))

    V = pltpu.VMEM
    pl.run_scoped(phase1, V((S, C), bf16), V((M + 1, H, D), bf16), V((C + 1, H, D), bf16),
                  V((C + 1, H, D), bf16),
                  V((1, M), bf16), V((M + PAD, 6 * M), bf16))

    def next_head(hd, slot):
        jobs = qv(hd, slot)
        cuts = [0, 1] + [1 + (27 * n) // NB for n in range(1, NB + 1)] + [len(jobs)]
        return lambda n: _weave(jobs[cuts[n]:cuts[n + 1]], [])

    def pair(p, _):
        _attention(q_s, k_s, v_s, ctx_s, 2 * p + 1, 1, next_head(2 * p + 2, 0))
        _attention(q_s, k_s, v_s, ctx_s, 2 * p + 2, 0, next_head(2 * p + 3, 1))

    _attention(q_s, k_s, v_s, ctx_s, 0, 0, next_head(1, 1))
    lax.fori_loop(0, H // 2 - 1, pair, None)

    def phase3(y_s, key_s, top_s, xh_s, out_s, wgu_s):
        wait(stage4)
        zero = _zero(wo_s[pl.ds(0, 16), pl.ds(0, D)])
        sub = lax.broadcasted_iota(i32, (TOPK, D), 0)
        lane = lax.broadcasted_iota(i32, (TOPK, D), 1)

        def oproj(r0, n, slot):
            acc = {}

            def job(j, h0):
                ctx = jnp.concatenate([_ld(ctx_s, h0 + t, r0=r0, n=n) for t in range(CH)], axis=1)
                y = _dot(ctx, wo_s[pl.ds(h0 * D, CH * D), pl.ds(j * D, D)])
                acc[j] = acc[j] + y if h0 else y
                if h0 + CH == H:
                    y_s[slot][pl.ds(0, n), pl.ds(j * D, D)] = acc[j]
                return y
            return [functools.partial(job, j, h0) for j in range(M // D) for h0 in range(0, H, CH)]

        def out_copy(b):
            return pltpu.make_async_copy(out_s.at[_rows(b * RB, RB)], out_hbm.at[_rows(b * RB, RB)],
                                         out_sem.at[b])

        def epilogue(r0, slot, off, n, tok=None):
            _after(tok, zero, x_s, y_s[slot])
            rows = _rows(r0, n)
            ga, sb, cb, gb = mod(2), mod(3), _rb(1.0 + mod(4)), mod(5)
            x1 = _rb(x_s[rows, :].astype(f32) + _rb(ga * _rb(y_s[slot][pl.ds(off, n), :])))
            mean = jnp.mean(x1, axis=1, keepdims=True)
            xc = x1 - mean
            var = _rb(jnp.mean(xc * xc, axis=1, keepdims=True))
            inv = 1.0 / _rb(jnp.sqrt(_rb(var + EPS)))
            h2 = _rb(_rb(_rb(_rb(x1 - _rb(mean)) * inv) * cb) + sb)
            xh_s[rows, :] = pltpu.bitcast(x1, u32) | (pltpu.bitcast(h2, u32) >> 16)
            out_s[rows, :] = (x1 + _rb(gb * h2)).astype(bf16)
            wr = wr_s[...].astype(f32)
            prod = h2[:, 0:D] * wr[0:1]
            for j in range(1, M // D):
                prod = prod + h2[:, j * D:(j + 1) * D] * wr[j:j + 1]
            r = jnp.broadcast_to(_rb(jnp.sum(prod, axis=1, keepdims=True)), (n, D))
            bits = lax.bitcast_convert_type(r, i32)
            code = lax.shift_right_logical(bits, 16)
            code = jnp.where(bits < 0, 0xFFFF - code, code + 0x8000)
            code = jnp.where(r == 0.0, 0x8000, code)
            code = jnp.where(r != r, 0, code)
            key = code * S + (S - 1 + KEY0 - r0) - lax.broadcasted_iota(i32, (n, D), 0)
            key_s[pl.ds(off % T, n), :] = lax.bitcast_convert_type(key, f32)

        def select(tok=None):
            best = top_s[...]
            cols = [key_s[pl.ds(8 * t, 8), :] for t in range(T // 8)]
            flat = jnp.zeros((TOPK, D), f32)
            for t, col in enumerate(cols):
                flat = jnp.where(lane - sub == 8 * t, col, flat)
            new = None
            for cand in (flat, jnp.where(lane == sub, best, 0.0)):
                cand = jnp.broadcast_to(jnp.max(cand, axis=0, keepdims=True), (TOPK, D))
                above = sum((col > cand).astype(f32) for col in cols + [best])
                rank = jnp.sum(above, axis=0, keepdims=True)
                pick = jnp.where(rank == sub.astype(f32), cand, 0.0)
                new = pick if new is None else jnp.maximum(new, pick)
            top_s[...] = jnp.broadcast_to(jnp.max(new, axis=1, keepdims=True), (TOPK, D))

        def epilogues(r0, slot, rows=RB, n=16):
            jobs = []
            for off in range(0, rows, n):
                jobs.append(functools.partial(epilogue, r0 + off, slot, off, n))
                if (off + n) % T == 0:
                    jobs.append(select)
            return jobs

        def flip(t, src):
            def job(r0, tok):
                _after(tok, zero, src)
                wgu_s[t, :, pl.ds(r0, D)] = src[pl.ds(r0, D), :].T
            return [functools.partial(job, r0) for r0 in range(0, F - D, D)] + [
                functools.partial(job, F - D)]

        NR = S // RB
        top_s[...] = jnp.zeros(top_s.shape, f32)
        last = oproj((NR - 1) * RB, RB, 1)
        cuts = [0] * 4 + [len(last) * n // 15 for n in range(1, 16)]
        _attention(q_s, k_s, v_s, ctx_s, H - 1, 1, lambda n: _weave(last[cuts[n]:cuts[n + 1]]))

        def blocks(n, _):
            b = NR - 2 - 2 * n
            _weave(oproj(b * RB, RB, 0), epilogues((b + 1) * RB, 1))
            out_copy(b + 1).start()
            _weave(oproj((b - 1) * RB, RB, 1), epilogues(b * RB, 0))
            out_copy(b).start()

        lax.fori_loop(0, NR // 2 - 1, blocks, None)
        _weave(oproj(T, T, 0), epilogues(RB, 1), flip(0, wg_s))
        out_copy(1).start()
        _weave(oproj(0, T, 1), epilogues(T, 0, T), flip(1, wu_s))
        _weave(epilogues(0, 1, T, T))
        out_copy(0).start()

        top = lax.bitcast_convert_type(top_s[...], i32) - KEY0
        sel = S - 1 - (top & (S - 1))
        code = lax.shift_right_logical(top, 11)
        code = jnp.where(code >= 0x8000, code - 0x8000, 0xFFFF - code)
        r_sel = lax.bitcast_convert_type(code * 0x10000, f32)[:, 0:1]
        idx = [sel[j, 0] for j in range(TOPK)]

        both = jnp.concatenate([xh_s[pl.ds(t, 1), :] for t in idx], axis=0)
        hsel = pltpu.bitcast(both << 16, f32)
        xsel = pltpu.bitcast((both >> 16) << 16, f32)
        lhs = jnp.concatenate([hsel, hsel], axis=0).astype(bf16)
        gate = _rb(_dot(lhs, wgu_s[0]))
        act = _rb(gate * _sigmoid(gate)) * _rb(_dot(lhs, wgu_s[1]))
        y = _rb(_rb(_dot(act.astype(bf16), wd_s[...])[0:TOPK]) * _sigmoid(r_sel))
        fixed = xsel + _rb(mod(5) * _rb(hsel + y))

        for b in range(NR):
            out_copy(b).wait()
        tiles = [pl.multiple_of((t // 16) * 16, 16) for t in idx]
        row = lax.broadcasted_iota(i32, (16, M), 0)
        for j in range(TOPK):
            cur = out_s[pl.ds(tiles[j], 16), :].astype(f32)
            cur = jnp.where(row == idx[j] - tiles[j], fixed[j:j + 1], cur)
            out_s[pl.ds(tiles[j], 16), :] = cur.astype(bf16)

        def fix_copy(j):
            return pltpu.make_async_copy(out_s.at[pl.ds(tiles[j], 16)], out_hbm.at[pl.ds(tiles[j], 16)],
                                         fix_sem.at[j])

        fresh = []
        for j in range(TOPK):
            new = tiles[j] >= 0
            for k in range(j):
                new = jnp.logical_and(new, tiles[j] != tiles[k])
            fresh.append(new)
        for j in range(TOPK):
            pl.when(fresh[j])(fix_copy(j).start)
        for j in range(TOPK):
            pl.when(fresh[j])(fix_copy(j).wait)

    pl.run_scoped(phase3, [V((RB + PAD, M), f32)] * 2, V((T, D), f32), V((TOPK, D), f32),
                  V((S, M), u32), V((S, M), bf16), V((2, M, F), bf16))


@jax.jit
def pallas_adaLN_cond__compressed_kv_cla__moe_arch_mod__prompt_kernel(
    A_x: jax.Array,
    A_c_kv: jax.Array,
    A_w_q: jax.Array,
    A_w_uk: jax.Array,
    A_w_uv: jax.Array,
    A_w_o: jax.Array,
    B_x: jax.Array,
    B_w_r: jax.Array,
    B_w_gate: jax.Array,
    B_w_up: jax.Array,
    B_w_down: jax.Array,
    c: jax.Array,
    w_mod: jax.Array,
):
    del B_x
    V = pltpu.VMEM
    scratch = [
        V((S + PAD, M), bf16), V((S // 2, C), u32),
        V((H * D, M), bf16), V((M // D, D), bf16),
        V((F + PAD, M), bf16), V((F + PAD, M), bf16), V((F, M), bf16),
        V((1, 6 * M), f32),
        V((H + M // D, S // 2, D), u32),
        V((H, S // 2, D), u32),
        V((2, S // 2, D), u32), V((2, S // 2, D), u32),
        V((H, S // 2, D), u32),
        pltpu.SemaphoreType.DMA((16,)), pltpu.SemaphoreType.DMA((S // RB,)),
        pltpu.SemaphoreType.DMA((TOPK,)),
    ]
    out = pl.pallas_call(
        _kernel,
        in_specs=[pl.BlockSpec(memory_space=pltpu.HBM)] * 12,
        out_specs=pl.BlockSpec(memory_space=pltpu.HBM),
        out_shape=jax.ShapeDtypeStruct((S, M), bf16),
        scratch_shapes=scratch,
        compiler_params=pltpu.CompilerParams(vmem_limit_bytes=120 * 2 ** 20),
    )(A_x.reshape(S, M), A_c_kv.reshape(S, C), A_w_q, A_w_uk, A_w_uv, A_w_o.reshape(H * D, M),
      B_w_r.reshape(M // D, D), B_w_gate.T, B_w_up.T, B_w_down, c, w_mod)
    return out.reshape(A_x.shape)
```

```python
import functools

import jax
import jax.numpy as jnp
from jax import lax
import jax.experimental.pallas as pl
import jax.experimental.pallas.tpu as pltpu

S, M, C, D, H, F, TOPK = 2048, 640, 512, 128, 32, 1728, 8
G = 8
NG = H // G
T = 128
NB = S // T
CH = 4
RB = 256
PAD = 16
EPS = 1e-5
KEY0 = 0x00800000
QSCALE = D ** -0.5 * 1.4426950408889634
NT = (((1,), (1,)), ((), ()))

f32, bf16, u32, i32 = jnp.float32, jnp.bfloat16, jnp.uint32, jnp.int32


def _rb(a):
    return a.astype(bf16).astype(f32)


def _sigmoid(a):
    return _rb(1.0 / _rb(1.0 + _rb(jnp.exp(-a))))


def _rows(r0, n):
    if isinstance(r0, int):
        return pl.ds(r0, n)
    return pl.ds(pl.multiple_of(r0, n & -n), n)


def _ld(ref, *idx, r0, n):
    return pltpu.bitcast(ref[(*idx, _rows(r0 // 2, n // 2), slice(None))], bf16)


def _st(ref, *idx, r0, val):
    ref[(*idx, _rows(r0 // 2, val.shape[0] // 2), slice(None))] = pltpu.bitcast(
        val.astype(bf16), u32)


def _dot(a, b):
    return jnp.dot(a, b, preferred_element_type=f32)


def _dot_nt(a, b):
    return lax.dot_general(a, b, NT, preferred_element_type=f32)


class _Blk:
    def __init__(self, i):
        self.i, self.s, self.mx, self.m, self.l, self.acc = i, {}, None, None, None, None


def _attention(q_s, k_s, v_s, zero, hd, slot, filler, lag=3):
    tri = (lax.broadcasted_iota(i32, (T, T), 1) <= lax.broadcasted_iota(i32, (T, T), 0))

    def chunks(b):
        n = b.i + 1 if b else 0
        return [(a, min(a + CH, n)) for a in range(0, n, CH)]

    def scores(b, a, e):
        return _dot_nt(_ld(q_s, slot, r0=b.i * T, n=T), _ld(k_s, hd, r0=a * T, n=(e - a) * T))

    def keep(b, a, e, s):
        for t in range(a, e):
            x = s[:, (t - a) * T:(t - a + 1) * T]
            if t == b.i:
                x = jnp.where(tri, x, -1e9)
            b.mx = x if b.mx is None else jnp.maximum(b.mx, x)
            b.s[t] = x

    def context(b, a, e):
        ps = sums = [jnp.exp2(b.s[t] - b.m) for t in range(a, e)]
        while len(sums) > 1:
            sums = [functools.reduce(jnp.add, sums[t:t + 2]) for t in range(0, len(sums), 2)]
        b.l = sums[0] if b.l is None else b.l + sums[0]
        p = (jnp.concatenate(ps, axis=1) if len(ps) > 1 else ps[0]).astype(bf16)
        o = _dot(p, _ld(v_s, slot, r0=a * T, n=(e - a) * T))
        b.acc = o if b.acc is None else b.acc + o

    def finish(b):
        l = jnp.sum(b.l, axis=1, keepdims=True)
        r = pltpu.reciprocal(l, approx=True)
        r = r * (2.0 - l * r)
        _st(k_s, hd + zero, r0=b.i * T, val=b.acc * r)

    filler(0)
    prev, done = None, []
    for n, i in enumerate(list(range(NB - 1, -1, -1)) + [None]):
        b = _Blk(i) if i is not None else None
        ca, cb = chunks(b), chunks(prev)
        for c in range(max(len(ca), len(cb))):
            s = scores(b, *ca[c]) if c < len(ca) else None
            if c < len(cb):
                context(prev, *cb[c])
            if s is not None:
                keep(b, *ca[c], s)
        if b:
            b.m = jnp.max(b.mx, axis=1, keepdims=True)
        if prev:
            done.append(prev)
        if len(done) > lag:
            finish(done.pop(0))
        filler(n + 1)
        prev = b
    for b in done:
        finish(b)


def _weave(mxu, *others):
    for n, job in enumerate(mxu):
        out = job()
        todo = [other for vpu in others
                for other in vpu[n * len(vpu) // len(mxu):(n + 1) * len(vpu) // len(mxu)]]
        for t, other in enumerate(todo):
            r0 = t * (out.shape[0] // PAD) // len(todo) * PAD
            other(out[r0:r0 + PAD, 0:D])


def _skip(n):
    return [lambda tok: None] * n


def _zero(a):
    return jnp.minimum(pltpu.bitcast(a, i32)[0, 0] & 0xFFFF, 0)


def _after(tok, zero, *refs):
    if tok is None:
        return
    for ref in refs:
        if len(ref.shape) == 3:
            ref[zero + ref.shape[0] - 1, pl.ds(0, PAD), :] = tok.astype(ref.dtype)
        else:
            ref[_rows(zero + ref.shape[0] - PAD, PAD), pl.ds(0, D)] = tok.astype(ref.dtype)


def _kernel(x_hbm, ckv_hbm, wq_hbm, wk_hbm, wv_hbm, wo_hbm, wr_hbm, wg_hbm, wu_hbm, wd_hbm,
            c_hbm, wmod_hbm, out_hbm,
            x_s, ckv_s, wo_s, wr_s, wg_s, wu_s, wd_s, mod_s, w_s, k_s, q_s, v_s,
            in_sem, out_sem, fix_sem):
    copies = []

    def copy(hbm, vmem, *idx):
        if not idx and hbm.shape != vmem.shape:
            idx = (pl.ds(0, hbm.shape[0]),)
        if idx:
            hbm, vmem = hbm.at[idx], vmem.at[idx]
        copies.append(pltpu.make_async_copy(hbm, vmem, in_sem.at[len(copies)]))
        return copies[-1]

    def start(cps):
        for cp in cps:
            cp.start()

    def wait(cps):
        for cp in cps:
            cp.wait()

    stage4 = [copy(wo_hbm, wo_s), copy(wr_hbm, wr_s), copy(wg_hbm, wg_s), copy(wu_hbm, wu_s),
              copy(wd_hbm, wd_s)]

    def mod(j):
        return mod_s[:, pl.ds(j * M, M)]

    def qproj(hd, slot, i):
        h = jnp.concatenate([_ld(w_s, H + j, r0=i * T, n=T) for j in range(M // D)], axis=1)
        _st(q_s, slot, r0=i * T, val=_dot(h, _ld(w_s, hd, r0=0, n=M)) * QSCALE)

    def vproj(hd, slot, i):
        _st(v_s, slot, r0=i * T, val=_dot(_ld(ckv_s, r0=i * T, n=T), _ld(w_s, hd, r0=M + C, n=C)))

    def qv(hd, slot):
        return [functools.partial(f, hd, slot, i) for i in range(NB) for f in (qproj, vproj)]

    def phase1(ckv_raw, wq_raw, wk_raw, wv_raw, c_s, wmod_s):
        R0, R1 = 256, 1024
        first = [copy(wk_hbm, wk_raw, pl.ds(r0, D), pl.ds(0, G)) for r0 in range(0, C, D)]
        ckv0_cp = copy(ckv_hbm, ckv_raw, pl.ds(0, R0))
        ckv1_cp = copy(ckv_hbm, ckv_raw, pl.ds(R0, R1 - R0))
        stage1 = [copy(ckv_hbm, ckv_raw, pl.ds(R1, S - R1)),
                  copy(wk_hbm, wk_raw, pl.ds(0, C), pl.ds(G, G))]
        stage2 = [copy(wk_hbm, wk_raw, pl.ds(0, C), pl.ds(2 * G, 2 * G)),
                  copy(c_hbm, c_s), copy(wmod_hbm, wmod_s), copy(x_hbm, x_s)]
        stage3 = [copy(wq_hbm, wq_raw), copy(wv_hbm, wv_raw)]

        def per_head(raw, base, g):
            def job(r0, tok=None):
                _after(tok, zero, raw)
                w = raw[pl.ds(r0, 16), pl.ds(g * G, G), :].reshape(16, G * D)
                for j in range(G):
                    _st(w_s, g * G + j, r0=base + r0, val=w[:, j * D:(j + 1) * D])
            return [functools.partial(job, r0) for r0 in range(0, raw.shape[0] - 1, 16)]

        def kproj(heads, lo, hi):
            def job(hd, r0):
                if hd == 0:
                    ckv = ckv_raw[pl.ds(r0, 256), :]
                    _st(ckv_s, r0=r0, val=ckv)
                else:
                    ckv = _ld(ckv_s, r0=r0, n=256)
                k = _dot(ckv, _ld(w_s, hd, r0=M, n=C))
                _st(k_s, hd, r0=r0, val=k)
                return k
            return [functools.partial(job, hd, r0) for hd in heads for r0 in range(lo, hi, 256)]

        def modulation():
            cf = c_s[...].astype(f32)
            col = jnp.broadcast_to(_rb(cf * _sigmoid(cf)), (D, M)).T

            acc = {}

            def job(c0, r0, tok):
                _after(tok, zero, wmod_s)
                w = wmod_s[pl.ds(r0, D), pl.ds(c0, 2 * D)].astype(f32)
                w = w * jnp.concatenate([col[r0:r0 + D]] * 2, axis=1)
                w = jnp.sum(w.reshape(D // 8, 8, 2 * D), axis=0)
                acc[c0] = acc[c0] + w if r0 else w
                if r0 + D == M:
                    mod_s[:, pl.ds(c0, 2 * D)] = _rb(jnp.sum(acc[c0], axis=0, keepdims=True))
            return [functools.partial(job, c0, r0)
                    for c0 in range(0, 6 * M, 2 * D) for r0 in range(0, M, D)]

        def norm1(r0, tok):
            _after(tok, zero, x_s)
            xf = x_s[pl.ds(r0, 16), :].astype(f32)
            xc = xf - jnp.mean(xf, axis=1, keepdims=True)
            xn = xc * lax.rsqrt(jnp.mean(xc * xc, axis=1, keepdims=True) + EPS)
            h = xn * (1.0 + mod(1)) + mod(0)
            for j in range(M // D):
                _st(w_s, H + j, r0=r0, val=h[:, j * D:(j + 1) * D])

        start(first + [ckv0_cp, ckv1_cp])
        for n, cp in enumerate(first):
            cp.wait()
            if n == 0:
                zero = _zero(wk_raw[0, pl.ds(0, G), :])
            _weave(per_head(wk_raw, M, 0)[n * D // 16:(n + 1) * D // 16])
        start(stage1)
        ckv0_cp.wait()
        _weave(kproj(range(8), 0, R0))
        start(stage2)
        ckv1_cp.wait()
        _weave(kproj(range(8), R0, R1))
        wait(stage1)
        _weave(kproj(range(8), R1, S), per_head(wk_raw, M, 1))
        _weave(kproj(range(8, 13), 0, S))
        start(stage3)
        wait(stage2)
        _weave(kproj(range(13, 17), 0, S), per_head(wk_raw, M, 2) + _skip(14),
               _skip(6) + modulation())
        _weave(kproj(range(17, 24), 0, S), per_head(wk_raw, M, 3),
               [functools.partial(norm1, r0) for r0 in range(0, S, 16)] + _skip(12))
        start(stage4)
        wait(stage3)
        _weave(kproj(range(24, H), 0, S),
               [job for g in range(NG) for job in per_head(wq_raw, 0, g) + per_head(wv_raw, M + C, g)])
        _weave(qv(0, 0))

    V = pltpu.VMEM
    pl.run_scoped(phase1, V((S, C), bf16), V((M + 1, H, D), bf16), V((C + 1, H, D), bf16),
                  V((C + 1, H, D), bf16),
                  V((1, M), bf16), V((M + PAD, 6 * M), bf16))

    zero = _zero(x_s[pl.ds(0, 16), pl.ds(0, D)])

    def next_head(hd, slot):
        jobs = qv(hd, slot)
        cuts = [0, 1] + [1 + (27 * n) // NB for n in range(1, NB + 1)] + [len(jobs)]
        return lambda n: _weave(jobs[cuts[n]:cuts[n + 1]])

    def pair(p, _):
        _attention(q_s, k_s, v_s, zero, 2 * p + 1, 1, next_head(2 * p + 2, 0))
        _attention(q_s, k_s, v_s, zero, 2 * p + 2, 0, next_head(2 * p + 3, 1))

    _attention(q_s, k_s, v_s, zero, 0, 0, next_head(1, 1))
    lax.fori_loop(0, H // 2 - 1, pair, None)

    def phase3(y_s, key_s, top_s, xh_s, out_s, wgu_s):
        wait(stage4)
        sub = lax.broadcasted_iota(i32, (TOPK, D), 0)
        lane = lax.broadcasted_iota(i32, (TOPK, D), 1)

        def oproj(r0, n, slot):
            acc = {}

            def job(j, h0):
                ctx = jnp.concatenate([_ld(k_s, h0 + t, r0=r0, n=n) for t in range(CH)], axis=1)
                y = _dot(ctx, wo_s[pl.ds(h0 * D, CH * D), pl.ds(j * D, D)])
                acc[j] = acc[j] + y if h0 else y
                if h0 + CH == H:
                    y_s[slot][pl.ds(0, n), pl.ds(j * D, D)] = acc[j]
                return y
            return [functools.partial(job, j, h0) for j in range(M // D) for h0 in range(0, H, CH)]

        def out_copy(b):
            return pltpu.make_async_copy(out_s.at[_rows(b * RB, RB)], out_hbm.at[_rows(b * RB, RB)],
                                         out_sem.at[b])

        def epilogue(r0, slot, off, n, tok=None):
            _after(tok, zero, x_s, y_s[slot])
            rows = _rows(r0, n)
            ga, sb, cb, gb = mod(2), mod(3), _rb(1.0 + mod(4)), mod(5)
            x1 = _rb(x_s[rows, :].astype(f32) + _rb(ga * _rb(y_s[slot][pl.ds(off, n), :])))
            mean = jnp.mean(x1, axis=1, keepdims=True)
            xc = x1 - mean
            var = _rb(jnp.mean(xc * xc, axis=1, keepdims=True))
            inv = 1.0 / _rb(jnp.sqrt(_rb(var + EPS)))
            h2 = _rb(_rb(_rb(_rb(x1 - _rb(mean)) * inv) * cb) + sb)
            xh_s[rows, :] = pltpu.bitcast(x1, u32) | (pltpu.bitcast(h2, u32) >> 16)
            out_s[rows, :] = (x1 + _rb(gb * h2)).astype(bf16)
            wr = wr_s[...].astype(f32)
            prod = h2[:, 0:D] * wr[0:1]
            for j in range(1, M // D):
                prod = prod + h2[:, j * D:(j + 1) * D] * wr[j:j + 1]
            r = jnp.broadcast_to(_rb(jnp.sum(prod, axis=1, keepdims=True)), (n, D))
            bits = lax.bitcast_convert_type(r, i32)
            code = lax.shift_right_logical(bits, 16)
            code = jnp.where(bits < 0, 0xFFFF - code, code + 0x8000)
            code = jnp.where(r == 0.0, 0x8000, code)
            code = jnp.where(r != r, 0, code)
            key = code * S + (S - 1 + KEY0 - r0) - lax.broadcasted_iota(i32, (n, D), 0)
            key_s[pl.ds(off % T, n), :] = lax.bitcast_convert_type(key, f32)

        def select(tok=None):
            best = top_s[...]
            cols = [key_s[pl.ds(8 * t, 8), :] for t in range(T // 8)]
            flat = jnp.zeros((TOPK, D), f32)
            for t, col in enumerate(cols):
                flat = jnp.where(lane - sub == 8 * t, col, flat)
            new = None
            for cand in (flat, jnp.where(lane == sub, best, 0.0)):
                cand = jnp.broadcast_to(jnp.max(cand, axis=0, keepdims=True), (TOPK, D))
                above = sum((col > cand).astype(f32) for col in cols + [best])
                rank = jnp.sum(above, axis=0, keepdims=True)
                pick = jnp.where(rank == sub.astype(f32), cand, 0.0)
                new = pick if new is None else jnp.maximum(new, pick)
            top_s[...] = jnp.broadcast_to(jnp.max(new, axis=1, keepdims=True), (TOPK, D))

        def epilogues(r0, slot, rows=RB, n=16):
            jobs = []
            for off in range(0, rows, n):
                jobs.append(functools.partial(epilogue, r0 + off, slot, off, n))
                if (off + n) % T == 0:
                    jobs.append(select)
            return jobs

        def flip(t, src):
            def job(r0, tok):
                _after(tok, zero, src)
                wgu_s[t, :, pl.ds(r0, D)] = src[pl.ds(r0, D), :].T
            return [functools.partial(job, r0) for r0 in range(0, F - D, D)] + [
                functools.partial(job, F - D)]

        NR = S // RB
        top_s[...] = jnp.zeros(top_s.shape, f32)
        last = oproj((NR - 1) * RB, RB, 1)
        cuts = [0] * 4 + [len(last) * n // 15 for n in range(1, 16)]
        flips = _skip(10) + flip(0, wg_s) + flip(1, wu_s) + _skip(2)
        _attention(q_s, k_s, v_s, 0, H - 1, 1, lag=0, filler=lambda n: _weave(
            last[cuts[n]:cuts[n + 1]], flips[cuts[n]:cuts[n + 1]]))

        def blocks(n, _):
            b = NR - 2 - 2 * n
            _weave(oproj(b * RB, RB, 0), epilogues((b + 1) * RB, 1) + _skip(2))
            out_copy(b + 1).start()
            _weave(oproj((b - 1) * RB, RB, 1), epilogues(b * RB, 0) + _skip(2))
            out_copy(b).start()

        lax.fori_loop(0, NR // 2 - 1, blocks, None)
        _weave(oproj(T, T, 0), epilogues(RB, 1))
        out_copy(1).start()
        _weave(oproj(0, T, 1), epilogues(T, 0, T) + _skip(2))
        _weave(epilogues(0, 1, T, T))
        out_copy(0).start()

        top = lax.bitcast_convert_type(top_s[...], i32) - KEY0
        sel = S - 1 - (top & (S - 1))
        code = lax.shift_right_logical(top, 11)
        code = jnp.where(code >= 0x8000, code - 0x8000, 0xFFFF - code)
        r_sel = lax.bitcast_convert_type(code * 0x10000, f32)[:, 0:1]
        idx = [sel[j, 0] for j in range(TOPK)]

        both = jnp.concatenate([xh_s[pl.ds(t, 1), :] for t in idx], axis=0)
        hsel = pltpu.bitcast(both << 16, f32)
        xsel = pltpu.bitcast((both >> 16) << 16, f32)
        lhs = jnp.concatenate([hsel, hsel], axis=0).astype(bf16)
        gate = _rb(_dot(lhs, wgu_s[0]))
        act = _rb(gate * _sigmoid(gate)) * _rb(_dot(lhs, wgu_s[1]))
        y = _rb(_rb(_dot(act.astype(bf16), wd_s[...])[0:TOPK]) * _sigmoid(r_sel))
        fixed = xsel + _rb(mod(5) * _rb(hsel + y))

        for b in range(NR):
            out_copy(b).wait()
        tiles = [pl.multiple_of((t // 16) * 16, 16) for t in idx]
        row = lax.broadcasted_iota(i32, (16, M), 0)
        for j in range(TOPK):
            cur = out_s[pl.ds(tiles[j], 16), :].astype(f32)
            cur = jnp.where(row == idx[j] - tiles[j], fixed[j:j + 1], cur)
            out_s[pl.ds(tiles[j], 16), :] = cur.astype(bf16)

        def fix_copy(j):
            return pltpu.make_async_copy(out_s.at[pl.ds(tiles[j], 16)], out_hbm.at[pl.ds(tiles[j], 16)],
                                         fix_sem.at[j])

        fresh = []
        for j in range(TOPK):
            new = tiles[j] >= 0
            for k in range(j):
                new = jnp.logical_and(new, tiles[j] != tiles[k])
            fresh.append(new)
        for j in range(TOPK):
            pl.when(fresh[j])(fix_copy(j).start)
        for j in range(TOPK):
            pl.when(fresh[j])(fix_copy(j).wait)

    pl.run_scoped(phase3, [V((RB + PAD, M), f32)] * 2, V((T, D), f32), V((TOPK, D), f32),
                  V((S, M), u32), V((S, M), bf16), V((2, M, F), bf16))


@jax.jit
def pallas_adaLN_cond__compressed_kv_cla__moe_arch_mod__prompt_kernel(
    A_x: jax.Array,
    A_c_kv: jax.Array,
    A_w_q: jax.Array,
    A_w_uk: jax.Array,
    A_w_uv: jax.Array,
    A_w_o: jax.Array,
    B_x: jax.Array,
    B_w_r: jax.Array,
    B_w_gate: jax.Array,
    B_w_up: jax.Array,
    B_w_down: jax.Array,
    c: jax.Array,
    w_mod: jax.Array,
):
    del B_x
    V = pltpu.VMEM
    scratch = [
        V((S + PAD, M), bf16), V((S // 2, C), u32),
        V((H * D, M), bf16), V((M // D, D), bf16),
        V((F + PAD, M), bf16), V((F + PAD, M), bf16), V((F, M), bf16),
        V((1, 6 * M), f32),
        V((H + M // D, S // 2, D), u32),
        V((H, S // 2, D), u32),
        V((2, S // 2, D), u32), V((2, S // 2, D), u32),
        pltpu.SemaphoreType.DMA((19,)), pltpu.SemaphoreType.DMA((S // RB,)),
        pltpu.SemaphoreType.DMA((TOPK,)),
    ]
    out = pl.pallas_call(
        _kernel,
        in_specs=[pl.BlockSpec(memory_space=pltpu.HBM)] * 12,
        out_specs=pl.BlockSpec(memory_space=pltpu.HBM),
        out_shape=jax.ShapeDtypeStruct((S, M), bf16),
        scratch_shapes=scratch,
        compiler_params=pltpu.CompilerParams(vmem_limit_bytes=120 * 2 ** 20),
    )(A_x.reshape(S, M), A_c_kv.reshape(S, C), A_w_q, A_w_uk, A_w_uv, A_w_o.reshape(H * D, M),
      B_w_r.reshape(M // D, D), B_w_gate.T, B_w_up.T, B_w_down, c, w_mod)
    return out.reshape(A_x.shape)
```

```python
import functools

import jax
import jax.numpy as jnp
from jax import lax
import jax.experimental.pallas as pl
import jax.experimental.pallas.tpu as pltpu

S, M, C, D, H, F, TOPK = 2048, 640, 512, 128, 32, 1728, 8
G = 8
NG = H // G
T = 128
NB = S // T
CH = 4
RB = 256
PAD = 16
EPS = 1e-5
KEY0 = 0x00800000
QSCALE = D ** -0.5 * 1.4426950408889634
NT = (((1,), (1,)), ((), ()))

f32, bf16, u32, i32 = jnp.float32, jnp.bfloat16, jnp.uint32, jnp.int32


def _rb(a):
    return a.astype(bf16).astype(f32)


def _sigmoid(a):
    return _rb(1.0 / _rb(1.0 + _rb(jnp.exp(-a))))


def _rows(r0, n):
    if isinstance(r0, int):
        return pl.ds(r0, n)
    return pl.ds(pl.multiple_of(r0, n & -n), n)


def _ld(ref, *idx, r0, n):
    return pltpu.bitcast(ref[(*idx, _rows(r0 // 2, n // 2), slice(None))], bf16)


def _st(ref, *idx, r0, val):
    ref[(*idx, _rows(r0 // 2, val.shape[0] // 2), slice(None))] = pltpu.bitcast(
        val.astype(bf16), u32)


def _dot(a, b):
    return jnp.dot(a, b, preferred_element_type=f32)


def _dot_nt(a, b):
    return lax.dot_general(a, b, NT, preferred_element_type=f32)


class _Blk:
    def __init__(self, i):
        self.i, self.s, self.mx, self.m, self.l, self.acc = i, {}, None, None, None, None


def _attention(q_s, k_s, v_s, zero, hd, slot, filler, lag=3):
    tri = (lax.broadcasted_iota(i32, (T, T), 1) <= lax.broadcasted_iota(i32, (T, T), 0))

    def chunks(b):
        n = b.i + 1 if b else 0
        return [(a, min(a + CH, n)) for a in range(0, n, CH)]

    def scores(b, a, e):
        return _dot_nt(_ld(q_s, slot, r0=b.i * T, n=T), _ld(k_s, hd, r0=a * T, n=(e - a) * T))

    def keep(b, a, e, s):
        for t in range(a, e):
            x = s[:, (t - a) * T:(t - a + 1) * T]
            if t == b.i:
                x = jnp.where(tri, x, -1e9)
            b.mx = x if b.mx is None else jnp.maximum(b.mx, x)
            b.s[t] = x

    def context(b, a, e):
        ps = sums = [jnp.exp2(b.s[t] - b.m) for t in range(a, e)]
        while len(sums) > 1:
            sums = [functools.reduce(jnp.add, sums[t:t + 2]) for t in range(0, len(sums), 2)]
        b.l = sums[0] if b.l is None else b.l + sums[0]
        p = (jnp.concatenate(ps, axis=1) if len(ps) > 1 else ps[0]).astype(bf16)
        o = _dot(p, _ld(v_s, slot, r0=a * T, n=(e - a) * T))
        b.acc = o if b.acc is None else b.acc + o

    def finish(b):
        l = jnp.sum(b.l, axis=1, keepdims=True)
        r = pltpu.reciprocal(l, approx=True)
        r = r * (2.0 - l * r)
        _st(k_s, hd + zero, r0=b.i * T, val=b.acc * r)

    filler(0)
    prev, done = None, []
    for n, i in enumerate(list(range(NB - 1, -1, -1)) + [None]):
        b = _Blk(i) if i is not None else None
        ca, cb = chunks(b), chunks(prev)
        for c in range(max(len(ca), len(cb))):
            s = scores(b, *ca[c]) if c < len(ca) else None
            if c < len(cb):
                context(prev, *cb[c])
            if s is not None:
                keep(b, *ca[c], s)
        if b:
            b.m = jnp.max(b.mx, axis=1, keepdims=True)
        if prev:
            done.append(prev)
        if len(done) > lag:
            finish(done.pop(0))
        filler(n + 1)
        prev = b
    for b in done:
        finish(b)


def _weave(mxu, *others):
    for n, job in enumerate(mxu):
        out = job()
        todo = [other for vpu in others
                for other in vpu[n * len(vpu) // len(mxu):(n + 1) * len(vpu) // len(mxu)]]
        for t, other in enumerate(todo):
            r0 = t * (out.shape[0] // PAD) // len(todo) * PAD
            other(out[r0:r0 + PAD, 0:D])


def _skip(n):
    return [lambda tok: None] * n


def _zero(a):
    return jnp.minimum(pltpu.bitcast(a, i32)[0, 0] & 0xFFFF, 0)


def _after(tok, zero, *refs):
    if tok is None:
        return
    for ref in refs:
        if len(ref.shape) == 3:
            ref[zero + ref.shape[0] - 1, pl.ds(0, PAD), :] = tok.astype(ref.dtype)
        else:
            ref[_rows(zero + ref.shape[0] - PAD, PAD), pl.ds(0, D)] = tok.astype(ref.dtype)


def _kernel(x_hbm, ckv_hbm, wq_hbm, wk_hbm, wv_hbm, wo_hbm, wr_hbm, wg_hbm, wu_hbm, wd_hbm,
            c_hbm, wmod_hbm, out_hbm,
            x_s, ckv_s, wo_s, wr_s, wg_s, wu_s, wd_s, mod_s, w_s, k_s, q_s, v_s,
            in_sem, out_sem, fix_sem):
    copies = []

    def copy(hbm, vmem, *idx):
        if not idx and hbm.shape != vmem.shape:
            idx = (pl.ds(0, hbm.shape[0]),)
        if idx:
            hbm, vmem = hbm.at[idx], vmem.at[idx]
        copies.append(pltpu.make_async_copy(hbm, vmem, in_sem.at[len(copies)]))
        return copies[-1]

    def start(cps):
        for cp in cps:
            cp.start()

    def wait(cps):
        for cp in cps:
            cp.wait()

    stage4 = [copy(wo_hbm, wo_s), copy(wr_hbm, wr_s), copy(wg_hbm, wg_s), copy(wu_hbm, wu_s),
              copy(wd_hbm, wd_s)]

    def mod(j):
        return mod_s[:, pl.ds(j * M, M)]

    def qproj(hd, slot, i):
        h = jnp.concatenate([_ld(w_s, H + j, r0=i * T, n=T) for j in range(M // D)], axis=1)
        _st(q_s, slot, r0=i * T, val=_dot(h, _ld(w_s, hd, r0=0, n=M)) * QSCALE)

    def vproj(hd, slot, i):
        _st(v_s, slot, r0=i * T, val=_dot(_ld(ckv_s, r0=i * T, n=T), _ld(w_s, hd, r0=M + C, n=C)))

    def qv(hd, slot):
        return [functools.partial(f, hd, slot, i) for i in range(NB) for f in (qproj, vproj)]

    def phase1(ckv_raw, wq_raw, wk_raw, wv_raw, c_s, wmod_s):
        R0, R1 = 256, 1024
        first = [copy(wk_hbm, wk_raw, pl.ds(r0, D), pl.ds(0, G)) for r0 in range(0, C, D)]
        ckv0_cp = copy(ckv_hbm, ckv_raw, pl.ds(0, R0))
        ckv1_cp = copy(ckv_hbm, ckv_raw, pl.ds(R0, R1 - R0))
        stage1 = [copy(ckv_hbm, ckv_raw, pl.ds(R1, S - R1)),
                  copy(wk_hbm, wk_raw, pl.ds(0, C), pl.ds(G, G))]
        stage2 = [copy(wk_hbm, wk_raw, pl.ds(0, C), pl.ds(2 * G, 2 * G)),
                  copy(c_hbm, c_s), copy(wmod_hbm, wmod_s), copy(x_hbm, x_s)]
        stage3 = [copy(wq_hbm, wq_raw), copy(wv_hbm, wv_raw)]

        def per_head(raw, base, g):
            def job(r0, tok=None):
                _after(tok, zero, raw)
                w = raw[pl.ds(r0, 16), pl.ds(g * G, G), :].reshape(16, G * D)
                for j in range(G):
                    _st(w_s, g * G + j, r0=base + r0, val=w[:, j * D:(j + 1) * D])
            return [functools.partial(job, r0) for r0 in range(0, raw.shape[0] - 1, 16)]

        def kproj(heads, lo, hi):
            def job(hd, r0):
                if hd == 0:
                    ckv = ckv_raw[pl.ds(r0, 256), :]
                    _st(ckv_s, r0=r0, val=ckv)
                else:
                    ckv = _ld(ckv_s, r0=r0, n=256)
                k = _dot(ckv, _ld(w_s, hd, r0=M, n=C))
                _st(k_s, hd, r0=r0, val=k)
                return k
            return [functools.partial(job, hd, r0) for hd in heads for r0 in range(lo, hi, 256)]

        def modulation():
            cf = c_s[...].astype(f32)
            col = jnp.broadcast_to(_rb(cf * _sigmoid(cf)), (D, M)).T

            acc = {}

            def job(c0, r0, tok):
                _after(tok, zero, wmod_s)
                w = wmod_s[pl.ds(r0, D), pl.ds(c0, 2 * D)].astype(f32)
                w = w * jnp.concatenate([col[r0:r0 + D]] * 2, axis=1)
                w = jnp.sum(w.reshape(D // 8, 8, 2 * D), axis=0)
                acc[c0] = acc[c0] + w if r0 else w
                if r0 + D == M:
                    mod_s[:, pl.ds(c0, 2 * D)] = _rb(jnp.sum(acc[c0], axis=0, keepdims=True))
            return [functools.partial(job, c0, r0)
                    for c0 in range(0, 6 * M, 2 * D) for r0 in range(0, M, D)]

        def norm1(r0, tok):
            _after(tok, zero, x_s)
            xf = x_s[pl.ds(r0, 16), :].astype(f32)
            xc = xf - jnp.mean(xf, axis=1, keepdims=True)
            xn = xc * lax.rsqrt(jnp.mean(xc * xc, axis=1, keepdims=True) + EPS)
            h = xn * (1.0 + mod(1)) + mod(0)
            for j in range(M // D):
                _st(w_s, H + j, r0=r0, val=h[:, j * D:(j + 1) * D])

        start(first + [ckv0_cp, ckv1_cp])
        for n, cp in enumerate(first):
            cp.wait()
            if n == 0:
                zero = _zero(wk_raw[0, pl.ds(0, G), :])
            _weave(per_head(wk_raw, M, 0)[n * D // 16:(n + 1) * D // 16])
        start(stage1)
        ckv0_cp.wait()
        _weave(kproj(range(8), 0, R0))
        start(stage2)
        ckv1_cp.wait()
        _weave(kproj(range(8), R0, R1))
        wait(stage1)
        _weave(kproj(range(8), R1, S), per_head(wk_raw, M, 1))
        _weave(kproj(range(8, 13), 0, S))
        start(stage3)
        wait(stage2)
        _weave(kproj(range(13, 17), 0, S), per_head(wk_raw, M, 2) + _skip(14),
               _skip(6) + modulation())
        _weave(kproj(range(17, 24), 0, S), per_head(wk_raw, M, 3),
               [functools.partial(norm1, r0) for r0 in range(0, S, 16)] + _skip(12))
        start(stage4)
        wait(stage3)
        _weave(kproj(range(24, H), 0, S),
               [job for g in range(NG) for job in per_head(wq_raw, 0, g) + per_head(wv_raw, M + C, g)])
        _weave(qv(0, 0))

    V = pltpu.VMEM
    pl.run_scoped(phase1, V((S, C), bf16), V((M + 1, H, D), bf16), V((C + 1, H, D), bf16),
                  V((C + 1, H, D), bf16),
                  V((1, M), bf16), V((M + PAD, 6 * M), bf16))

    zero = _zero(x_s[pl.ds(0, 16), pl.ds(0, D)])

    def next_head(hd, slot):
        jobs = qv(hd, slot)
        cuts = [0, 1] + [1 + (27 * n) // NB for n in range(1, NB + 1)] + [len(jobs)]
        return lambda n: _weave(jobs[cuts[n]:cuts[n + 1]])

    def pair(p, _):
        _attention(q_s, k_s, v_s, zero, 2 * p + 1, 1, next_head(2 * p + 2, 0))
        _attention(q_s, k_s, v_s, zero, 2 * p + 2, 0, next_head(2 * p + 3, 1))

    _attention(q_s, k_s, v_s, zero, 0, 0, next_head(1, 1))
    lax.fori_loop(0, H // 2 - 1, pair, None)

    def phase3(y_s, key_s, top_s, xh_s, out_s, wgu_s):
        wait(stage4)
        sub = lax.broadcasted_iota(i32, (TOPK, D), 0)
        lane = lax.broadcasted_iota(i32, (TOPK, D), 1)

        def oproj(r0, n, slot):
            acc = {}

            def job(j, h0):
                ctx = jnp.concatenate([_ld(k_s, h0 + t, r0=r0, n=n) for t in range(CH)], axis=1)
                y = _dot(ctx, wo_s[pl.ds(h0 * D, CH * D), pl.ds(j * D, D)])
                acc[j] = acc[j] + y if h0 else y
                if h0 + CH == H:
                    y_s[slot][pl.ds(0, n), pl.ds(j * D, D)] = acc[j]
                return y
            return [functools.partial(job, j, h0) for j in range(M // D) for h0 in range(0, H, CH)]

        def out_copy(b):
            return pltpu.make_async_copy(out_s.at[_rows(b * RB, RB)], out_hbm.at[_rows(b * RB, RB)],
                                         out_sem.at[b])

        def epilogue(r0, slot, off, n, tok=None):
            _after(tok, zero, x_s, y_s[slot])
            rows = _rows(r0, n)
            ga, sb, cb, gb = mod(2), mod(3), _rb(1.0 + mod(4)), mod(5)
            x1 = _rb(x_s[rows, :].astype(f32) + _rb(ga * _rb(y_s[slot][pl.ds(off, n), :])))
            mean = jnp.mean(x1, axis=1, keepdims=True)
            xc = x1 - mean
            var = _rb(jnp.mean(xc * xc, axis=1, keepdims=True))
            inv = 1.0 / _rb(jnp.sqrt(_rb(var + EPS)))
            h2 = _rb(_rb(_rb(_rb(x1 - _rb(mean)) * inv) * cb) + sb)
            xh_s[rows, :] = pltpu.bitcast(x1, u32) | (pltpu.bitcast(h2, u32) >> 16)
            out_s[rows, :] = (x1 + _rb(gb * h2)).astype(bf16)
            wr = wr_s[...].astype(f32)
            prod = h2[:, 0:D] * wr[0:1]
            for j in range(1, M // D):
                prod = prod + h2[:, j * D:(j + 1) * D] * wr[j:j + 1]
            r = jnp.broadcast_to(_rb(jnp.sum(prod, axis=1, keepdims=True)), (n, D))
            bits = lax.bitcast_convert_type(r, i32)
            code = lax.shift_right_logical(bits, 16)
            code = jnp.where(bits < 0, 0xFFFF - code, code + 0x8000)
            code = jnp.where(r == 0.0, 0x8000, code)
            code = jnp.where(r != r, 0, code)
            key = code * S + (S - 1 + KEY0 - r0) - lax.broadcasted_iota(i32, (n, D), 0)
            key_s[pl.ds(off % T, n), :] = lax.bitcast_convert_type(key, f32)

        def select(tok=None):
            best = top_s[...]
            cols = [key_s[pl.ds(8 * t, 8), :] for t in range(T // 8)]
            flat = jnp.zeros((TOPK, D), f32)
            for t, col in enumerate(cols):
                flat = jnp.where(lane - sub == 8 * t, col, flat)
            new = None
            for cand in (flat, jnp.where(lane == sub, best, 0.0)):
                cand = jnp.broadcast_to(jnp.max(cand, axis=0, keepdims=True), (TOPK, D))
                above = sum((col > cand).astype(f32) for col in cols + [best])
                rank = jnp.sum(above, axis=0, keepdims=True)
                pick = jnp.where(rank == sub.astype(f32), cand, 0.0)
                new = pick if new is None else jnp.maximum(new, pick)
            top_s[...] = jnp.broadcast_to(jnp.max(new, axis=1, keepdims=True), (TOPK, D))

        def epilogues(r0, slot, rows=RB, n=16):
            jobs = []
            for off in range(0, rows, n):
                jobs.append(functools.partial(epilogue, r0 + off, slot, off, n))
                if (off + n) % T == 0:
                    jobs.append(select)
            return jobs

        def flip(t, src):
            def job(r0, tok):
                _after(tok, zero, src)
                wgu_s[t, :, pl.ds(r0, D)] = src[pl.ds(r0, D), :].T
            return [functools.partial(job, r0) for r0 in range(0, F - D, D)] + [
                functools.partial(job, F - D)]

        NR = S // RB
        top_s[...] = jnp.zeros(top_s.shape, f32)
        last = oproj((NR - 1) * RB, RB, 1)
        cuts = [0] * 4 + [len(last) * n // 15 for n in range(1, 16)]
        _attention(q_s, k_s, v_s, 0, H - 1, 1, lambda n: _weave(last[cuts[n]:cuts[n + 1]]), lag=0)

        flips = flip(0, wg_s) + flip(1, wu_s)
        for n, b in enumerate(range(NR - 2, 0, -1)):
            _weave(oproj(b * RB, RB, b % 2), epilogues((b + 1) * RB, (b + 1) % 2) + _skip(2),
                   flips[7 * n:7 * n + 7])
            out_copy(b + 1).start()
            if n == 4:
                wait([out_copy(b) for b in range(b + 2, NR)])
        _weave(oproj(T, T, 0), epilogues(RB, 1))
        out_copy(1).start()
        _weave(oproj(0, T, 1), epilogues(T, 0, T) + _skip(2))
        _weave(epilogues(0, 1, T, T))
        out_copy(0).start()

        top = lax.bitcast_convert_type(top_s[...], i32) - KEY0
        sel = S - 1 - (top & (S - 1))
        code = lax.shift_right_logical(top, 11)
        code = jnp.where(code >= 0x8000, code - 0x8000, 0xFFFF - code)
        r_sel = lax.bitcast_convert_type(code * 0x10000, f32)[:, 0:1]
        idx = [sel[j, 0] for j in range(TOPK)]

        both = jnp.concatenate([xh_s[pl.ds(t, 1), :] for t in idx], axis=0)
        hsel = pltpu.bitcast(both << 16, f32)
        xsel = pltpu.bitcast((both >> 16) << 16, f32)
        lhs = jnp.concatenate([hsel, hsel], axis=0).astype(bf16)
        gate = _rb(_dot(lhs, wgu_s[0]))
        act = _rb(gate * _sigmoid(gate)) * _rb(_dot(lhs, wgu_s[1]))
        y = _rb(_rb(_dot(act.astype(bf16), wd_s[...])[0:TOPK]) * _sigmoid(r_sel))
        fixed = xsel + _rb(mod(5) * _rb(hsel + y))

        wait([out_copy(b) for b in range(4)])
        tiles = [pl.multiple_of((t // 16) * 16, 16) for t in idx]
        row = lax.broadcasted_iota(i32, (16, M), 0)
        for j in range(TOPK):
            cur = out_s[pl.ds(tiles[j], 16), :].astype(f32)
            cur = jnp.where(row == idx[j] - tiles[j], fixed[j:j + 1], cur)
            out_s[pl.ds(tiles[j], 16), :] = cur.astype(bf16)

        def fix_copy(j):
            return pltpu.make_async_copy(out_s.at[pl.ds(tiles[j], 16)], out_hbm.at[pl.ds(tiles[j], 16)],
                                         fix_sem.at[j])

        fresh = []
        for j in range(TOPK):
            new = tiles[j] >= 0
            for k in range(j):
                new = jnp.logical_and(new, tiles[j] != tiles[k])
            fresh.append(new)
        for j in range(TOPK):
            pl.when(fresh[j])(fix_copy(j).start)
        for j in range(TOPK):
            pl.when(fresh[j])(fix_copy(j).wait)

    pl.run_scoped(phase3, [V((RB + PAD, M), f32)] * 2, V((T, D), f32), V((TOPK, D), f32),
                  V((S, M), u32), V((S, M), bf16), V((2, M, F), bf16))


@jax.jit
def pallas_adaLN_cond__compressed_kv_cla__moe_arch_mod__prompt_kernel(
    A_x: jax.Array,
    A_c_kv: jax.Array,
    A_w_q: jax.Array,
    A_w_uk: jax.Array,
    A_w_uv: jax.Array,
    A_w_o: jax.Array,
    B_x: jax.Array,
    B_w_r: jax.Array,
    B_w_gate: jax.Array,
    B_w_up: jax.Array,
    B_w_down: jax.Array,
    c: jax.Array,
    w_mod: jax.Array,
):
    del B_x
    V = pltpu.VMEM
    scratch = [
        V((S + PAD, M), bf16), V((S // 2, C), u32),
        V((H * D, M), bf16), V((M // D, D), bf16),
        V((F + PAD, M), bf16), V((F + PAD, M), bf16), V((F, M), bf16),
        V((1, 6 * M), f32),
        V((H + M // D, S // 2, D), u32),
        V((H, S // 2, D), u32),
        V((2, S // 2, D), u32), V((2, S // 2, D), u32),
        pltpu.SemaphoreType.DMA((19,)), pltpu.SemaphoreType.DMA((S // RB,)),
        pltpu.SemaphoreType.DMA((TOPK,)),
    ]
    out = pl.pallas_call(
        _kernel,
        in_specs=[pl.BlockSpec(memory_space=pltpu.HBM)] * 12,
        out_specs=pl.BlockSpec(memory_space=pltpu.HBM),
        out_shape=jax.ShapeDtypeStruct((S, M), bf16),
        scratch_shapes=scratch,
        compiler_params=pltpu.CompilerParams(vmem_limit_bytes=120 * 2 ** 20),
    )(A_x.reshape(S, M), A_c_kv.reshape(S, C), A_w_q, A_w_uk, A_w_uv, A_w_o.reshape(H * D, M),
      B_w_r.reshape(M // D, D), B_w_gate.T, B_w_up.T, B_w_down, c, w_mod)
    return out.reshape(A_x.shape)
```

```python
import functools

import jax
import jax.numpy as jnp
from jax import lax
import jax.experimental.pallas as pl
import jax.experimental.pallas.tpu as pltpu

S, M, C, D, H, F, TOPK = 2048, 640, 512, 128, 32, 1728, 8
G = 8
NG = H // G
T = 128
NB = S // T
CH = 4
RB = 256
PAD = 16
EPS = 1e-5
KEY0 = 0x00800000
QSCALE = D ** -0.5 * 1.4426950408889634
NT = (((1,), (1,)), ((), ()))

f32, bf16, u32, i32 = jnp.float32, jnp.bfloat16, jnp.uint32, jnp.int32


def _rb(a):
    return a.astype(bf16).astype(f32)


def _sigmoid(a):
    return _rb(1.0 / _rb(1.0 + _rb(jnp.exp(-a))))


def _rows(r0, n):
    if isinstance(r0, int):
        return pl.ds(r0, n)
    return pl.ds(pl.multiple_of(r0, n & -n), n)


def _ld(ref, *idx, r0, n):
    return pltpu.bitcast(ref[(*idx, _rows(r0 // 2, n // 2), slice(None))], bf16)


def _st(ref, *idx, r0, val):
    ref[(*idx, _rows(r0 // 2, val.shape[0] // 2), slice(None))] = pltpu.bitcast(
        val.astype(bf16), u32)


def _dot(a, b):
    return jnp.dot(a, b, preferred_element_type=f32)


def _dot_nt(a, b):
    return lax.dot_general(a, b, NT, preferred_element_type=f32)


class _Blk:
    def __init__(self, i):
        self.i, self.s, self.mx, self.m, self.l, self.acc = i, {}, None, None, None, None


def _attention(q_s, k_s, v_s, zero, hd, slot, filler, lag=3):
    tri = (lax.broadcasted_iota(i32, (T, T), 1) <= lax.broadcasted_iota(i32, (T, T), 0))

    def chunks(b):
        n = b.i + 1 if b else 0
        return [(a, min(a + CH, n)) for a in range(0, n, CH)]

    def scores(b, a, e):
        return _dot_nt(_ld(q_s, slot, r0=b.i * T, n=T), _ld(k_s, hd, r0=a * T, n=(e - a) * T))

    def keep(b, a, e, s):
        for t in range(a, e):
            x = s[:, (t - a) * T:(t - a + 1) * T]
            if t == b.i:
                x = jnp.where(tri, x, -1e9)
            b.mx = x if b.mx is None else jnp.maximum(b.mx, x)
            b.s[t] = x

    def context(b, a, e):
        ps = sums = [jnp.exp2(b.s[t] - b.m) for t in range(a, e)]
        while len(sums) > 1:
            sums = [functools.reduce(jnp.add, sums[t:t + 2]) for t in range(0, len(sums), 2)]
        b.l = sums[0] if b.l is None else b.l + sums[0]
        p = (jnp.concatenate(ps, axis=1) if len(ps) > 1 else ps[0]).astype(bf16)
        o = _dot(p, _ld(v_s, slot, r0=a * T, n=(e - a) * T))
        b.acc = o if b.acc is None else b.acc + o

    def finish(b):
        l = jnp.sum(b.l, axis=1, keepdims=True)
        r = pltpu.reciprocal(l, approx=True)
        r = r * (2.0 - l * r)
        _st(k_s, hd + zero, r0=b.i * T, val=b.acc * r)

    filler(0)
    prev, done = None, []
    for n, i in enumerate(list(range(NB - 1, -1, -1)) + [None]):
        b = _Blk(i) if i is not None else None
        ca, cb = chunks(b), chunks(prev)
        for c in range(max(len(ca), len(cb))):
            s = scores(b, *ca[c]) if c < len(ca) else None
            if c < len(cb):
                context(prev, *cb[c])
            if s is not None:
                keep(b, *ca[c], s)
        if b:
            b.m = jnp.max(b.mx, axis=1, keepdims=True)
        if prev:
            done.append(prev)
        if len(done) > lag:
            finish(done.pop(0))
        filler(n + 1)
        prev = b
    for b in done:
        finish(b)


def _weave(mxu, *others):
    for n, job in enumerate(mxu):
        out = job()
        todo = [other for vpu in others
                for other in vpu[n * len(vpu) // len(mxu):(n + 1) * len(vpu) // len(mxu)]]
        for t, other in enumerate(todo):
            r0 = t * (out.shape[0] // PAD) // len(todo) * PAD
            other(out[r0:r0 + PAD, 0:D])


def _skip(n):
    return [lambda tok: None] * n


def _zero(a):
    return jnp.minimum(pltpu.bitcast(a, i32)[0, 0] & 0xFFFF, 0)


def _after(tok, zero, *refs):
    if tok is None:
        return
    for ref in refs:
        if len(ref.shape) == 3:
            ref[zero + ref.shape[0] - 1, pl.ds(0, PAD), :] = tok.astype(ref.dtype)
        else:
            ref[_rows(zero + ref.shape[0] - PAD, PAD), pl.ds(0, D)] = tok.astype(ref.dtype)


def _kernel(x_hbm, ckv_hbm, wq_hbm, wk_hbm, wv_hbm, wo_hbm, wr_hbm, wg_hbm, wu_hbm, wd_hbm,
            c_hbm, wmod_hbm, out_hbm,
            k_s, w_s, q_s, v_s, ckv_s, wo_s, x_s, wg_s, wu_s, wd_s, mod_s, wr_s,
            in_sem, out_sem, fix_sem):
    copies = []

    def copy(hbm, vmem, *idx):
        if not idx and hbm.shape != vmem.shape:
            idx = (pl.ds(0, hbm.shape[0]),)
        if idx:
            hbm, vmem = hbm.at[idx], vmem.at[idx]
        copies.append(pltpu.make_async_copy(hbm, vmem, in_sem.at[len(copies)]))
        return copies[-1]

    def start(cps):
        for cp in cps:
            cp.start()

    def wait(cps):
        for cp in cps:
            cp.wait()

    stage4 = [copy(wo_hbm, wo_s), copy(wr_hbm, wr_s), copy(wg_hbm, wg_s), copy(wu_hbm, wu_s),
              copy(wd_hbm, wd_s)]

    def mod(j):
        return mod_s[:, pl.ds(j * M, M)]

    def qproj(hd, slot, i):
        h = jnp.concatenate([_ld(w_s, H + j, r0=i * T, n=T) for j in range(M // D)], axis=1)
        _st(q_s, slot, r0=i * T, val=_dot(h, _ld(w_s, hd, r0=0, n=M)) * QSCALE)

    def vproj(hd, slot, i):
        _st(v_s, slot, r0=i * T, val=_dot(_ld(ckv_s, r0=i * T, n=T), _ld(w_s, hd, r0=M + C, n=C)))

    def qv(hd, slot):
        return [functools.partial(f, hd, slot, i) for i in range(NB) for f in (qproj, vproj)]

    def phase1(ckv_raw, wq_raw, wk_raw, wv_raw, c_s, wmod_s):
        R0, R1 = 256, 1024
        first = [copy(wk_hbm, wk_raw, pl.ds(r0, D), pl.ds(0, G)) for r0 in range(0, C, D)]
        ckv0_cp = copy(ckv_hbm, ckv_raw, pl.ds(0, R0))
        ckv1_cp = copy(ckv_hbm, ckv_raw, pl.ds(R0, R1 - R0))
        stage1 = [copy(ckv_hbm, ckv_raw, pl.ds(R1, S - R1)),
                  copy(wk_hbm, wk_raw, pl.ds(0, C), pl.ds(G, G))]
        stage2 = [copy(wk_hbm, wk_raw, pl.ds(0, C), pl.ds(2 * G, 2 * G)),
                  copy(c_hbm, c_s), copy(wmod_hbm, wmod_s), copy(x_hbm, x_s)]
        stage3 = [copy(wq_hbm, wq_raw), copy(wv_hbm, wv_raw)]

        def per_head(raw, base, g):
            def job(r0, tok=None):
                _after(tok, zero, raw)
                w = raw[pl.ds(r0, 16), pl.ds(g * G, G), :].reshape(16, G * D)
                for j in range(G):
                    _st(w_s, g * G + j, r0=base + r0, val=w[:, j * D:(j + 1) * D])
            return [functools.partial(job, r0) for r0 in range(0, raw.shape[0] - 1, 16)]

        def kproj(heads, lo, hi):
            def job(hd, r0):
                if hd == 0:
                    ckv = ckv_raw[pl.ds(r0, 256), :]
                    _st(ckv_s, r0=r0, val=ckv)
                else:
                    ckv = _ld(ckv_s, r0=r0, n=256)
                k = _dot(ckv, _ld(w_s, hd, r0=M, n=C))
                _st(k_s, hd, r0=r0, val=k)
                return k
            return [functools.partial(job, hd, r0) for hd in heads for r0 in range(lo, hi, 256)]

        def modulation():
            cf = c_s[...].astype(f32)
            col = jnp.broadcast_to(_rb(cf * _sigmoid(cf)), (D, M)).T

            acc = {}

            def job(c0, r0, tok):
                _after(tok, zero, wmod_s)
                w = wmod_s[pl.ds(r0, D), pl.ds(c0, 2 * D)].astype(f32)
                w = w * jnp.concatenate([col[r0:r0 + D]] * 2, axis=1)
                w = jnp.sum(w.reshape(D // 8, 8, 2 * D), axis=0)
                acc[c0] = acc[c0] + w if r0 else w
                if r0 + D == M:
                    mod_s[:, pl.ds(c0, 2 * D)] = _rb(jnp.sum(acc[c0], axis=0, keepdims=True))
            return [functools.partial(job, c0, r0)
                    for c0 in range(0, 6 * M, 2 * D) for r0 in range(0, M, D)]

        def norm1(r0, tok):
            _after(tok, zero, x_s)
            xf = x_s[pl.ds(r0, 16), :].astype(f32)
            xc = xf - jnp.mean(xf, axis=1, keepdims=True)
            xn = xc * lax.rsqrt(jnp.mean(xc * xc, axis=1, keepdims=True) + EPS)
            h = xn * (1.0 + mod(1)) + mod(0)
            for j in range(M // D):
                _st(w_s, H + j, r0=r0, val=h[:, j * D:(j + 1) * D])

        start(first + [ckv0_cp])
        for n, cp in enumerate(first):
            if n == 2:
                ckv1_cp.start()
            cp.wait()
            if n == 0:
                zero = _zero(wk_raw[0, pl.ds(0, G), :])
            _weave(per_head(wk_raw, M, 0)[n * D // 16:(n + 1) * D // 16])
        start(stage1)
        ckv0_cp.wait()
        _weave(kproj(range(8), 0, R0))
        start(stage2)
        ckv1_cp.wait()
        _weave(kproj(range(8), R0, R1))
        wait(stage1)
        _weave(kproj(range(8), R1, S), per_head(wk_raw, M, 1))
        _weave(kproj(range(8, 13), 0, S))
        start(stage3)
        wait(stage2)
        _weave(kproj(range(13, 17), 0, S), per_head(wk_raw, M, 2) + _skip(14),
               _skip(6) + modulation())
        _weave(kproj(range(17, 24), 0, S), per_head(wk_raw, M, 3),
               [functools.partial(norm1, r0) for r0 in range(0, S, 16)] + _skip(12))
        start(stage4)
        wait(stage3)
        _weave(kproj(range(24, H), 0, S),
               [job for g in range(NG) for job in per_head(wq_raw, 0, g) + per_head(wv_raw, M + C, g)])
        _weave(qv(0, 0))

    V = pltpu.VMEM
    pl.run_scoped(phase1, V((S, C), bf16), V((M + 1, H, D), bf16), V((C + 1, H, D), bf16),
                  V((C + 1, H, D), bf16),
                  V((1, M), bf16), V((M + PAD, 6 * M), bf16))

    zero = _zero(x_s[pl.ds(0, 16), pl.ds(0, D)])

    def next_head(hd, slot):
        jobs = qv(hd, slot)
        cuts = [0, 1] + [1 + (27 * n) // NB for n in range(1, NB + 1)] + [len(jobs)]
        return lambda n: _weave(jobs[cuts[n]:cuts[n + 1]])

    def pair(p, _):
        _attention(q_s, k_s, v_s, zero, 2 * p + 1, 1, next_head(2 * p + 2, 0))
        _attention(q_s, k_s, v_s, zero, 2 * p + 2, 0, next_head(2 * p + 3, 1))

    _attention(q_s, k_s, v_s, zero, 0, 0, next_head(1, 1))
    lax.fori_loop(0, H // 2 - 1, pair, None)

    def phase3(y_s, key_s, top_s, xh_s, out_s, wgu_s):
        wait(stage4)
        sub = lax.broadcasted_iota(i32, (TOPK, D), 0)
        lane = lax.broadcasted_iota(i32, (TOPK, D), 1)

        def oproj(r0, n, slot):
            acc = {}

            def job(j, h0):
                ctx = jnp.concatenate([_ld(k_s, h0 + t, r0=r0, n=n) for t in range(CH)], axis=1)
                y = _dot(ctx, wo_s[pl.ds(h0 * D, CH * D), pl.ds(j * D, D)])
                acc[j] = acc[j] + y if h0 else y
                if h0 + CH == H:
                    y_s[slot][pl.ds(0, n), pl.ds(j * D, D)] = acc[j]
                return y
            return [functools.partial(job, j, h0) for j in range(M // D) for h0 in range(0, H, CH)]

        def out_copy(b):
            return pltpu.make_async_copy(out_s.at[_rows(b * RB, RB)], out_hbm.at[_rows(b * RB, RB)],
                                         out_sem.at[b])

        def epilogue(r0, slot, off, n, tok=None):
            _after(tok, zero, x_s, y_s[slot])
            rows = _rows(r0, n)
            ga, sb, cb, gb = mod(2), mod(3), _rb(1.0 + mod(4)), mod(5)
            x1 = _rb(x_s[rows, :].astype(f32) + _rb(ga * _rb(y_s[slot][pl.ds(off, n), :])))
            mean = jnp.mean(x1, axis=1, keepdims=True)
            xc = x1 - mean
            var = _rb(jnp.mean(xc * xc, axis=1, keepdims=True))
            inv = 1.0 / _rb(jnp.sqrt(_rb(var + EPS)))
            h2 = _rb(_rb(_rb(_rb(x1 - _rb(mean)) * inv) * cb) + sb)
            xh_s[rows, :] = pltpu.bitcast(x1, u32) | (pltpu.bitcast(h2, u32) >> 16)
            out_s[rows, :] = (x1 + _rb(gb * h2)).astype(bf16)
            wr = wr_s[...].astype(f32)
            prod = h2[:, 0:D] * wr[0:1]
            for j in range(1, M // D):
                prod = prod + h2[:, j * D:(j + 1) * D] * wr[j:j + 1]
            r = jnp.broadcast_to(_rb(jnp.sum(prod, axis=1, keepdims=True)), (n, D))
            bits = lax.bitcast_convert_type(r, i32)
            code = lax.shift_right_logical(bits, 16)
            code = jnp.where(bits < 0, 0xFFFF - code, code + 0x8000)
            code = jnp.where(r == 0.0, 0x8000, code)
            code = jnp.where(r != r, 0, code)
            key = code * S + (S - 1 + KEY0 - r0) - lax.broadcasted_iota(i32, (n, D), 0)
            key_s[pl.ds(off % T, n), :] = lax.bitcast_convert_type(key, f32)

        def select(tok=None):
            best = top_s[...]
            cols = [key_s[pl.ds(8 * t, 8), :] for t in range(T // 8)]
            flat = jnp.zeros((TOPK, D), f32)
            for t, col in enumerate(cols):
                flat = jnp.where(lane - sub == 8 * t, col, flat)
            new = None
            for cand in (flat, jnp.where(lane == sub, best, 0.0)):
                cand = jnp.broadcast_to(jnp.max(cand, axis=0, keepdims=True), (TOPK, D))
                above = sum((col > cand).astype(f32) for col in cols + [best])
                rank = jnp.sum(above, axis=0, keepdims=True)
                pick = jnp.where(rank == sub.astype(f32), cand, 0.0)
                new = pick if new is None else jnp.maximum(new, pick)
            top_s[...] = jnp.broadcast_to(jnp.max(new, axis=1, keepdims=True), (TOPK, D))

        def epilogues(r0, slot, rows=RB, n=16):
            jobs = []
            for off in range(0, rows, n):
                jobs.append(functools.partial(epilogue, r0 + off, slot, off, n))
                if (off + n) % T == 0:
                    jobs.append(select)
            return jobs

        def flip(t, src):
            def job(r0, tok):
                _after(tok, zero, src)
                wgu_s[t, :, pl.ds(r0, D)] = src[pl.ds(r0, D), :].T
            return [functools.partial(job, r0) for r0 in range(0, F - D, D)] + [
                functools.partial(job, F - D)]

        NR = S // RB
        top_s[...] = jnp.zeros(top_s.shape, f32)
        last = oproj((NR - 1) * RB, RB, 1)
        cuts = [0] * 4 + [len(last) * n // 15 for n in range(1, 16)]
        _attention(q_s, k_s, v_s, 0, H - 1, 1, lambda n: _weave(last[cuts[n]:cuts[n + 1]]), lag=0)

        flips = flip(0, wg_s) + flip(1, wu_s)
        for n, b in enumerate(range(NR - 2, 0, -1)):
            _weave(oproj(b * RB, RB, b % 2), epilogues((b + 1) * RB, (b + 1) % 2) + _skip(2),
                   flips[7 * n:7 * n + 7])
            out_copy(b + 1).start()
            if n == 4:
                wait([out_copy(b) for b in range(b + 2, NR)])
        _weave(oproj(T, T, 0), epilogues(RB, 1))
        out_copy(1).start()
        _weave(oproj(0, T, 1), epilogues(T, 0, T) + _skip(2))
        _weave(epilogues(0, 1, T, T))
        out_copy(0).start()

        top = lax.bitcast_convert_type(top_s[...], i32) - KEY0
        sel = S - 1 - (top & (S - 1))
        code = lax.shift_right_logical(top, 11)
        code = jnp.where(code >= 0x8000, code - 0x8000, 0xFFFF - code)
        r_sel = lax.bitcast_convert_type(code * 0x10000, f32)[:, 0:1]
        idx = [sel[j, 0] for j in range(TOPK)]

        both = jnp.concatenate([xh_s[pl.ds(t, 1), :] for t in idx], axis=0)
        hsel = pltpu.bitcast(both << 16, f32)
        xsel = pltpu.bitcast((both >> 16) << 16, f32)
        lhs = jnp.concatenate([hsel, hsel], axis=0).astype(bf16)
        gate = _rb(_dot(lhs, wgu_s[0]))
        act = _rb(gate * _sigmoid(gate)) * _rb(_dot(lhs, wgu_s[1]))
        y = _rb(_rb(_dot(act.astype(bf16), wd_s[...])[0:TOPK]) * _sigmoid(r_sel))
        fixed = xsel + _rb(mod(5) * _rb(hsel + y))

        wait([out_copy(b) for b in range(4)])
        tiles = [pl.multiple_of((t // 16) * 16, 16) for t in idx]
        row = lax.broadcasted_iota(i32, (16, M), 0)
        for j in range(TOPK):
            cur = out_s[pl.ds(tiles[j], 16), :].astype(f32)
            cur = jnp.where(row == idx[j] - tiles[j], fixed[j:j + 1], cur)
            out_s[pl.ds(tiles[j], 16), :] = cur.astype(bf16)

        def fix_copy(j):
            return pltpu.make_async_copy(out_s.at[pl.ds(tiles[j], 16)], out_hbm.at[pl.ds(tiles[j], 16)],
                                         fix_sem.at[j])

        fresh = []
        for j in range(TOPK):
            new = tiles[j] >= 0
            for k in range(j):
                new = jnp.logical_and(new, tiles[j] != tiles[k])
            fresh.append(new)
        for j in range(TOPK):
            pl.when(fresh[j])(fix_copy(j).start)
        for j in range(TOPK):
            pl.when(fresh[j])(fix_copy(j).wait)

    pl.run_scoped(phase3, [V((RB + PAD, M), f32)] * 2, V((T, D), f32), V((TOPK, D), f32),
                  V((S, M), u32), V((S, M), bf16), V((2, M, F), bf16))


@jax.jit
def pallas_adaLN_cond__compressed_kv_cla__moe_arch_mod__prompt_kernel(
    A_x: jax.Array,
    A_c_kv: jax.Array,
    A_w_q: jax.Array,
    A_w_uk: jax.Array,
    A_w_uv: jax.Array,
    A_w_o: jax.Array,
    B_x: jax.Array,
    B_w_r: jax.Array,
    B_w_gate: jax.Array,
    B_w_up: jax.Array,
    B_w_down: jax.Array,
    c: jax.Array,
    w_mod: jax.Array,
):
    del B_x
    V = pltpu.VMEM
    scratch = [
        V((H, S // 2, D), u32),
        V((H + M // D, S // 2, D), u32),
        V((2, S // 2, D), u32), V((2, S // 2, D), u32), V((S // 2, C), u32),
        V((H * D, M), bf16), V((S + PAD, M), bf16),
        V((F + PAD, M), bf16), V((F + PAD, M), bf16), V((F, M), bf16),
        V((1, 6 * M), f32), V((M // D, D), bf16),
        pltpu.SemaphoreType.DMA((19,)), pltpu.SemaphoreType.DMA((S // RB,)),
        pltpu.SemaphoreType.DMA((TOPK,)),
    ]
    out = pl.pallas_call(
        _kernel,
        in_specs=[pl.BlockSpec(memory_space=pltpu.HBM)] * 12,
        out_specs=pl.BlockSpec(memory_space=pltpu.HBM),
        out_shape=jax.ShapeDtypeStruct((S, M), bf16),
        scratch_shapes=scratch,
        compiler_params=pltpu.CompilerParams(vmem_limit_bytes=120 * 2 ** 20),
    )(A_x.reshape(S, M), A_c_kv.reshape(S, C), A_w_q, A_w_uk, A_w_uv, A_w_o.reshape(H * D, M),
      B_w_r.reshape(M // D, D), B_w_gate.T, B_w_up.T, B_w_down, c, w_mod)
    return out.reshape(A_x.shape)
```

```python
import functools

import jax
import jax.numpy as jnp
from jax import lax
import jax.experimental.pallas as pl
import jax.experimental.pallas.tpu as pltpu

S, M, C, D, H, F, TOPK = 2048, 640, 512, 128, 32, 1728, 8
G = 8
NG = H // G
T = 128
NB = S // T
CH = 4
RB = 256
PAD = 16
EPS = 1e-5
KEY0 = 0x00800000
QSCALE = D ** -0.5 * 1.4426950408889634
NT = (((1,), (1,)), ((), ()))

f32, bf16, u32, i32 = jnp.float32, jnp.bfloat16, jnp.uint32, jnp.int32


def _rb(a):
    return a.astype(bf16).astype(f32)


def _sigmoid(a):
    return _rb(1.0 / _rb(1.0 + _rb(jnp.exp(-a))))


def _rows(r0, n):
    if isinstance(r0, int):
        return pl.ds(r0, n)
    return pl.ds(pl.multiple_of(r0, n & -n), n)


def _ld(ref, *idx, r0, n):
    return pltpu.bitcast(ref[(*idx, _rows(r0 // 2, n // 2), slice(None))], bf16)


def _st(ref, *idx, r0, val):
    ref[(*idx, _rows(r0 // 2, val.shape[0] // 2), slice(None))] = pltpu.bitcast(
        val.astype(bf16), u32)


def _dot(a, b):
    return jnp.dot(a, b, preferred_element_type=f32)


def _dot_nt(a, b):
    return lax.dot_general(a, b, NT, preferred_element_type=f32)


class _Blk:
    def __init__(self, i):
        self.i, self.s, self.mx, self.m, self.l, self.acc = i, {}, None, None, None, None


def _attention(q_s, k_s, v_s, zero, hd, slot, filler, lag=3):
    tri = (lax.broadcasted_iota(i32, (T, T), 1) <= lax.broadcasted_iota(i32, (T, T), 0))

    def chunks(b):
        n = b.i + 1 if b else 0
        return [(a, min(a + CH, n)) for a in range(0, n, CH)]

    def scores(b, a, e):
        return _dot_nt(_ld(q_s, slot, r0=b.i * T, n=T), _ld(k_s, hd, r0=a * T, n=(e - a) * T))

    def keep(b, a, e, s):
        for t in range(a, e):
            x = s[:, (t - a) * T:(t - a + 1) * T]
            if t == b.i:
                x = jnp.where(tri, x, -1e9)
            b.mx = x if b.mx is None else jnp.maximum(b.mx, x)
            b.s[t] = x

    def context(b, a, e):
        ps = sums = [jnp.exp2(b.s[t] - b.m) for t in range(a, e)]
        while len(sums) > 1:
            sums = [functools.reduce(jnp.add, sums[t:t + 2]) for t in range(0, len(sums), 2)]
        b.l = sums[0] if b.l is None else b.l + sums[0]
        p = (jnp.concatenate(ps, axis=1) if len(ps) > 1 else ps[0]).astype(bf16)
        o = _dot(p, _ld(v_s, slot, r0=a * T, n=(e - a) * T))
        b.acc = o if b.acc is None else b.acc + o

    def finish(b):
        l = jnp.sum(b.l, axis=1, keepdims=True)
        r = pltpu.reciprocal(l, approx=True)
        r = r * (2.0 - l * r)
        _st(k_s, hd + zero, r0=b.i * T, val=b.acc * r)

    filler(0)
    prev, done = None, []
    for n, i in enumerate(list(range(NB - 1, -1, -1)) + [None]):
        b = _Blk(i) if i is not None else None
        ca, cb = chunks(b), chunks(prev)
        for c in range(max(len(ca), len(cb))):
            s = scores(b, *ca[c]) if c < len(ca) else None
            if c < len(cb):
                context(prev, *cb[c])
            if s is not None:
                keep(b, *ca[c], s)
        if b:
            b.m = jnp.max(b.mx, axis=1, keepdims=True)
        if prev:
            done.append(prev)
        if len(done) > lag:
            finish(done.pop(0))
        filler(n + 1)
        prev = b
    for b in done:
        finish(b)


def _weave(mxu, *others):
    for n, job in enumerate(mxu):
        out = job()
        todo = [other for vpu in others
                for other in vpu[n * len(vpu) // len(mxu):(n + 1) * len(vpu) // len(mxu)]]
        for t, other in enumerate(todo):
            r0 = t * (out.shape[0] // PAD) // len(todo) * PAD
            other(out[r0:r0 + PAD, 0:D])


def _skip(n):
    return [lambda tok: None] * n


def _zero(a):
    return jnp.minimum(pltpu.bitcast(a, i32)[0, 0] & 0xFFFF, 0)


def _after(tok, zero, *refs):
    if tok is None:
        return
    for ref in refs:
        if len(ref.shape) == 3:
            ref[zero + ref.shape[0] - 1, pl.ds(0, G), :] = tok[0:G].astype(ref.dtype)
        else:
            ref[_rows(zero + ref.shape[0] - PAD, PAD), pl.ds(0, D)] = tok.astype(ref.dtype)


def _kernel(x_hbm, ckv_hbm, wq_hbm, wk_hbm, wv_hbm, wo_hbm, wr_hbm, wg_hbm, wu_hbm, wd_hbm,
            c_hbm, wmod_hbm, out_hbm,
            k_s, w_s, q_s, v_s, ckv_s, wo_s, wo_raw, x_s, wg_s, wu_s, wd_s, mod_s, wr_s,
            in_sem, out_sem, fix_sem):
    copies = []

    def copy(hbm, vmem, rows=None):
        if rows is not None:
            hbm, vmem = hbm.at[rows], vmem.at[rows]
        elif hbm.shape != vmem.shape:
            vmem = vmem.at[pl.ds(0, hbm.shape[0])]
        copies.append(pltpu.make_async_copy(hbm, vmem, in_sem.at[len(copies)]))
        return copies[-1]

    def start(cps):
        for cp in cps:
            cp.start()

    def wait(cps):
        for cp in cps:
            cp.wait()

    stage4 = [copy(wo_hbm, wo_raw), copy(wr_hbm, wr_s), copy(wg_hbm, wg_s), copy(wu_hbm, wu_s),
              copy(wd_hbm, wd_s)]

    def mod(j):
        return mod_s[:, pl.ds(j * M, M)]

    def qproj(hd, slot, i):
        h = jnp.concatenate([_ld(w_s, H + j, r0=i * T, n=T) for j in range(M // D)], axis=1)
        _st(q_s, slot, r0=i * T, val=_dot(h, _ld(w_s, hd, r0=0, n=M)) * QSCALE)

    def vproj(hd, slot, i):
        _st(v_s, slot, r0=i * T, val=_dot(_ld(ckv_s, r0=i * T, n=T), _ld(w_s, hd, r0=M + C, n=C)))

    def qv(hd, slot):
        return [functools.partial(f, hd, slot, i) for i in range(NB) for f in (qproj, vproj)]

    def phase1(ckv_raw, wq_raw, wv_raw, wk0, wk1, wk2, wmod_s, c_s):
        R0, R1 = 256, 1024
        first = [copy(wk_hbm.at[:, pl.ds(0, G)], wk0, pl.ds(r0, D)) for r0 in range(0, C, D)]
        ckv0_cp = copy(ckv_hbm, ckv_raw, pl.ds(0, R0))
        ckv1_cp = copy(ckv_hbm, ckv_raw, pl.ds(R0, R1 - R0))
        stage1 = [copy(ckv_hbm, ckv_raw, pl.ds(R1, S - R1)),
                  copy(wk_hbm.at[:, pl.ds(G, G)], wk1)]
        stage2 = [copy(wk_hbm.at[:, pl.ds(2 * G, 2 * G)], wk2),
                  copy(c_hbm, c_s), copy(wmod_hbm, wmod_s), copy(x_hbm, x_s)]
        stage3 = [copy(wq_hbm, wq_raw), copy(wv_hbm, wv_raw)]

        def per_head(raw, base, g):
            def job(r0, tok=None):
                _after(tok, zero, raw)
                w = raw[pl.ds(r0, 16), pl.ds(g * G % raw.shape[1], G), :].reshape(16, G * D)
                for j in range(G):
                    _st(w_s, g * G + j, r0=base + r0, val=w[:, j * D:(j + 1) * D])
            return [functools.partial(job, r0) for r0 in range(0, raw.shape[0] - 1, 16)]

        def kproj(heads, lo, hi):
            def job(hd, r0):
                if hd == 0:
                    ckv = ckv_raw[pl.ds(r0, 256), :]
                    _st(ckv_s, r0=r0, val=ckv)
                else:
                    ckv = _ld(ckv_s, r0=r0, n=256)
                k = _dot(ckv, _ld(w_s, hd, r0=M, n=C))
                _st(k_s, hd, r0=r0, val=k)
                return k
            return [functools.partial(job, hd, r0) for hd in heads for r0 in range(lo, hi, 256)]

        def modulation():
            cf = c_s[...].astype(f32)
            col = jnp.broadcast_to(_rb(cf * _sigmoid(cf)), (D, M)).T

            acc = {}

            def job(c0, r0, tok):
                _after(tok, zero, wmod_s)
                w = wmod_s[pl.ds(r0, D), pl.ds(c0, 2 * D)].astype(f32)
                w = w * jnp.concatenate([col[r0:r0 + D]] * 2, axis=1)
                w = jnp.sum(w.reshape(D // 8, 8, 2 * D), axis=0)
                acc[c0] = acc[c0] + w if r0 else w
                if r0 + D == M:
                    mod_s[:, pl.ds(c0, 2 * D)] = _rb(jnp.sum(acc[c0], axis=0, keepdims=True))
            return [functools.partial(job, c0, r0)
                    for c0 in range(0, 6 * M, 2 * D) for r0 in range(0, M, D)]

        def norm1(r0, tok):
            _after(tok, zero, x_s)
            xf = x_s[pl.ds(r0, 16), :].astype(f32)
            xc = xf - jnp.mean(xf, axis=1, keepdims=True)
            xn = xc * lax.rsqrt(jnp.mean(xc * xc, axis=1, keepdims=True) + EPS)
            h = xn * (1.0 + mod(1)) + mod(0)
            for j in range(M // D):
                _st(w_s, H + j, r0=r0, val=h[:, j * D:(j + 1) * D])

        start(first + [ckv0_cp])
        for n, cp in enumerate(first):
            if n == 2:
                ckv1_cp.start()
            cp.wait()
            if n == 0:
                zero = _zero(wk0[0])
            _weave(per_head(wk0, M, 0)[n * D // 16:(n + 1) * D // 16])
        start(stage1)
        ckv0_cp.wait()
        _weave(kproj(range(8), 0, R0))
        start(stage2)
        ckv1_cp.wait()
        _weave(kproj(range(8), R0, R1))
        wait(stage1)
        _weave(kproj(range(8), R1, S), per_head(wk1, M, 1))
        _weave(kproj(range(8, 13), 0, S))
        start(stage3)
        wait(stage2)
        _weave(kproj(range(13, 17), 0, S), per_head(wk2, M, 2) + _skip(14),
               _skip(6) + modulation())
        _weave(kproj(range(17, 24), 0, S), per_head(wk2, M, 3),
               [functools.partial(norm1, r0) for r0 in range(0, S, 16)] + _skip(12))
        start(stage4)
        wait(stage3)
        _weave(kproj(range(24, H), 0, S),
               [job for g in range(NG) for job in per_head(wq_raw, 0, g) + per_head(wv_raw, M + C, g)])
        _weave(qv(0, 0))

    V = pltpu.VMEM
    pl.run_scoped(phase1, V((S, C), bf16), V((M + 1, H, D), bf16), V((C + 1, H, D), bf16),
                  V((C, G, D), bf16), V((C + 1, G, D), bf16), V((C + 1, 2 * G, D), bf16),
                  V((M + PAD, 6 * M), bf16), V((1, M), bf16))

    zero = _zero(x_s[pl.ds(0, 16), pl.ds(0, D)])

    def next_head(hd, slot):
        jobs = qv(hd, slot)
        cuts = [0, 1] + [1 + (27 * n) // NB for n in range(1, NB + 1)] + [len(jobs)]
        return lambda n: _weave(jobs[cuts[n]:cuts[n + 1]])

    def pair(p, _):
        _attention(q_s, k_s, v_s, zero, 2 * p + 1, 1, next_head(2 * p + 2, 0))
        _attention(q_s, k_s, v_s, zero, 2 * p + 2, 0, next_head(2 * p + 3, 1))

    _attention(q_s, k_s, v_s, zero, 0, 0, next_head(1, 1))
    lax.fori_loop(0, H // 2 - 1, pair, None)

    def phase3(xh_s, out_s, wgu_s, key_s, y_s, top_s):
        wait(stage4)
        sub = lax.broadcasted_iota(i32, (TOPK, D), 0)
        lane = lax.broadcasted_iota(i32, (TOPK, D), 1)

        def oproj(r0, n, slot, first=False):
            acc = {}

            def job(j, h0):
                ctx = jnp.concatenate([_ld(k_s, h0 + t, r0=r0, n=n) for t in range(CH)], axis=1)
                if first:
                    w = wo_raw[pl.ds(h0 * D, CH * D), pl.ds(j * D, D)]
                    _st(wo_s, j, r0=h0 * D, val=w)
                else:
                    w = _ld(wo_s, j, r0=h0 * D, n=CH * D)
                y = _dot(ctx, w)
                acc[j] = acc[j] + y if h0 else y
                if h0 + CH == H:
                    y_s[slot][pl.ds(0, n), pl.ds(j * D, D)] = acc[j]
                return y
            return [functools.partial(job, j, h0) for j in range(M // D) for h0 in range(0, H, CH)]

        def out_copy(b):
            return pltpu.make_async_copy(out_s.at[_rows(b * RB, RB)], out_hbm.at[_rows(b * RB, RB)],
                                         out_sem.at[b])

        def epilogue(r0, slot, off, n, tok=None):
            _after(tok, zero, x_s, y_s[slot])
            rows = _rows(r0, n)
            ga, sb, cb, gb = mod(2), mod(3), _rb(1.0 + mod(4)), mod(5)
            x1 = _rb(x_s[rows, :].astype(f32) + _rb(ga * _rb(y_s[slot][pl.ds(off, n), :])))
            mean = jnp.mean(x1, axis=1, keepdims=True)
            xc = x1 - mean
            var = _rb(jnp.mean(xc * xc, axis=1, keepdims=True))
            inv = 1.0 / _rb(jnp.sqrt(_rb(var + EPS)))
            h2 = _rb(_rb(_rb(_rb(x1 - _rb(mean)) * inv) * cb) + sb)
            xh_s[rows, :] = pltpu.bitcast(x1, u32) | (pltpu.bitcast(h2, u32) >> 16)
            out_s[rows, :] = (x1 + _rb(gb * h2)).astype(bf16)
            wr = wr_s[...].astype(f32)
            prod = h2[:, 0:D] * wr[0:1]
            for j in range(1, M // D):
                prod = prod + h2[:, j * D:(j + 1) * D] * wr[j:j + 1]
            r = jnp.broadcast_to(_rb(jnp.sum(prod, axis=1, keepdims=True)), (n, D))
            bits = lax.bitcast_convert_type(r, i32)
            code = lax.shift_right_logical(bits, 16)
            code = jnp.where(bits < 0, 0xFFFF - code, code + 0x8000)
            code = jnp.where(r == 0.0, 0x8000, code)
            code = jnp.where(r != r, 0, code)
            key = code * S + (S - 1 + KEY0 - r0) - lax.broadcasted_iota(i32, (n, D), 0)
            key_s[pl.ds(off % T, n), :] = lax.bitcast_convert_type(key, f32)

        def select(tok=None):
            best = top_s[...]
            cols = [key_s[pl.ds(8 * t, 8), :] for t in range(T // 8)]
            flat = jnp.zeros((TOPK, D), f32)
            for t, col in enumerate(cols):
                flat = jnp.where(lane - sub == 8 * t, col, flat)
            new = None
            for cand in (flat, jnp.where(lane == sub, best, 0.0)):
                cand = jnp.broadcast_to(jnp.max(cand, axis=0, keepdims=True), (TOPK, D))
                above = sum((col > cand).astype(f32) for col in cols + [best])
                rank = jnp.sum(above, axis=0, keepdims=True)
                pick = jnp.where(rank == sub.astype(f32), cand, 0.0)
                new = pick if new is None else jnp.maximum(new, pick)
            top_s[...] = jnp.broadcast_to(jnp.max(new, axis=1, keepdims=True), (TOPK, D))

        def epilogues(r0, slot, rows=RB, n=16):
            jobs = []
            for off in range(0, rows, n):
                jobs.append(functools.partial(epilogue, r0 + off, slot, off, n))
                if (off + n) % T == 0:
                    jobs.append(select)
            return jobs

        def flip(t, src):
            def job(r0, tok):
                _after(tok, zero, src)
                wgu_s[t, :, pl.ds(r0, D)] = src[pl.ds(r0, D), :].T
            return [functools.partial(job, r0) for r0 in range(0, F - D, D)] + [
                functools.partial(job, F - D)]

        NR = S // RB
        top_s[...] = jnp.zeros(top_s.shape, f32)
        last = oproj((NR - 1) * RB, RB, 1, first=True)
        cuts = [0] * 4 + [len(last) * n // 15 for n in range(1, 16)]
        _attention(q_s, k_s, v_s, 0, H - 1, 1, lambda n: _weave(last[cuts[n]:cuts[n + 1]]), lag=0)

        flips = flip(0, wg_s) + flip(1, wu_s)
        for n, b in enumerate(range(NR - 2, 0, -1)):
            _weave(oproj(b * RB, RB, b % 2), epilogues((b + 1) * RB, (b + 1) % 2) + _skip(2),
                   flips[7 * n:7 * n + 7])
            out_copy(b + 1).start()
            if n == 4:
                wait([out_copy(b) for b in range(b + 2, NR)])
        _weave(oproj(T, T, 0), epilogues(RB, 1))
        out_copy(1).start()
        _weave(oproj(0, T, 1), epilogues(T, 0, T) + _skip(2))
        _weave(epilogues(0, 1, T, T))
        out_copy(0).start()

        top = lax.bitcast_convert_type(top_s[...], i32) - KEY0
        sel = S - 1 - (top & (S - 1))
        code = lax.shift_right_logical(top, 11)
        code = jnp.where(code >= 0x8000, code - 0x8000, 0xFFFF - code)
        r_sel = lax.bitcast_convert_type(code * 0x10000, f32)[:, 0:1]
        idx = [sel[j, 0] for j in range(TOPK)]

        both = jnp.concatenate([xh_s[pl.ds(t, 1), :] for t in idx], axis=0)
        hsel = pltpu.bitcast(both << 16, f32)
        xsel = pltpu.bitcast((both >> 16) << 16, f32)
        lhs = jnp.concatenate([hsel, hsel], axis=0).astype(bf16)
        gate = _rb(_dot(lhs, wgu_s[0]))
        act = _rb(gate * _sigmoid(gate)) * _rb(_dot(lhs, wgu_s[1]))
        y = _rb(_rb(_dot(act.astype(bf16), wd_s[...])[0:TOPK]) * _sigmoid(r_sel))
        fixed = xsel + _rb(mod(5) * _rb(hsel + y))

        wait([out_copy(b) for b in range(4)])
        tiles = [pl.multiple_of((t // 16) * 16, 16) for t in idx]
        row = lax.broadcasted_iota(i32, (16, M), 0)
        for j in range(TOPK):
            cur = out_s[pl.ds(tiles[j], 16), :].astype(f32)
            cur = jnp.where(row == idx[j] - tiles[j], fixed[j:j + 1], cur)
            out_s[pl.ds(tiles[j], 16), :] = cur.astype(bf16)

        def fix_copy(j):
            return pltpu.make_async_copy(out_s.at[pl.ds(tiles[j], 16)], out_hbm.at[pl.ds(tiles[j], 16)],
                                         fix_sem.at[j])

        fresh = []
        for j in range(TOPK):
            new = tiles[j] >= 0
            for k in range(j):
                new = jnp.logical_and(new, tiles[j] != tiles[k])
            fresh.append(new)
        for j in range(TOPK):
            pl.when(fresh[j])(fix_copy(j).start)
        for j in range(TOPK):
            pl.when(fresh[j])(fix_copy(j).wait)

    pl.run_scoped(phase3, V((S, M), u32), V((S, M), bf16), V((2, M, F), bf16), V((T, D), f32),
                  [V((RB + PAD, M), f32)] * 2, V((TOPK, D), f32))


@jax.jit
def pallas_adaLN_cond__compressed_kv_cla__moe_arch_mod__prompt_kernel(
    A_x: jax.Array,
    A_c_kv: jax.Array,
    A_w_q: jax.Array,
    A_w_uk: jax.Array,
    A_w_uv: jax.Array,
    A_w_o: jax.Array,
    B_x: jax.Array,
    B_w_r: jax.Array,
    B_w_gate: jax.Array,
    B_w_up: jax.Array,
    B_w_down: jax.Array,
    c: jax.Array,
    w_mod: jax.Array,
):
    del B_x
    V = pltpu.VMEM
    scratch = [
        V((H, S // 2, D), u32),
        V((H + M // D, S // 2, D), u32),
        V((2, S // 2, D), u32), V((2, S // 2, D), u32), V((S // 2, C), u32),
        V((M // D, H * D // 2, D), u32), V((H * D, M), bf16),
        V((S + PAD, M), bf16),
        V((F + PAD, M), bf16), V((F + PAD, M), bf16), V((F, M), bf16),
        V((1, 6 * M), f32), V((M // D, D), bf16),
        pltpu.SemaphoreType.DMA((19,)), pltpu.SemaphoreType.DMA((S // RB,)),
        pltpu.SemaphoreType.DMA((TOPK,)),
    ]
    out = pl.pallas_call(
        _kernel,
        in_specs=[pl.BlockSpec(memory_space=pltpu.HBM)] * 12,
        out_specs=pl.BlockSpec(memory_space=pltpu.HBM),
        out_shape=jax.ShapeDtypeStruct((S, M), bf16),
        scratch_shapes=scratch,
        compiler_params=pltpu.CompilerParams(vmem_limit_bytes=120 * 2 ** 20),
    )(A_x.reshape(S, M), A_c_kv.reshape(S, C), A_w_q, A_w_uk, A_w_uv, A_w_o.reshape(H * D, M),
      B_w_r.reshape(M // D, D), B_w_gate.T, B_w_up.T, B_w_down, c, w_mod)
    return out.reshape(A_x.shape)
```

```python
import functools

import jax
import jax.numpy as jnp
from jax import lax
import jax.experimental.pallas as pl
import jax.experimental.pallas.tpu as pltpu

S, M, C, D, H, F, TOPK = 2048, 640, 512, 128, 32, 1728, 8
G = 8
NG = H // G
T = 128
NB = S // T
CH = 4
RB = 256
NF = -(-F // D)
PAD = 16
EPS = 1e-5
KEY0 = 0x00800000
QSCALE = D ** -0.5 * 1.4426950408889634
NT = (((1,), (1,)), ((), ()))

f32, bf16, u32, i32 = jnp.float32, jnp.bfloat16, jnp.uint32, jnp.int32


def _rb(a):
    return a.astype(bf16).astype(f32)


def _sigmoid(a):
    return _rb(1.0 / _rb(1.0 + _rb(jnp.exp(-a))))


def _rows(r0, n):
    if isinstance(r0, int):
        return pl.ds(r0, n)
    return pl.ds(pl.multiple_of(r0, n & -n), n)


def _ld(ref, *idx, r0, n):
    return pltpu.bitcast(ref[(*idx, _rows(r0 // 2, n // 2), slice(None))], bf16)


def _st(ref, *idx, r0, val):
    ref[(*idx, _rows(r0 // 2, val.shape[0] // 2), slice(None))] = pltpu.bitcast(
        val.astype(bf16), u32)


def _dot(a, b):
    return jnp.dot(a, b, preferred_element_type=f32)


def _dot_nt(a, b):
    return lax.dot_general(a, b, NT, preferred_element_type=f32)


class _Blk:
    def __init__(self, i):
        self.i, self.s, self.mx, self.m, self.l, self.acc = i, {}, None, None, None, None


def _attention(q_s, k_s, v_s, zero, hd, slot, filler, lag=3):
    tri = (lax.broadcasted_iota(i32, (T, T), 1) <= lax.broadcasted_iota(i32, (T, T), 0))

    def chunks(b):
        n = b.i + 1 if b else 0
        return [(a, min(a + CH, n)) for a in range(0, n, CH)]

    def scores(b, a, e):
        return _dot_nt(_ld(q_s, slot, r0=b.i * T, n=T), _ld(k_s, hd, r0=a * T, n=(e - a) * T))

    def keep(b, a, e, s):
        for t in range(a, e):
            x = s[:, (t - a) * T:(t - a + 1) * T]
            if t == b.i:
                x = jnp.where(tri, x, -1e9)
            b.mx = x if b.mx is None else jnp.maximum(b.mx, x)
            b.s[t] = x

    def context(b, a, e):
        ps = sums = [jnp.exp2(b.s[t] - b.m) for t in range(a, e)]
        while len(sums) > 1:
            sums = [functools.reduce(jnp.add, sums[t:t + 2]) for t in range(0, len(sums), 2)]
        b.l = sums[0] if b.l is None else b.l + sums[0]
        p = (jnp.concatenate(ps, axis=1) if len(ps) > 1 else ps[0]).astype(bf16)
        o = _dot(p, _ld(v_s, slot, r0=a * T, n=(e - a) * T))
        b.acc = o if b.acc is None else b.acc + o

    def finish(b):
        l = jnp.sum(b.l, axis=1, keepdims=True)
        r = pltpu.reciprocal(l, approx=True)
        r = r * (2.0 - l * r)
        _st(k_s, hd + zero, r0=b.i * T, val=b.acc * r)

    filler(0)
    prev, done = None, []
    for n, i in enumerate(list(range(NB - 1, -1, -1)) + [None]):
        b = _Blk(i) if i is not None else None
        ca, cb = chunks(b), chunks(prev)
        for c in range(max(len(ca), len(cb))):
            s = scores(b, *ca[c]) if c < len(ca) else None
            if c < len(cb):
                context(prev, *cb[c])
            if s is not None:
                keep(b, *ca[c], s)
        if b:
            b.m = jnp.max(b.mx, axis=1, keepdims=True)
        if prev:
            done.append(prev)
        if len(done) > lag:
            finish(done.pop(0))
        filler(n + 1)
        prev = b
    for b in done:
        finish(b)


def _weave(mxu, *others):
    for n, job in enumerate(mxu):
        out = job()
        todo = [other for vpu in others
                for other in vpu[n * len(vpu) // len(mxu):(n + 1) * len(vpu) // len(mxu)]]
        for t, other in enumerate(todo):
            r0 = t * (out.shape[0] // PAD) // len(todo) * PAD
            other(out[r0:r0 + PAD, 0:D])


def _skip(n):
    return [lambda tok: None] * n


def _zero(a):
    return jnp.minimum(pltpu.bitcast(a, i32)[0, 0] & 0xFFFF, 0)


def _after(tok, zero, *refs):
    if tok is None:
        return
    for ref in refs:
        if len(ref.shape) == 3:
            ref[zero + ref.shape[0] - 1, pl.ds(0, G), :] = tok[0:G].astype(ref.dtype)
        else:
            ref[_rows(zero + ref.shape[0] - PAD, PAD), pl.ds(0, D)] = tok.astype(ref.dtype)


def _kernel(x_hbm, ckv_hbm, wq_hbm, wk_hbm, wv_hbm, wo_hbm, wr_hbm, wg_hbm, wu_hbm, wd_hbm,
            c_hbm, wmod_hbm, out_hbm,
            k_s, w_s, q_s, v_s, ckv_s, wo_s, x_s, wg_s, wu_s, wd_s, mod_s, wr_s,
            in_sem, out_sem, fix_sem):
    copies = []

    def copy(hbm, vmem, rows=None):
        if rows is not None:
            hbm, vmem = hbm.at[rows], vmem.at[rows]
        elif hbm.shape != vmem.shape:
            vmem = vmem.at[pl.ds(0, hbm.shape[0])]
        copies.append(pltpu.make_async_copy(hbm, vmem, in_sem.at[len(copies)]))
        return copies[-1]

    def start(cps):
        for cp in cps:
            cp.start()

    def wait(cps):
        for cp in cps:
            cp.wait()

    stage4 = [copy(wo_hbm, wo_s), copy(wr_hbm, wr_s), copy(wg_hbm, wg_s), copy(wu_hbm, wu_s),
              copy(wd_hbm, wd_s)]

    def mod(j):
        return mod_s[:, pl.ds(j * M, M)]

    def qproj(hd, slot, i):
        h = jnp.concatenate([_ld(w_s, H + j, r0=i * T, n=T) for j in range(M // D)], axis=1)
        _st(q_s, slot, r0=i * T, val=_dot(h, _ld(w_s, hd, r0=0, n=M)) * QSCALE)

    def vproj(hd, slot, i):
        _st(v_s, slot, r0=i * T, val=_dot(_ld(ckv_s, r0=i * T, n=T), _ld(w_s, hd, r0=M + C, n=C)))

    def qv(hd, slot):
        return [functools.partial(f, hd, slot, i) for i in range(NB) for f in (qproj, vproj)]

    def phase1(ckv_raw, wq_raw, wv_raw, wk0, wk1, wk2, wmod_s, c_s):
        R0, R1 = 256, 1024
        first = [copy(wk_hbm.at[:, pl.ds(0, G)], wk0, pl.ds(r0, D)) for r0 in range(0, C, D)]
        ckv0_cp = copy(ckv_hbm, ckv_raw, pl.ds(0, R0))
        ckv1_cp = copy(ckv_hbm, ckv_raw, pl.ds(R0, R1 - R0))
        stage1 = [copy(ckv_hbm, ckv_raw, pl.ds(R1, S - R1)),
                  copy(wk_hbm.at[:, pl.ds(G, G)], wk1)]
        stage2 = [copy(wk_hbm.at[:, pl.ds(2 * G, 2 * G)], wk2),
                  copy(c_hbm, c_s), copy(wmod_hbm, wmod_s), copy(x_hbm, x_s)]
        stage3 = [copy(wq_hbm, wq_raw), copy(wv_hbm, wv_raw)]

        def per_head(raw, base, g):
            def job(r0, tok=None):
                _after(tok, zero, raw)
                w = raw[pl.ds(r0, 16), pl.ds(g * G % raw.shape[1], G), :].reshape(16, G * D)
                for j in range(G):
                    _st(w_s, g * G + j, r0=base + r0, val=w[:, j * D:(j + 1) * D])
            return [functools.partial(job, r0) for r0 in range(0, raw.shape[0] - 1, 16)]

        def kproj(heads, lo, hi):
            def job(hd, r0):
                if hd == 0:
                    ckv = ckv_raw[pl.ds(r0, 256), :]
                    _st(ckv_s, r0=r0, val=ckv)
                else:
                    ckv = _ld(ckv_s, r0=r0, n=256)
                k = _dot(ckv, _ld(w_s, hd, r0=M, n=C))
                _st(k_s, hd, r0=r0, val=k)
                return k
            return [functools.partial(job, hd, r0) for hd in heads for r0 in range(lo, hi, 256)]

        def modulation():
            cf = c_s[...].astype(f32)
            col = jnp.broadcast_to(_rb(cf * _sigmoid(cf)), (D, M)).T
            acc = {}

            def job(c0, r0, tok):
                _after(tok, zero, wmod_s)
                w = wmod_s[pl.ds(r0, D), pl.ds(c0, 2 * D)].astype(f32)
                w = w * jnp.concatenate([col[r0:r0 + D]] * 2, axis=1)
                w = jnp.sum(w.reshape(D // 8, 8, 2 * D), axis=0)
                acc[c0] = acc[c0] + w if r0 else w
                if r0 + D == M:
                    mod_s[:, pl.ds(c0, 2 * D)] = _rb(jnp.sum(acc[c0], axis=0, keepdims=True))
            return [functools.partial(job, c0, r0)
                    for c0 in range(0, 6 * M, 2 * D) for r0 in range(0, M, D)]

        def norm1(r0, tok):
            _after(tok, zero, x_s)
            xf = x_s[pl.ds(r0, 16), :].astype(f32)
            xc = xf - jnp.mean(xf, axis=1, keepdims=True)
            xn = xc * lax.rsqrt(jnp.mean(xc * xc, axis=1, keepdims=True) + EPS)
            h = xn * (1.0 + mod(1)) + mod(0)
            for j in range(M // D):
                _st(w_s, H + j, r0=r0, val=h[:, j * D:(j + 1) * D])

        start(first + [ckv0_cp])
        for n, cp in enumerate(first):
            if n == 2:
                ckv1_cp.start()
            cp.wait()
            if n == 0:
                zero = _zero(wk0[0])
            _weave(per_head(wk0, M, 0)[n * D // 16:(n + 1) * D // 16])
        start(stage1)
        ckv0_cp.wait()
        _weave(kproj(range(8), 0, R0))
        start(stage2)
        ckv1_cp.wait()
        _weave(kproj(range(8), R0, R1))
        wait(stage1)
        _weave(kproj(range(8), R1, S), per_head(wk1, M, 1))
        _weave(kproj(range(8, 13), 0, S))
        start(stage3)
        wait(stage2)
        _weave(kproj(range(13, 17), 0, S), per_head(wk2, M, 2) + _skip(14),
               _skip(6) + modulation())
        _weave(kproj(range(17, 24), 0, S), per_head(wk2, M, 3),
               [functools.partial(norm1, r0) for r0 in range(0, S, 16)] + _skip(12))
        start(stage4)
        wait(stage3)
        _weave(kproj(range(24, H), 0, S),
               [job for g in range(NG) for job in per_head(wq_raw, 0, g) + per_head(wv_raw, M + C, g)])
        _weave(qv(0, 0))

    V = pltpu.VMEM
    pl.run_scoped(phase1, V((S, C), bf16), V((M + 1, H, D), bf16), V((C + 1, H, D), bf16),
                  V((C, G, D), bf16), V((C + 1, G, D), bf16), V((C + 1, 2 * G, D), bf16),
                  V((M + PAD, 6 * M), bf16), V((1, M), bf16))

    zero = _zero(x_s[pl.ds(0, 16), pl.ds(0, D)])

    def next_head(hd, slot):
        jobs = qv(hd, slot)
        cuts = [0, 1] + [1 + (27 * n) // NB for n in range(1, NB + 1)] + [len(jobs)]
        return lambda n: _weave(jobs[cuts[n]:cuts[n + 1]])

    def pair(p, _):
        _attention(q_s, k_s, v_s, zero, 2 * p + 1, 1, next_head(2 * p + 2, 0))
        _attention(q_s, k_s, v_s, zero, 2 * p + 2, 0, next_head(2 * p + 3, 1))

    _attention(q_s, k_s, v_s, zero, 0, 0, next_head(1, 1))
    lax.fori_loop(0, H // 2 - 1, pair, None)

    def phase3(xh_s, out_s, wgu_s, key_s, y_s, top_s):
        wait(stage4)
        sub = lax.broadcasted_iota(i32, (TOPK, D), 0)
        lane = lax.broadcasted_iota(i32, (TOPK, D), 1)

        def oproj(r0, n, slot):
            acc = {}

            def job(j, h0):
                ctx = jnp.concatenate([_ld(k_s, h0 + t, r0=r0, n=n) for t in range(CH)], axis=1)
                y = _dot(ctx, wo_s[pl.ds(h0 * D, CH * D), pl.ds(j * D, D)])
                acc[j] = acc[j] + y if h0 else y
                if h0 + CH == H:
                    y_s[slot][pl.ds(0, n), pl.ds(j * D, D)] = acc[j]
                return y
            return [functools.partial(job, j, h0) for j in range(M // D) for h0 in range(0, H, CH)]

        def out_copy(b):
            return pltpu.make_async_copy(out_s.at[_rows(b * RB, RB)], out_hbm.at[_rows(b * RB, RB)],
                                         out_sem.at[b])

        def epilogue(r0, slot, off, n, tok=None):
            _after(tok, zero, x_s, y_s[slot])
            rows = _rows(r0, n)
            ga, sb, cb, gb = mod(2), mod(3), _rb(1.0 + mod(4)), mod(5)
            x1 = _rb(x_s[rows, :].astype(f32) + _rb(ga * _rb(y_s[slot][pl.ds(off, n), :])))
            mean = jnp.mean(x1, axis=1, keepdims=True)
            xc = x1 - mean
            var = _rb(jnp.mean(xc * xc, axis=1, keepdims=True))
            inv = 1.0 / _rb(jnp.sqrt(_rb(var + EPS)))
            h2 = _rb(_rb(_rb(_rb(x1 - _rb(mean)) * inv) * cb) + sb)
            xh_s[rows, :] = pltpu.bitcast(x1, u32) | (pltpu.bitcast(h2, u32) >> 16)
            out_s[rows, :] = (x1 + _rb(gb * h2)).astype(bf16)
            wr = wr_s[...].astype(f32)
            prod = h2[:, 0:D] * wr[0:1]
            for j in range(1, M // D):
                prod = prod + h2[:, j * D:(j + 1) * D] * wr[j:j + 1]
            r = jnp.broadcast_to(_rb(jnp.sum(prod, axis=1, keepdims=True)), (n, D))
            bits = lax.bitcast_convert_type(r, i32)
            code = lax.shift_right_logical(bits, 16)
            code = jnp.where(bits < 0, 0xFFFF - code, code + 0x8000)
            code = jnp.where(r == 0.0, 0x8000, code)
            code = jnp.where(r != r, 0, code)
            key = code * S + (S - 1 + KEY0 - r0) - lax.broadcasted_iota(i32, (n, D), 0)
            key_s[pl.ds(off % T, n), :] = lax.bitcast_convert_type(key, f32)

        def select(tok=None):
            best = top_s[...]
            cols = [key_s[pl.ds(8 * t, 8), :] for t in range(T // 8)]
            flat = jnp.zeros((TOPK, D), f32)
            for t, col in enumerate(cols):
                flat = jnp.where(lane - sub == 8 * t, col, flat)
            new = None
            for cand in (flat, jnp.where(lane == sub, best, 0.0)):
                cand = jnp.broadcast_to(jnp.max(cand, axis=0, keepdims=True), (TOPK, D))
                above = sum((col > cand).astype(f32) for col in cols + [best])
                rank = jnp.sum(above, axis=0, keepdims=True)
                pick = jnp.where(rank == sub.astype(f32), cand, 0.0)
                new = pick if new is None else jnp.maximum(new, pick)
            top_s[...] = jnp.broadcast_to(jnp.max(new, axis=1, keepdims=True), (TOPK, D))

        def epilogues(r0, slot, rows=RB, n=16):
            jobs = []
            for off in range(0, rows, n):
                jobs.append(functools.partial(epilogue, r0 + off, slot, off, n))
                if (off + n) % T == 0:
                    jobs.append(select)
            return jobs

        def flip(src, dst, f0, n):
            def job(f, tok):
                _after(tok, zero, src)
                f = jnp.minimum(f, NF - 1)
                dst[f] = src[pl.ds(pl.multiple_of(jnp.minimum(f * D, F - D), 64), D), :].T
            return [functools.partial(job, f0 + t) for t in range(n)]

        NR = S // RB
        top_s[...] = jnp.zeros(top_s.shape, f32)
        last = oproj((NR - 1) * RB, RB, 1)
        cuts = [0] * 4 + [len(last) * n // 15 for n in range(1, 16)]
        _attention(q_s, k_s, v_s, 0, H - 1, 1, lambda n: _weave(last[cuts[n]:cuts[n + 1]]), lag=0)

        def blocks(n, _):
            b = NR - 2 - 2 * n
            _weave(oproj(b * RB, RB, 0), epilogues((b + 1) * RB, 1) + _skip(2),
                   flip(wg_s, wgu_s[0], 5 * n, 5))
            out_copy(b + 1).start()
            _weave(oproj((b - 1) * RB, RB, 1), epilogues(b * RB, 0) + _skip(2),
                   flip(wu_s, wgu_s[1], 5 * n, 5) + _skip(1))
            out_copy(b).start()

        lax.fori_loop(0, NR // 2 - 1, blocks, None)
        _weave(oproj(T, T, 0), epilogues(RB, 1))
        out_copy(1).start()
        _weave(oproj(0, T, 1), epilogues(T, 0, T) + _skip(2))
        _weave(epilogues(0, 1, T, T))
        out_copy(0).start()

        top = lax.bitcast_convert_type(top_s[...], i32) - KEY0
        sel = S - 1 - (top & (S - 1))
        code = lax.shift_right_logical(top, 11)
        code = jnp.where(code >= 0x8000, code - 0x8000, 0xFFFF - code)
        r_sel = lax.bitcast_convert_type(code * 0x10000, f32)[:, 0:1]
        idx = [sel[j, 0] for j in range(TOPK)]

        both = jnp.concatenate([xh_s[pl.ds(t, 1), :] for t in idx], axis=0)
        hsel = pltpu.bitcast(both << 16, f32)
        xsel = pltpu.bitcast((both >> 16) << 16, f32)
        lhs = jnp.concatenate([hsel, hsel], axis=0).astype(bf16)
        acts = []
        for f in range(NF):
            gate = _rb(_dot(lhs, wgu_s[0][f]))
            acts.append(_rb(gate * _sigmoid(gate)) * _rb(_dot(lhs, wgu_s[1][f])))
        seen = lax.broadcasted_iota(i32, acts[-1].shape, 1) < NF * D - F
        acts[-1] = jnp.where(seen, 0.0, acts[-1])
        y = sum(_dot(act.astype(bf16), wd_s[pl.ds(min(f * D, F - D), D), :])
                for f, act in enumerate(acts))
        y = _rb(_rb(y[0:TOPK]) * _sigmoid(r_sel))
        fixed = xsel + _rb(mod(5) * _rb(hsel + y))

        wait([out_copy(b) for b in range(NR)])
        tiles = [pl.multiple_of((t // 16) * 16, 16) for t in idx]
        row = lax.broadcasted_iota(i32, (16, M), 0)
        for j in range(TOPK):
            cur = out_s[pl.ds(tiles[j], 16), :].astype(f32)
            cur = jnp.where(row == idx[j] - tiles[j], fixed[j:j + 1], cur)
            out_s[pl.ds(tiles[j], 16), :] = cur.astype(bf16)

        def fix_copy(j):
            return pltpu.make_async_copy(out_s.at[pl.ds(tiles[j], 16)], out_hbm.at[pl.ds(tiles[j], 16)],
                                         fix_sem.at[j])

        fresh = []
        for j in range(TOPK):
            new = tiles[j] >= 0
            for k in range(j):
                new = jnp.logical_and(new, tiles[j] != tiles[k])
            fresh.append(new)
        for j in range(TOPK):
            pl.when(fresh[j])(fix_copy(j).start)
        for j in range(TOPK):
            pl.when(fresh[j])(fix_copy(j).wait)

    pl.run_scoped(phase3, V((S, M), u32), V((S, M), bf16), [V((NF, M, D), bf16)] * 2, V((T, D), f32),
                  [V((RB + PAD, M), f32)] * 2, V((TOPK, D), f32))


@jax.jit
def pallas_adaLN_cond__compressed_kv_cla__moe_arch_mod__prompt_kernel(
    A_x: jax.Array,
    A_c_kv: jax.Array,
    A_w_q: jax.Array,
    A_w_uk: jax.Array,
    A_w_uv: jax.Array,
    A_w_o: jax.Array,
    B_x: jax.Array,
    B_w_r: jax.Array,
    B_w_gate: jax.Array,
    B_w_up: jax.Array,
    B_w_down: jax.Array,
    c: jax.Array,
    w_mod: jax.Array,
):
    del B_x
    V = pltpu.VMEM
    scratch = [
        V((H, S // 2, D), u32),
        V((H + M // D, S // 2, D), u32),
        V((2, S // 2, D), u32), V((2, S // 2, D), u32), V((S // 2, C), u32),
        V((H * D, M), bf16), V((S + PAD, M), bf16),
        V((F + PAD, M), bf16), V((F + PAD, M), bf16), V((F, M), bf16),
        V((1, 6 * M), f32), V((M // D, D), bf16),
        pltpu.SemaphoreType.DMA((19,)), pltpu.SemaphoreType.DMA((S // RB,)),
        pltpu.SemaphoreType.DMA((TOPK,)),
    ]
    out = pl.pallas_call(
        _kernel,
        in_specs=[pl.BlockSpec(memory_space=pltpu.HBM)] * 12,
        out_specs=pl.BlockSpec(memory_space=pltpu.HBM),
        out_shape=jax.ShapeDtypeStruct((S, M), bf16),
        scratch_shapes=scratch,
        compiler_params=pltpu.CompilerParams(vmem_limit_bytes=120 * 2 ** 20),
    )(A_x.reshape(S, M), A_c_kv.reshape(S, C), A_w_q, A_w_uk, A_w_uv, A_w_o.reshape(H * D, M),
      B_w_r.reshape(M // D, D), B_w_gate.T, B_w_up.T, B_w_down, c, w_mod)
    return out.reshape(A_x.shape)
```

```python
import functools

import jax
import jax.numpy as jnp
from jax import lax
import jax.experimental.pallas as pl
import jax.experimental.pallas.tpu as pltpu

S, M, C, D, H, F, TOPK = 2048, 640, 512, 128, 32, 1728, 8
G = 8
NG = H // G
T = 128
NB = S // T
CH = 4
RB = 256
NF = -(-F // D)
PAD = 16
EPS = 1e-5
KEY0 = 0x00800000
QSCALE = D ** -0.5 * 1.4426950408889634
NT = (((1,), (1,)), ((), ()))

f32, bf16, u32, i32 = jnp.float32, jnp.bfloat16, jnp.uint32, jnp.int32


def _rb(a):
    return a.astype(bf16).astype(f32)


def _sigmoid(a):
    return _rb(1.0 / _rb(1.0 + _rb(jnp.exp(-a))))


def _rows(r0, n):
    if isinstance(r0, int):
        return pl.ds(r0, n)
    return pl.ds(pl.multiple_of(r0, n & -n), n)


def _ld(ref, *idx, r0, n):
    return pltpu.bitcast(ref[(*idx, _rows(r0 >> 1, n // 2), slice(None))], bf16)


def _st(ref, *idx, r0, val):
    ref[(*idx, _rows(r0 >> 1, val.shape[0] // 2), slice(None))] = pltpu.bitcast(
        val.astype(bf16), u32)


def _dot(a, b):
    return jnp.dot(a, b, preferred_element_type=f32)


def _dot_nt(a, b):
    return lax.dot_general(a, b, NT, preferred_element_type=f32)


class _Blk:
    def __init__(self, i):
        self.i, self.s, self.mx, self.m, self.l, self.acc = i, {}, None, None, None, None


def _attention(q_s, k_s, v_s, zero, hd, slot, filler, lag=3):
    tri = (lax.broadcasted_iota(i32, (T, T), 1) <= lax.broadcasted_iota(i32, (T, T), 0))

    def chunks(b):
        n = b.i + 1 if b else 0
        return [(a, min(a + CH, n)) for a in range(0, n, CH)]

    def scores(b, a, e):
        return _dot_nt(_ld(q_s, slot, r0=b.i * T, n=T), _ld(k_s, hd, r0=a * T, n=(e - a) * T))

    def keep(b, a, e, s):
        for t in range(a, e):
            x = s[:, (t - a) * T:(t - a + 1) * T]
            if t == b.i:
                x = jnp.where(tri, x, -1e9)
            b.mx = x if b.mx is None else jnp.maximum(b.mx, x)
            b.s[t] = x

    def context(b, a, e):
        ps = sums = [jnp.exp2(b.s[t] - b.m) for t in range(a, e)]
        while len(sums) > 1:
            sums = [functools.reduce(jnp.add, sums[t:t + 2]) for t in range(0, len(sums), 2)]
        b.l = sums[0] if b.l is None else b.l + sums[0]
        p = (jnp.concatenate(ps, axis=1) if len(ps) > 1 else ps[0]).astype(bf16)
        o = _dot(p, _ld(v_s, slot, r0=a * T, n=(e - a) * T))
        b.acc = o if b.acc is None else b.acc + o

    def finish(b):
        l = jnp.sum(b.l, axis=1, keepdims=True)
        r = pltpu.reciprocal(l, approx=True)
        r = r * (2.0 - l * r)
        _st(k_s, hd + zero, r0=b.i * T, val=b.acc * r)

    filler(0)
    prev, done = None, []
    for n, i in enumerate(list(range(NB - 1, -1, -1)) + [None]):
        b = _Blk(i) if i is not None else None
        ca, cb = chunks(b), chunks(prev)
        for c in range(max(len(ca), len(cb))):
            s = scores(b, *ca[c]) if c < len(ca) else None
            if c < len(cb):
                context(prev, *cb[c])
            if s is not None:
                keep(b, *ca[c], s)
        if b:
            b.m = jnp.max(b.mx, axis=1, keepdims=True)
        if prev:
            done.append(prev)
        if len(done) > lag:
            finish(done.pop(0))
        filler(n + 1)
        prev = b
    for b in done:
        finish(b)


def _weave(mxu, *others):
    for n, job in enumerate(mxu):
        out = job()
        todo = [other for vpu in others
                for other in vpu[n * len(vpu) // len(mxu):(n + 1) * len(vpu) // len(mxu)]]
        for t, other in enumerate(todo):
            r0 = t * (out.shape[0] // PAD) // len(todo) * PAD
            other(out[r0:r0 + PAD, 0:D])


def _skip(n):
    return [lambda tok: None] * n


def _zero(a):
    return jnp.minimum(pltpu.bitcast(a, i32)[0, 0] & 0xFFFF, 0)


def _after(tok, zero, *refs):
    if tok is None:
        return
    for ref in refs:
        if len(ref.shape) == 3:
            ref[zero + ref.shape[0] - 1, pl.ds(0, G), :] = tok[0:G].astype(ref.dtype)
        else:
            ref[_rows(zero + ref.shape[0] - PAD, PAD), pl.ds(0, D)] = tok.astype(ref.dtype)


def _kernel(x_hbm, ckv_hbm, wq_hbm, wk_hbm, wv_hbm, wo_hbm, wr_hbm, wg_hbm, wu_hbm, wd_hbm,
            c_hbm, wmod_hbm, out_hbm,
            k_s, w_s, q_s, v_s, ckv_s, wo_s, x_s, wg_s, wu_s, wd_s, mod_s, wr_s,
            in_sem, out_sem, fix_sem):
    copies = []

    def copy(hbm, vmem, rows=None):
        if rows is not None:
            hbm, vmem = hbm.at[rows], vmem.at[rows]
        elif hbm.shape != vmem.shape:
            vmem = vmem.at[pl.ds(0, hbm.shape[0])]
        copies.append(pltpu.make_async_copy(hbm, vmem, in_sem.at[len(copies)]))
        return copies[-1]

    def start(cps):
        for cp in cps:
            cp.start()

    def wait(cps):
        for cp in cps:
            cp.wait()

    stage4 = [copy(wo_hbm, wo_s), copy(wr_hbm, wr_s), copy(wg_hbm, wg_s), copy(wu_hbm, wu_s),
              copy(wd_hbm, wd_s)]

    def mod(j):
        return mod_s[:, pl.ds(j * M, M)]

    def qproj(hd, slot, i):
        h = jnp.concatenate([_ld(w_s, H + j, r0=i * T, n=T) for j in range(M // D)], axis=1)
        _st(q_s, slot, r0=i * T, val=_dot(h, _ld(w_s, hd, r0=0, n=M)) * QSCALE)

    def vproj(hd, slot, i):
        _st(v_s, slot, r0=i * T, val=_dot(_ld(ckv_s, r0=i * T, n=T), _ld(w_s, hd, r0=M + C, n=C)))

    def qv(hd, slot):
        return [functools.partial(f, hd, slot, i) for i in range(NB) for f in (qproj, vproj)]

    def phase1(ckv_raw, wq_raw, wv_raw, wk0, wk1, wk2, wmod_s, c_s):
        R0, R1 = 256, 1024
        first = [copy(wk_hbm.at[:, pl.ds(0, G)], wk0, pl.ds(r0, D)) for r0 in range(0, C, D)]
        ckv0_cp = copy(ckv_hbm, ckv_raw, pl.ds(0, R0))
        ckv1_cp = copy(ckv_hbm, ckv_raw, pl.ds(R0, R1 - R0))
        stage1 = [copy(ckv_hbm, ckv_raw, pl.ds(R1, S - R1)),
                  copy(wk_hbm.at[:, pl.ds(G, G)], wk1)]
        stage2 = [copy(wk_hbm.at[:, pl.ds(2 * G, 2 * G)], wk2),
                  copy(c_hbm, c_s), copy(wmod_hbm, wmod_s), copy(x_hbm, x_s)]
        stage3 = [copy(wq_hbm, wq_raw), copy(wv_hbm, wv_raw)]

        def per_head(raw, base, g):
            def job(r0, tok=None):
                _after(tok, zero, raw)
                w = raw[pl.ds(r0, 16), pl.ds(g * G % raw.shape[1], G), :].reshape(16, G * D)
                w = pltpu.bitcast(w, u32)
                for j in range(G):
                    w_s[g * G + j, pl.ds((base + r0) // 2, 8), :] = w[:, j * D:(j + 1) * D]
            return [functools.partial(job, r0) for r0 in range(0, raw.shape[0] - 1, 16)]

        def kproj(heads, lo, hi):
            def job(hd, r0):
                if hd == 0:
                    ckv = ckv_raw[pl.ds(r0, 256), :]
                    _st(ckv_s, r0=r0, val=ckv)
                else:
                    ckv = _ld(ckv_s, r0=r0, n=256)
                k = _dot(ckv, _ld(w_s, hd, r0=M, n=C))
                _st(k_s, hd, r0=r0, val=k)
                return k
            return [functools.partial(job, hd, r0) for hd in heads for r0 in range(lo, hi, 256)]

        def modulation():
            cf = c_s[...].astype(f32)
            col = jnp.broadcast_to(_rb(cf * _sigmoid(cf)), (D, M)).T
            acc = {}

            def job(c0, r0, tok):
                _after(tok, zero, wmod_s)
                w = wmod_s[pl.ds(r0, D), pl.ds(c0, 2 * D)].astype(f32)
                w = w * jnp.concatenate([col[r0:r0 + D]] * 2, axis=1)
                w = jnp.sum(w.reshape(D // 8, 8, 2 * D), axis=0)
                acc[c0] = acc[c0] + w if r0 else w
                if r0 + D == M:
                    mod_s[:, pl.ds(c0, 2 * D)] = _rb(jnp.sum(acc[c0], axis=0, keepdims=True))
            return [functools.partial(job, c0, r0)
                    for c0 in range(0, 6 * M, 2 * D) for r0 in range(0, M, D)]

        def norm1(r0, tok):
            _after(tok, zero, x_s)
            xf = x_s[pl.ds(r0, 16), :].astype(f32)
            xc = xf - jnp.mean(xf, axis=1, keepdims=True)
            xn = xc * lax.rsqrt(jnp.mean(xc * xc, axis=1, keepdims=True) + EPS)
            h = xn * (1.0 + mod(1)) + mod(0)
            for j in range(M // D):
                _st(w_s, H + j, r0=r0, val=h[:, j * D:(j + 1) * D])

        start(first + [ckv0_cp])
        for n, cp in enumerate(first):
            if n == 2:
                ckv1_cp.start()
            cp.wait()
            if n == 0:
                zero = _zero(wk0[0])
            _weave(per_head(wk0, M, 0)[n * D // 16:(n + 1) * D // 16])
        start(stage1)
        ckv0_cp.wait()
        _weave(kproj(range(8), 0, R0))
        start(stage2)
        ckv1_cp.wait()
        _weave(kproj(range(8), R0, R1))
        wait(stage1)
        _weave(kproj(range(8), R1, S), per_head(wk1, M, 1))
        _weave(kproj(range(8, 13), 0, S))
        start(stage3)
        wait(stage2)
        _weave(kproj(range(13, 17), 0, S), per_head(wk2, M, 2) + _skip(14),
               _skip(6) + modulation())
        _weave(kproj(range(17, 24), 0, S), per_head(wk2, M, 3),
               [functools.partial(norm1, r0) for r0 in range(0, S, 16)] + _skip(12))
        start(stage4)
        wait(stage3)
        _weave(kproj(range(24, H), 0, S),
               [job for g in range(NG) for job in per_head(wq_raw, 0, g) + per_head(wv_raw, M + C, g)])
        _weave(qv(0, 0))

    V = pltpu.VMEM
    pl.run_scoped(phase1, V((S, C), bf16), V((M + 1, H, D), bf16), V((C + 1, H, D), bf16),
                  V((C, G, D), bf16), V((C + 1, G, D), bf16), V((C + 1, 2 * G, D), bf16),
                  V((M + PAD, 6 * M), bf16), V((1, M), bf16))

    zero = _zero(x_s[pl.ds(0, 16), pl.ds(0, D)])

    def next_head(hd, slot):
        jobs = qv(hd, slot)
        cuts = [0, 1] + [1 + (27 * n) // NB for n in range(1, NB + 1)] + [len(jobs)]
        return lambda n: _weave(jobs[cuts[n]:cuts[n + 1]])

    def pair(p, _):
        _attention(q_s, k_s, v_s, zero, 2 * p + 1, 1, next_head(2 * p + 2, 0))
        _attention(q_s, k_s, v_s, zero, 2 * p + 2, 0, next_head(2 * p + 3, 1))

    _attention(q_s, k_s, v_s, zero, 0, 0, next_head(1, 1))
    lax.fori_loop(0, H // 2 - 1, pair, None)

    def phase3(xh_s, out_s, wgu_s, key_s, y_s, top_s):
        wait(stage4)
        sub = lax.broadcasted_iota(i32, (TOPK, D), 0)
        lane = lax.broadcasted_iota(i32, (TOPK, D), 1)

        def oproj(r0, n, slot):
            acc = {}

            def job(j, h0):
                ctx = jnp.concatenate([_ld(k_s, h0 + t, r0=r0, n=n) for t in range(CH)], axis=1)
                y = _dot(ctx, wo_s[pl.ds(h0 * D, CH * D), pl.ds(j * D, D)])
                acc[j] = acc[j] + y if h0 else y
                if h0 + CH == H:
                    y_s[slot][pl.ds(0, n), pl.ds(j * D, D)] = acc[j]
                return y
            return [functools.partial(job, j, h0) for j in range(M // D) for h0 in range(0, H, CH)]

        def out_copy(b):
            return pltpu.make_async_copy(out_s.at[_rows(b * RB, RB)], out_hbm.at[_rows(b * RB, RB)],
                                         out_sem.at[b])

        def epilogue(r0, slot, off, n, tok=None):
            _after(tok, zero, x_s, y_s[slot])
            rows = _rows(r0, n)
            ga, sb, cb, gb = mod(2), mod(3), _rb(1.0 + mod(4)), mod(5)
            x1 = _rb(x_s[rows, :].astype(f32) + _rb(ga * _rb(y_s[slot][pl.ds(off, n), :])))
            mean = jnp.mean(x1, axis=1, keepdims=True)
            xc = x1 - mean
            var = _rb(jnp.mean(xc * xc, axis=1, keepdims=True))
            inv = 1.0 / _rb(jnp.sqrt(_rb(var + EPS)))
            h2 = _rb(_rb(_rb(_rb(x1 - _rb(mean)) * inv) * cb) + sb)
            xh_s[rows, :] = pltpu.bitcast(x1, u32) | (pltpu.bitcast(h2, u32) >> 16)
            out_s[rows, :] = (x1 + _rb(gb * h2)).astype(bf16)
            wr = wr_s[...].astype(f32)
            prod = h2[:, 0:D] * wr[0:1]
            for j in range(1, M // D):
                prod = prod + h2[:, j * D:(j + 1) * D] * wr[j:j + 1]
            r = jnp.broadcast_to(_rb(jnp.sum(prod, axis=1, keepdims=True)), (n, D))
            bits = lax.bitcast_convert_type(r, i32)
            code = lax.shift_right_logical(bits, 16)
            code = jnp.where(bits < 0, 0xFFFF - code, code + 0x8000)
            code = jnp.where(r == 0.0, 0x8000, code)
            code = jnp.where(r != r, 0, code)
            key = code * S + (S - 1 + KEY0 - r0) - lax.broadcasted_iota(i32, (n, D), 0)
            key_s[pl.ds(off % T, n), :] = lax.bitcast_convert_type(key, f32)

        def select(tok=None):
            best = top_s[...]
            cols = [key_s[pl.ds(8 * t, 8), :] for t in range(T // 8)]
            flat = jnp.zeros((TOPK, D), f32)
            for t, col in enumerate(cols):
                flat = jnp.where(lane - sub == 8 * t, col, flat)
            new = None
            for cand in (flat, jnp.where(lane == sub, best, 0.0)):
                cand = jnp.broadcast_to(jnp.max(cand, axis=0, keepdims=True), (TOPK, D))
                above = sum((col > cand).astype(f32) for col in cols + [best])
                rank = jnp.sum(above, axis=0, keepdims=True)
                pick = jnp.where(rank == sub.astype(f32), cand, 0.0)
                new = pick if new is None else jnp.maximum(new, pick)
            top_s[...] = jnp.broadcast_to(jnp.max(new, axis=1, keepdims=True), (TOPK, D))

        def epilogues(r0, slot, rows=RB, n=16):
            jobs = []
            for off in range(0, rows, n):
                jobs.append(functools.partial(epilogue, r0 + off, slot, off, n))
                if (off + n) % T == 0:
                    jobs.append(select)
            return jobs

        def flip(src, dst, f0, n):
            def job(f, tok):
                _after(tok, zero, src)
                f = jnp.minimum(f, NF - 1)
                dst[f] = src[pl.ds(pl.multiple_of(jnp.minimum(f * D, F - D), 64), D), :].T
            return [functools.partial(job, f0 + t) for t in range(n)]

        NR = S // RB
        top_s[...] = jnp.zeros(top_s.shape, f32)
        last = oproj((NR - 1) * RB, RB, 1)
        cuts = [0] * 4 + [len(last) * n // 15 for n in range(1, 16)]
        _attention(q_s, k_s, v_s, 0, H - 1, 1, lambda n: _weave(last[cuts[n]:cuts[n + 1]]), lag=0)

        def blocks(n, _):
            b = NR - 2 - 2 * n
            _weave(oproj(b * RB, RB, 0), epilogues((b + 1) * RB, 1) + _skip(2),
                   flip(wg_s, wgu_s[0], 5 * n, 5))
            out_copy(b + 1).start()
            _weave(oproj((b - 1) * RB, RB, 1), epilogues(b * RB, 0) + _skip(2),
                   flip(wu_s, wgu_s[1], 5 * n, 5) + _skip(1))
            out_copy(b).start()

        lax.fori_loop(0, NR // 2 - 1, blocks, None)
        _weave(oproj(T, T, 0), epilogues(RB, 1))
        out_copy(1).start()
        _weave(oproj(0, T, 1), epilogues(T, 0, T) + _skip(2))
        _weave(epilogues(0, 1, T, T))
        out_copy(0).start()

        top = lax.bitcast_convert_type(top_s[...], i32) - KEY0
        sel = S - 1 - (top & (S - 1))
        code = lax.shift_right_logical(top, 11)
        code = jnp.where(code >= 0x8000, code - 0x8000, 0xFFFF - code)
        r_sel = lax.bitcast_convert_type(code * 0x10000, f32)[:, 0:1]
        idx = [sel[j, 0] for j in range(TOPK)]

        both = jnp.concatenate([xh_s[pl.ds(t, 1), :] for t in idx], axis=0)
        hsel = pltpu.bitcast(both << 16, f32)
        xsel = pltpu.bitcast((both >> 16) << 16, f32)
        lhs = jnp.concatenate([hsel, hsel], axis=0).astype(bf16)
        acts = []
        for f in range(NF):
            gate = _rb(_dot(lhs, wgu_s[0][f]))
            acts.append(_rb(gate * _sigmoid(gate)) * _rb(_dot(lhs, wgu_s[1][f])))
        seen = lax.broadcasted_iota(i32, acts[-1].shape, 1) < NF * D - F
        acts[-1] = jnp.where(seen, 0.0, acts[-1])
        y = sum(_dot(act.astype(bf16), wd_s[pl.ds(min(f * D, F - D), D), :])
                for f, act in enumerate(acts))
        y = _rb(_rb(y[0:TOPK]) * _sigmoid(r_sel))
        fixed = xsel + _rb(mod(5) * _rb(hsel + y))

        wait([out_copy(b) for b in range(NR)])
        tiles = [pl.multiple_of(t & -16, 16) for t in idx]
        row = lax.broadcasted_iota(i32, (16, M), 0)
        for j in range(TOPK):
            cur = out_s[pl.ds(tiles[j], 16), :].astype(f32)
            cur = jnp.where(row == idx[j] - tiles[j], fixed[j:j + 1], cur)
            out_s[pl.ds(tiles[j], 16), :] = cur.astype(bf16)

        def fix_copy(j):
            return pltpu.make_async_copy(out_s.at[pl.ds(tiles[j], 16)], out_hbm.at[pl.ds(tiles[j], 16)],
                                         fix_sem.at[j])

        fresh = []
        for j in range(TOPK):
            new = tiles[j] >= 0
            for k in range(j):
                new = jnp.logical_and(new, tiles[j] != tiles[k])
            fresh.append(new)
        for j in range(TOPK):
            pl.when(fresh[j])(fix_copy(j).start)
        for j in range(TOPK):
            pl.when(fresh[j])(fix_copy(j).wait)

    pl.run_scoped(phase3, V((S, M), u32), V((S, M), bf16), [V((NF, M, D), bf16)] * 2, V((T, D), f32),
                  [V((RB + PAD, M), f32)] * 2, V((TOPK, D), f32))


@jax.jit
def pallas_adaLN_cond__compressed_kv_cla__moe_arch_mod__prompt_kernel(
    A_x: jax.Array,
    A_c_kv: jax.Array,
    A_w_q: jax.Array,
    A_w_uk: jax.Array,
    A_w_uv: jax.Array,
    A_w_o: jax.Array,
    B_x: jax.Array,
    B_w_r: jax.Array,
    B_w_gate: jax.Array,
    B_w_up: jax.Array,
    B_w_down: jax.Array,
    c: jax.Array,
    w_mod: jax.Array,
):
    del B_x
    V = pltpu.VMEM
    scratch = [
        V((H, S // 2, D), u32),
        V((H + M // D, S // 2, D), u32),
        V((2, S // 2, D), u32), V((2, S // 2, D), u32), V((S // 2, C), u32),
        V((H * D, M), bf16), V((S + PAD, M), bf16),
        V((F + PAD, M), bf16), V((F + PAD, M), bf16), V((F, M), bf16),
        V((1, 6 * M), f32), V((M // D, D), bf16),
        pltpu.SemaphoreType.DMA((19,)), pltpu.SemaphoreType.DMA((S // RB,)),
        pltpu.SemaphoreType.DMA((TOPK,)),
    ]
    out = pl.pallas_call(
        _kernel,
        in_specs=[pl.BlockSpec(memory_space=pltpu.HBM)] * 12,
        out_specs=pl.BlockSpec(memory_space=pltpu.HBM),
        out_shape=jax.ShapeDtypeStruct((S, M), bf16),
        scratch_shapes=scratch,
        compiler_params=pltpu.CompilerParams(vmem_limit_bytes=120 * 2 ** 20),
    )(A_x.reshape(S, M), A_c_kv.reshape(S, C), A_w_q, A_w_uk, A_w_uv, A_w_o.reshape(H * D, M),
      B_w_r.reshape(M // D, D), B_w_gate.T, B_w_up.T, B_w_down, c, w_mod)
    return out.reshape(A_x.shape)
```
